```python
import jax
import jax.numpy as jnp

def _softmax(x, axis=-1):
    return jax.nn.softmax(x, axis=axis)

def _gelu(x):
    return jax.nn.gelu(x, approximate=True)

def _silu(x):
    return jax.nn.silu(x)

def _sigmoid(x):
    return jax.nn.sigmoid(x)

def _layernorm(x, axis=-1, eps=1e-05):
    m = jnp.mean(x, axis=axis, keepdims=True)
    v = jnp.var(x, axis=axis, keepdims=True)
    return (x - m) / jnp.sqrt(v + eps)

def _scatter_add(tgt, idx, src, axis=0):
    return tgt.at[idx].add(src)

def _segment_sum(src, seg, n):
    return jax.ops.segment_sum(src, seg, n)

class _Rng:

    def __init__(self, key):
        self._k = key

    def _next(self):
        self._k, sub = jax.random.split(self._k)
        return sub

    def normal(self, shape):
        return jax.random.normal(self._next(), shape, dtype=jnp.bfloat16)

    def randint(self, lo, hi, shape):
        return jax.random.randint(self._next(), shape, lo, hi, dtype=jnp.int32)

    def uniform(self, shape, lo=0.0, hi=1.0):
        return jax.random.uniform(self._next(), shape, jnp.bfloat16, lo, hi)

    def permutation(self, n):
        return jax.random.permutation(self._next(), n)
kernel_name = 'concat_heads__sliding_local_dilated__memory_aug_recurrent_mem_tr__prompt'

def setup_inputs():
    _rng = _Rng(jax.random.key(int.from_bytes(__import__("os").urandom(4), "little")))
    _w = lambda a: (lambda t: t.astype(jnp.bfloat16) if jnp.issubdtype(t.dtype, jnp.floating) else t)(jnp.asarray(a))

    def _A_setup():
        B, S, D = (1, 2048, 640)
        return {'x': _w((lambda *s: _rng.normal(s) * 0.05)(B, S, D)), 'wqkv': _w((lambda *s: _rng.normal(s) * 0.05)(D, 3 * D)), 'wo': _w((lambda *s: _rng.normal(s) * 0.05)(D, D))}
    _A_in = _A_setup()

    def _B_setup():
        B, S, Dm = (1, 2048, 640)
        H, Dh = (32, 192)
        M, seg = (8, 32)
        seg = min(seg, S)
        S = S // seg * seg
        return {'x': _w((lambda *s: _rng.normal(s) * 0.05)(B, S, Dm)), 'mem0': _w((lambda *s: _rng.normal(s) * 0.05)(B, M, Dm)), 'Wq': _w((lambda *s: _rng.normal(s) * 0.05)(Dm, H, Dh) * Dm ** (-0.5)), 'Wk': _w((lambda *s: _rng.normal(s) * 0.05)(Dm, H, Dh) * Dm ** (-0.5)), 'Wv': _w((lambda *s: _rng.normal(s) * 0.05)(Dm, H, Dh) * Dm ** (-0.5)), 'Wo': _w((lambda *s: _rng.normal(s) * 0.05)(H, Dh, Dm) * (H * Dh) ** (-0.5)), 'seg_len': seg}
    _B_in = _B_setup()
    return {'A_x': _A_in['x'], 'A_wqkv': _A_in['wqkv'], 'A_wo': _A_in['wo'], 'B_x': _B_in['x'], 'B_mem0': _B_in['mem0'], 'B_Wq': _B_in['Wq'], 'B_Wk': _B_in['Wk'], 'B_Wv': _B_in['Wv'], 'B_Wo': _B_in['Wo'], 'B_seg_len': _B_in['seg_len']}

def reference(A_x, A_wqkv, A_wo, B_x, B_mem0, B_Wq, B_Wk, B_Wv, B_Wo, B_seg_len):

    def _A_ref(x, wqkv, wo):
        B, S, D = x.shape
        H = 32
        Dh = D // H
        W, dil = (8, 2)
        qkv = (lambda x, *d: x.transpose(*d))((x @ wqkv).reshape(B, S, 3, H, Dh), 2, 0, 3, 1, 4)
        q, k, v = (qkv[0], qkv[1], qkv[2])
        scale = Dh ** (-0.5)
        pos = jnp.arange(S)
        off = jnp.arange(W) * dil
        idx = pos[:, None] - off[None, :]
        mask = idx >= 0
        idx_c = jnp.where(mask, idx, 0).reshape(-1)
        kg = k[:, :, idx_c, :].reshape(B, H, S, W, Dh)
        vg = v[:, :, idx_c, :].reshape(B, H, S, W, Dh)
        logits = jnp.einsum('bhsd,bhswd->bhsw', q, kg) * scale
        logits = jnp.where(mask[None, None, :, :], logits, -1000000000.0)
        attn = _softmax(logits, axis=-1)
        o = jnp.einsum('bhsw,bhswd->bhsd', attn, vg)
        return (lambda x, *d: x.transpose(*d))(o, 0, 2, 1, 3).reshape(B, S, D) @ wo

    def _B_ref(x, mem0, Wq, Wk, Wv, Wo, seg_len):
        B, S, Dm = x.shape
        H, Dh = (Wq.shape[1], Wq.shape[2])
        M = mem0.shape[1]
        scale = Dh ** (-0.5)
        n_seg = S // seg_len
        L = M + seg_len
        idx = jnp.arange(L)
        mask = (idx[:, None] < M) | (idx[:, None] >= idx[None, :])
        mem = mem0
        outs = []
        for s in range(n_seg):
            xs = x[:, s * seg_len:(s + 1) * seg_len, :].copy()
            h = jnp.concatenate([mem, xs], axis=1)
            q = jnp.einsum('btd,dhe->bhte', h, Wq)
            k = jnp.einsum('btd,dhe->bhte', h, Wk)
            v = jnp.einsum('btd,dhe->bhte', h, Wv)
            scores = jnp.einsum('bhqe,bhke->bhqk', q, k) * scale
            scores = jnp.where(mask[None, None], scores, -1000000000.0)
            p = _softmax(scores, axis=-1)
            o = jnp.einsum('bhqk,bhke->bhqe', p, v)
            o = jnp.einsum('bhte,hed->btd', o, Wo)
            mem = o[:, :M, :].copy()
            outs.append(o[:, M:, :])
        return jnp.concatenate(outs, axis=1)
    a = _A_ref(A_x, A_wqkv, A_wo)
    b = _B_ref(B_x, B_mem0, B_Wq, B_Wk, B_Wv, B_Wo, B_seg_len)
    return jnp.concatenate([a, b], axis=-1)
```

```python
import functools

import jax
import jax.numpy as jnp
from jax import lax
from jax.experimental import pallas as pl
from jax.experimental.pallas import tpu as pltpu

F32, BF16, U32 = jnp.float32, jnp.bfloat16, jnp.uint32
NT = (((1,), (1,)), ((), ()))
MASKED = -1000000000.0

S, D = 2048, 640
LT = D // 128

AH, AD, AW, ADIL = 32, 20, 8, 2
HALO = 16
TB = 128
NB = S // TB
RC = 8

H, DH, M, SEG = 32, 192, 8, 32
L = M + SEG
HALF = SEG // 2
NP = H // 2
NSEG = S // SEG
NF = H * DH // 128
NC = 3 * NF
SUMS = [(i, j) for i in range(LT) for j in range(i + 1, LT)]
MIXES = [(i, j) for i in range(LT) for j in range(LT) if i != j]


class _Group:
    def __init__(self, first, u_diag, w_diag, base):
        self.us = [(first + n, i) for n, i in enumerate(u_diag)]
        self.ws = [(first + len(u_diag) + n, j) for n, j in enumerate(w_diag)]
        self.pairs = [(u, i, w, j) for u, i in self.us for w, j in self.ws if i != j]
        paired = [(u, j) for u, i, w, j in self.pairs] + [(w, i) for u, i, w, j in self.pairs]
        self.direct = [(c, k) for c, d in self.us + self.ws for k in range(LT)
                       if k != d and (c, k) not in paired]
        names = [(sign, c) for sign in "-+" for c, _ in self.us + self.ws]
        names += [("cell", c, k) for c, k in paired + self.direct]
        names += [("both", u, w) for u, i, w, j in self.pairs]
        self.slot = {name: base + n for n, name in enumerate(names)}


def _groups(n, u_last, w_last):
    groups = [_Group(10 * g, range(LT), range(LT), 80 * g) for g in range(n // 10)]
    return groups + [_Group(n // 10 * 10, u_last, w_last, n // 10 * 80)]


GQ = _groups(NC, (0, 1), (2, 3))
GO = _groups(NF, (0, 1, 2, 3), (1, 2, 3, 4))


def _ds(i, n):
    return pl.ds(i * n if isinstance(i, int) else pl.multiple_of(i * n, n), n)


def _dot(a, b):
    return jnp.dot(a, b, preferred_element_type=F32)


def _add(a, b):
    return b if a is None else a + b


def _sub(a, b):
    return -b if a is None else a - b


def _vregs(x):
    return [x[r:r + 8] for r in range(0, x.shape[0], 8)]


def _cat(vs):
    return jnp.concatenate(vs, axis=0)


def _share(tasks, k, n):
    return tasks[k * len(tasks) // n:(k + 1) * len(tasks) // n]


def _run(tasks):
    for task in tasks:
        task()


def _block_diag(t0, t1, t2):
    lane = lax.broadcasted_iota(jnp.int32, (L, 128), 1)
    zero = jnp.zeros((L, 128), F32)
    top = jnp.concatenate([t0, jnp.where(lane < 64, t1, 0.0), zero], axis=1)
    bot = jnp.concatenate([zero, jnp.where(lane >= 64, t1, 0.0), t2], axis=1)
    return jnp.concatenate([top, bot], axis=0).astype(BF16)


def _kernel(ax_hbm, awqkv_hbm, awo_hbm, bx_hbm, mem_hbm, wq_hbm, wk_hbm, wv_hbm, wo_hbm,
            out_hbm,
            ax, awqkv, awo, tmp, wqkv_p, wo_p, q_s, kv_s, oa_s, outa,
            bx, mem, raw, wq, wo, mem_s, f_one, f_sum, f_dif, f_mix, cols0, cols1, part, att, keep, out_a, out_b, outb,
            sem_a, sem_x, sem_w, sem_b, sem_wo, sem_o):
    cp = pltpu.make_async_copy

    def rows_copy(src, dst, r0, r1, sem):
        return cp(src.at[pl.ds(r0, r1 - r0), :], dst.at[pl.ds(r0, r1 - r0), :], sem)

    c_wqkv = [cp(awqkv_hbm.at[:, pl.ds(j * D, D)], awqkv.at[j], sem_a.at[j]) for j in range(3)]
    c_awo = cp(awo_hbm, awo, sem_a.at[3])
    x_cuts = (0, 2 * TB, 4 * TB, S)
    c_ax = [rows_copy(ax_hbm, ax, x_cuts[c], x_cuts[c + 1], sem_x.at[c]) for c in range(3)]
    c_mem = cp(mem_hbm, mem, sem_b.at[0])
    c_bx0 = rows_copy(bx_hbm, bx, 0, 5 * SEG, sem_b.at[1])
    c_bx1 = rows_copy(bx_hbm, bx, 5 * SEG, S, sem_b.at[2])
    c_wo = [rows_copy(wo_hbm, raw, 1280 * g, min(1280 * g + 1280, H * DH), sem_wo.at[g]) for g in range(len(GO))]
    c_outa = cp(outa, out_hbm.at[:, pl.ds(0, D)], sem_o.at[0])

    def c_w(*pairs):
        return [cp(w.at[_ds(p, 384), :], raw.at[_ds(3 * p + j, 384), :], sem_w.at[p, j])
                for p in pairs for j, w in enumerate((wk_hbm, wq_hbm, wv_hbm))]

    def c_outb(r0, n):
        return cp(outb.at[pl.ds(r0, n), :], out_hbm.at[pl.ds(r0, n), pl.ds(D, D)], sem_o.at[1])

    def start(copies):
        for c in copies:
            c.start()

    def wait(copies):
        for c in copies:
            c.wait()

    def permute_rows(dst, base):
        for d in range(AD):
            for t in range(LT):
                dst[pl.ds((base + d * AH) // 2, AH // 2), t * 128:(t + 1) * 128] = pltpu.bitcast(
                    tmp[t, pl.ds(d, AH, stride=AD), :].astype(BF16), U32)

    def prep_wqkv(j):
        for t in range(LT):
            tmp[t] = awqkv[j, t * 128:(t + 1) * 128, :].astype(F32).T
        permute_rows(wqkv_p, j * D)

    def prep_wo():
        for t in range(LT):
            tmp[t] = awo[:, t * 128:(t + 1) * 128].astype(F32)
        permute_rows(wo_p, 0)

    def a_proj(i, b, j):
        w = pltpu.bitcast(wqkv_p[j * D // 2:(j + 1) * D // 2, :], BF16)
        r = lax.dot_general(ax[_ds(i, TB), :], w, NT, preferred_element_type=F32)
        for t in range(LT):
            rt = r[:, t * 128:(t + 1) * 128]
            if j == 0:
                q_s[b, t] = rt
                continue
            c = (j - 1) * LT + t
            kv_s[b, c, HALO:HALO + TB, :] = rt
            if isinstance(i, int) and i == 0:
                kv_s[b, c, 0:HALO, :] = jnp.broadcast_to(rt[0:1, :], (HALO, 128))
            else:
                kv_s[b, c, 0:HALO, :] = kv_s[1 - b, c, TB:TB + HALO, :]

    def a_attention(b, first_block=False):
        state = {}

        def window(c, r0, w):
            lo = HALO + r0 - ADIL * w
            return kv_s[b, c, lo:lo + RC, :]

        def logits(r0):
            q = [q_s[b, t, r0:r0 + RC, :] for t in range(LT)]
            state[r0] = []
            for w in range(AW):
                a = q[0] * window(0, r0, w)
                for t in range(1, LT):
                    a = a + q[t] * window(t, r0, w)
                state[r0].append(a + pltpu.roll(a, 2 * AH, 1))

        def fold(r0):
            state[r0] = [a + pltpu.roll(a, AH, 1) for a in state[r0]]

        def mix(r0):
            lg = []
            for w, a in enumerate(state.pop(r0)):
                a = a * (AD ** -0.5)
                if first_block and r0 < ADIL * w:
                    pos = lax.broadcasted_iota(jnp.int32, (RC, 128), 0) + r0
                    a = jnp.where(pos >= ADIL * w, a, MASKED)
                lg.append(a)
            m = functools.reduce(jnp.maximum, lg)
            e = [jnp.exp(a - m) for a in lg]
            inv = 1.0 / functools.reduce(jnp.add, e)
            p = [x * inv for x in e]
            for t in range(LT):
                o = p[0] * window(LT + t, r0, 0)
                for w in range(1, AW):
                    o = o + p[w] * window(LT + t, r0, w)
                oa_s[b, r0:r0 + RC, t * 128:(t + 1) * 128] = o

        n = TB // RC
        return [functools.partial(f, (k - lag) * RC) for k in range(n + 2)
                for lag, f in enumerate((logits, fold, mix)) if 0 <= k - lag < n]

    def a_out(i, b):
        outa[_ds(i, TB), :] = _dot(oa_s[b], pltpu.bitcast(wo_p[...], BF16)).astype(BF16)

    def a_stage(i, b, extra=(), first_block=False):
        side = a_attention(1 - b, first_block)
        for j in range(3):
            a_proj(i, b, j)
            _run(_share(side, j, 3) + _share(list(extra), j, 4))
        a_out(i - 1, 1 - b)
        _run(_share(list(extra), 3, 4))

    def w_prep(g, dst, shift=0):
        def tile(*name):
            return dst.at[g.slot[name] + 80 * shift]

        def copy(c, d, k):
            x = raw[_ds(c + 10 * shift, 128), k * 128:(k + 1) * 128]
            x = pltpu.bitcast(x.T if dst is wq else x, U32)
            (tile("+", c) if k == d else tile("cell", c, k))[...] = x

        def combine(r):
            def get(*name):
                return pltpu.bitcast(tile(*name)[r:r + 8], BF16).astype(F32)

            def put(x, *name):
                tile(*name)[r:r + 8] = pltpu.bitcast(x.astype(BF16), U32)
            minus = {c: get("+", c) for c, _ in g.us + g.ws}
            plus = dict(minus)
            for u, i, w, j in g.pairs:
                a, b = get("cell", u, j), get("cell", w, i)
                put(a + b, "both", u, w)
                if dst is wo:
                    a, b = b, a
                minus[u], plus[u], minus[w], plus[w] = minus[u] - a, plus[u] + b, minus[w] - b, plus[w] + a
            for c in minus:
                put(minus[c], "-", c)
                put(plus[c], "+", c)
        return ([functools.partial(copy, c, d, k) for c, d in g.us + g.ws for k in range(LT)],
                [functools.partial(combine, r) for r in range(0, 64, 8)])

    start([c_wqkv[0], c_ax[0], c_wqkv[1]])

    def touch(i, carry):
        for ref in (f_one, f_sum, f_dif, f_mix, cols0, cols1, part, att, keep, out_a, out_b):
            ref[i] = jnp.zeros(ref.shape[1:], F32)
        return carry
    lax.fori_loop(0, 2, touch, 0)
    c_wqkv[0].wait()
    c_wqkv[2].start()
    prep_wqkv(0)
    wait([c_ax[0], c_wqkv[1]])
    start([c_awo, c_ax[1]])
    a_proj(0, 0, 0)
    prep_wqkv(1)
    c_wqkv[2].wait()
    c_ax[2].start()
    a_proj(0, 0, 1)
    prep_wqkv(2)
    a_proj(0, 0, 2)
    c_awo.wait()
    start(c_w(0, 1))
    prep_wo()
    a_stage(1, 1, first_block=True)
    start(c_w(2, 3))

    def a_step(it, carry):
        def preps(i):
            return (w_prep(GQ[0], wq, jnp.where(i < 5, 12, i - 5))[1]
                    + w_prep(GQ[0], wq, jnp.where(i < 4, 13, i - 4))[0])

        @pl.when(it == 1)
        def _():
            c_ax[1].wait()

        @pl.when(it > 1)
        def _():
            @pl.when(it < 7)
            def _():
                start(c_w(2 * it + 2, 2 * it + 3))
            for k in range(2):
                @pl.when(it == 6 + k)
                def _():
                    start(c_wo[k:k + 1])

            @pl.when(it == 2)
            def _():
                wait(c_w(0, 1))
            wait(c_w(2 * it - 2, 2 * it - 1))

        a_stage(2 * it, 0, preps(2 * it))

        @pl.when(it == 1)
        def _():
            c_ax[2].wait()
            start([c_mem, c_bx0] + c_w(4, 5))
        a_stage(2 * it + 1, 1, preps(2 * it + 1))
        return carry

    lax.fori_loop(1, NB // 2, a_step, 0)
    wait(c_w(14, 15) + [c_mem, c_bx0])
    start(c_wo[2:])

    cols = (cols0, cols1)

    def tokens(s):
        return [bx[_ds(s, SEG), k * 128:(k + 1) * 128].astype(F32) for k in range(LT)]

    def qkv_group(odd, g, product, nm):
        pa, pb = (g.ws, g.us) if odd else (g.us, g.ws)
        h0 = 2 * odd

        def prod(lhs, *name):
            return product(lhs, wq.at[g.slot[name]])

        def direct(c, r):
            for _, k in [x for x in g.direct if x[0] == c]:
                r = list(map(_add, r, prod(lambda: f_one[odd, k, 0:SEG + nm], "cell", c, k)))
            return r
        parts = [pb[n:n + 3] for n in range(0, len(pb), 3)]
        for some in parts:
            same = {b: prod(lambda: _cat([f_dif[odd, j], f_one[odd, j, SEG:SEG + nm]]), "+", b) for b, j in some}
            for a, i in pa:
                mine = cols[1 - odd].at[a, M:L]
                other = cols1.at[a, M:L] if odd else part.at[a]
                half = slice(8 * h0, 8 * h0 + HALF)
                if some is parts[0]:
                    r = prod(lambda: f_one[odd, i, 0:SEG + nm], "-", a)
                    x = _cat(r[:4]) + other[...] if odd else _cat(r[:4])
                    other[HALF - 8 * h0:SEG - 8 * h0] = x[HALF - 8 * h0:SEG - 8 * h0]
                    cross = _vregs(x[half])
                    r = direct(a, r)
                else:
                    r, cross = _vregs(mine[...]) + _vregs(cols[odd][a, 0:nm]), _vregs(other[half])
                for b, j in some:
                    if i != j:
                        x = prod(lambda: f_sum[odd, SUMS.index((min(i, j), max(i, j))), 0:SEG + nm], "cell", a, j)
                        r = list(map(_add, r, x))
                        same[b] = list(map(_sub, same[b], x))
                        x = prod(lambda: _cat([f_mix[odd, MIXES.index((i, j))], f_one[odd, i, SEG:SEG + nm]]),
                                 "both", *((b, a) if odd else (a, b)))
                        cross = list(map(_add, cross, x))
                        for y, h in zip(x, [h0, h0 + 1] + list(range(4, len(r)))):
                            same[b][h] = same[b][h] + y
                mine[...], cols[odd][a, 0:nm], other[half] = _cat(r[:4]), _cat(r[4:]), _cat(cross)
            for b, _ in some:
                r = direct(b, same[b])
                cols[odd][b, 0:nm] = _cat(r[4:])
                cols[1 - odd][b, M:L] = part[b] + _cat(r[:4]) if odd else _cat(r[:4])

    def out_groups(odd, gs, same, cross, product, last=False):
        h0, nh = (0, SEG * odd) if last else (2 - 2 * odd, HALF)

        def xa(c, r0=0, n=SEG):
            return att[c, M + SEG * (1 - odd) + r0:M + SEG * (1 - odd) + r0 + n]

        def xb(c, r0=0, n=SEG):
            return att[c, L + r0:L + r0 + n] if odd else keep[c, r0:r0 + n]

        def xm(c):
            return att[c, 0:M]

        def prod(g, m, x, *name):
            r = product(lambda: x() if last else _cat([m(), x()]), wo.at[g.slot[name]])
            return r if last else r[1:] + r[:1]
        sides = [(g, {d: c for c, d in (g.us if odd else g.ws)}, {d: c for c, d in (g.ws if odd else g.us)})
                 for g in gs]
        for i in range(LT):
            shared = None
            for g, pa, pb in sides:
                rs = [prod(g, lambda: xm(pb[i]), lambda: xa(pb[i]) - xb(pb[i]), "+", pb[i])] if i in pb else []
                rs += [prod(g, lambda: xm(c), lambda: xa(c), "cell", c, k) for c, k in g.direct if k == i]
                for r in rs:
                    same[i] = list(map(_add, same[i], r))
                if i in pa:
                    r = prod(g, lambda: xm(pa[i]), lambda: xa(pa[i]), "-", pa[i])
                    shared = list(map(_add, shared or [None] * 5, r))
                    if odd:
                        keep[pa[i]] = xa(pa[i])
            same[i] = list(map(_add, same[i], shared))
            cross[i] = list(map(_add, cross[i], shared))
            for j in range(i + 1, LT):
                diff = None
                for s, t in ((i, j), (j, i)):
                    mix = None
                    for g, pa, pb in sides:
                        if s in pa and t in pb:
                            a, b = pa[s], pb[t]
                            r = prod(g, lambda: xm(a) + xm(b), lambda: xa(a) + xa(b), "cell", b, s)
                            diff = list(map(_add if s == i else _sub, diff or [None] * 5, r))
                            if nh:
                                r = prod(g, lambda: xm(a), lambda: xa(a, 8 * h0, nh) + xb(b, 8 * h0, nh),
                                         "both", *((a, b) if odd else (b, a)))
                                mix = list(map(_add, mix or [None] * 4, r))
                    for x, h in zip(mix or [], list(range(h0, h0 + nh // 8)) + [4]):
                        same[t][h] = _add(same[t][h], x)
                        if h < 4:
                            cross[s][h] = _add(cross[s][h], x)
                same[i] = list(map(_add, same[i], diff))
                same[j] = list(map(_sub, same[j], diff))

    def project_out(odd, s, product, last=False):
        same, cross = [[None] * 5 for _ in range(LT)], [[None] * 4 for _ in range(LT)]
        for gs in (GO[:3], GO[3:]):
            out_groups(odd, gs, same, cross, product, last)
        for k in range(LT):
            lanes = slice(k * 128, (k + 1) * 128)
            if odd:
                out_a[k], out_b[k] = _cat(same[k][:4]), _cat(cross[k])
            else:
                outb[_ds(s - 2, SEG), lanes] = (out_a[k] + _cat(cross[k])).astype(BF16)
                outb[_ds(s - 1, SEG), lanes] = (out_b[k] + _cat(same[k][:4])).astype(BF16)
        return [x[-1] for x in same]

    def attend(odd, s, m, events):
        xa, xb = tokens(jnp.minimum(s + 1, NSEG - 1)), tokens(s if odd else jnp.minimum(s + 2, NSEG - 1))
        nm = m[0].shape[0]
        rows = slice(HALF * odd, HALF * odd + HALF)
        for k in range(LT):
            f_one[odd, k, 0:SEG + nm] = _cat([xa[k], m[k]])
            f_dif[odd, k] = xa[k] - xb[k]
        for n, (i, j) in enumerate(SUMS):
            f_sum[odd, n, 0:SEG + nm] = _cat([xa[i] + xa[j], m[i] + m[j]])
        for n, (i, j) in enumerate(MIXES):
            f_mix[odd, n] = xa[i][rows] + xb[j][rows]

        row = lax.broadcasted_iota(jnp.int32, (L, 2 * L), 0)
        col = lax.broadcasted_iota(jnp.int32, (L, 2 * L), 1)
        head0 = col < L
        visible = (row < M) | (row >= jnp.where(head0, col, col - L))
        st = {}

        def operand(j, p):
            return [cols[odd][9 * p + 3 * j + t] for t in range(3)]

        def score(p):
            q = jnp.concatenate(operand(1, p), axis=1)
            sc = lax.dot_general(q, _block_diag(*operand(0, p)), NT, preferred_element_type=F32)
            st[p] = jnp.where(visible, sc * (DH ** -0.5), MASKED)

        def shift(p):
            m0 = jnp.max(jnp.where(head0, st[p], -jnp.inf), axis=1, keepdims=True)
            m1 = jnp.max(jnp.where(head0, -jnp.inf, st[p]), axis=1, keepdims=True)
            st[p] = st[p] - jnp.where(head0, m0, m1)

        def normalize(p):
            e = jnp.exp(st[p])
            l0 = jnp.sum(jnp.where(head0, e, 0.0), axis=1, keepdims=True)
            l1 = jnp.sum(jnp.where(head0, 0.0, e), axis=1, keepdims=True)
            st[p] = e / jnp.where(head0, l0, l1)

        def pv(p):
            r = _dot(st[p], _block_diag(*operand(2, p)))
            for t in range(3):
                att[3 * p + t, 0:M] = r[0:M, t * 128:(t + 1) * 128]
                att[3 * p + t, M + SEG * odd:L + SEG * odd] = r[M:L, t * 128:(t + 1) * 128]

        for p in range(NP):
            ready = min((9 * p + 15) // 10 * 50, LT * NC)
            for f, lag in ((score, 20), (shift, 40), (normalize, 60), (pv, 85)):
                events.setdefault(ready + lag, []).append(functools.partial(f, p))
        count = [0]

        def product(lhs, rhs):
            _run(events.pop(count[0], []))
            count[0] += 1
            return _vregs(_dot(lhs(), pltpu.bitcast(rhs[...], BF16) if rhs.dtype == U32 else rhs[...]))
        for g in GQ:
            qkv_group(odd, g, product, nm)
        return product

    events = {}

    def spread(tasks, t0, t1):
        for t in range(t0, t1):
            events.setdefault(t, []).extend(_share(tasks, t - t0, t1 - t0))
    preps = [w_prep(g, wq) for g in GQ]
    spread(a_attention(1), 0, 200)
    spread(preps[11][1] + preps[12][0], 0, 150)
    spread(preps[12][1] + preps[13][0], 150, 300)
    spread(preps[13][1] + preps[14][0] + preps[14][1], 300, 500)
    preps = [sum(w_prep(g, wo), []) for g in GO]
    t_wait = 50 * 10
    spread([lambda: wait(c_wo[:3])] + preps[0] + preps[1] + preps[2], t_wait, LT * NC)
    spread([lambda: wait(c_wo[3:]), c_bx1.start, lambda: a_out(NB - 1, 1)], LT * NC, LT * NC + 1)
    spread(preps[3] + preps[4], LT * NC + 1, LT * (NC + NF))
    product = attend(0, 0, [_cat([mem[:, k * 128:(k + 1) * 128].astype(F32), x]) for k, x in enumerate(tokens(0))],
                     events)
    m = [None] * LT
    for c in range(NF):
        for k in range(LT):
            m[k] = _add(m[k], product(lambda: att[c, 0:M], raw.at[c * 128:(c + 1) * 128, k * 128:(k + 1) * 128])[0])
    for k in range(LT):
        mem_s[k] = m[k]
    c_outa.start()

    def b_step(n, carry):
        @pl.when(n == 1)
        def _():
            c_bx1.wait()
        m = project_out(1, 2 * n + 1, attend(1, 2 * n + 1, [mem_s[k] for k in range(LT)], {}))
        m = project_out(0, 2 * n + 2, attend(0, 2 * n + 2, m, {}))
        for k in range(LT):
            mem_s[k] = m[k]
        c_outb(pl.multiple_of(2 * n * SEG, SEG), 2 * SEG).start()
        return carry

    lax.fori_loop(0, NSEG // 2 - 1, b_step, 0)
    product = attend(1, NSEG - 1, [mem_s[k] for k in range(LT)], {})
    project_out(1, NSEG - 1, product, last=True)
    project_out(0, NSEG, product, last=True)
    c_outb(S - 2 * SEG, 2 * SEG).start()
    c_outa.wait()
    c_outb(0, S).wait()


def pallas_concat_heads__sliding_local_dilated__memory_aug_recurrent_mem_tr__prompt_kernel(
    A_x, A_wqkv, A_wo, B_x, B_mem0, B_Wq, B_Wk, B_Wv, B_Wo, B_seg_len,
):
    assert B_seg_len == SEG
    assert A_x.shape == B_x.shape == (1, S, D) and B_mem0.shape == (1, M, D)
    assert B_Wq.shape == B_Wk.shape == B_Wv.shape == (D, H, DH) and B_Wo.shape == (H, DH, D)
    vmem, dma = pltpu.VMEM, pltpu.SemaphoreType.DMA
    call = pl.pallas_call(
        _kernel,
        out_shape=jax.ShapeDtypeStruct((S, 2 * D), BF16),
        in_specs=[pl.BlockSpec(memory_space=pl.ANY)] * 9,
        out_specs=pl.BlockSpec(memory_space=pl.ANY),
        scratch_shapes=[
            vmem((S, D), BF16),
            vmem((3, D, D), BF16),
            vmem((D, D), BF16),
            vmem((LT, D, 128), F32),
            vmem((3 * D // 2, D), U32),
            vmem((D // 2, D), U32),
            vmem((2, LT, TB, 128), F32),
            vmem((2, 2 * LT, HALO + TB, 128), F32),
            vmem((2, TB, D), F32),
            vmem((S, D), BF16),
            vmem((S, D), BF16),
            vmem((M, D), BF16),
            vmem((NC * 128, D), BF16),
            vmem((max(GQ[-1].slot.values()) + 1, 64, 128), U32),
            vmem((max(GO[-1].slot.values()) + 1, 64, 128), U32),
            vmem((LT, M, 128), F32),
            vmem((2, LT, L + SEG, 128), F32),
            vmem((2, len(SUMS), L + SEG, 128), F32),
            vmem((2, LT, SEG, 128), F32),
            vmem((2, len(MIXES), HALF, 128), F32),
            vmem((NC, L, 128), F32), vmem((NC, L, 128), F32),
            vmem((NC, SEG, 128), F32),
            vmem((NF, L + SEG, 128), F32),
            vmem((NF, SEG, 128), F32),
            vmem((LT, SEG, 128), F32), vmem((LT, SEG, 128), F32),
            vmem((S, D), BF16),
            dma((4,)), dma((3,)), dma((NP, 3)), dma((3,)), dma((len(GO),)), dma((2,)),
        ],
        compiler_params=pltpu.CompilerParams(vmem_limit_bytes=120 * 1024 * 1024),
        name="sliding_and_memory_attention",
    )

    def by_feature(w):
        return w.transpose(1, 2, 0).reshape(H * DH, D)

    out = call(A_x.reshape(S, D), A_wqkv, A_wo, B_x.reshape(S, D), B_mem0.reshape(M, D),
               by_feature(B_Wq), by_feature(B_Wk), by_feature(B_Wv), B_Wo.reshape(H * DH, D))
    return out.reshape(1, S, 2 * D)
```

```python
import functools

import jax
import jax.numpy as jnp
from jax import lax
from jax.experimental import pallas as pl
from jax.experimental.pallas import tpu as pltpu

F32, BF16, U32 = jnp.float32, jnp.bfloat16, jnp.uint32
NT = (((1,), (1,)), ((), ()))
MASKED = -1000000000.0
LOG2E = 1.4426950408889634

S, D = 2048, 640
LT = D // 128

AH, AD, AW, ADIL = 32, 20, 8, 2
HALO = 16
TB = 128
NB = S // TB
RC = 8

H, DH, M, SEG = 32, 192, 8, 32
L = M + SEG
HALF = SEG // 2
NP = H // 2
NSEG = S // SEG
NF = H * DH // 128
NC = 3 * NF
SUMS = [(i, j) for i in range(LT) for j in range(i + 1, LT)]
MIXES = [(i, j) for i in range(LT) for j in range(LT) if i != j]


class _Group:
    def __init__(self, first, u_diag, w_diag):
        self.us = [(first + n, i) for n, i in enumerate(u_diag)]
        self.ws = [(first + len(u_diag) + n, j) for n, j in enumerate(w_diag)]
        self.pairs = [(u, i, w, j) for u, i in self.us for w, j in self.ws if i != j]
        paired = [(u, j) for u, i, w, j in self.pairs] + [(w, i) for u, i, w, j in self.pairs]
        self.direct = [(c, k) for c, d in self.us + self.ws for k in range(LT)
                       if k != d and (c, k) not in paired]
        sums = [(sign, c) for sign in "-+" for c, _ in self.us + self.ws]
        self.sums = sums + [("both", u, w) for u, i, w, j in self.pairs]
        self.first = first

    def tile(self, refs, name, shift=0):
        g = self.first // 10
        if name[0] != "cell" and g > 11:
            return refs[-2].at[40 * (g - 12) + self.sums.index(name)]
        if g > 12:
            return refs[2 + g % 2].at[LT * (name[1] - self.first) + name[2]]
        if name[0] != "cell":
            return refs[-1].at[40 * (g + shift) + self.sums.index(name)]
        if refs[0].shape[0] == LT:
            return refs[0].at[name[2], 64 * name[1]:64 * name[1] + 64]
        n = min(len(refs) - 1, 2)
        return refs[g % n].at[50 * (g // n + shift // n) + LT * (name[1] - self.first) + name[2]]


def _groups(n, u_last, w_last):
    groups = [_Group(10 * g, range(LT), range(LT)) for g in range(n // 10)]
    return groups + [_Group(n // 10 * 10, u_last, w_last)]


GQ = _groups(NC, (0, 1), (2, 3))
GO = _groups(NF, (0, 1, 2, 3), (1, 2, 3, 4))


def _ds(i, n):
    return pl.ds(i * n if isinstance(i, int) else pl.multiple_of(i * n, n), n)


def _dot(a, b):
    return jnp.dot(a, b, preferred_element_type=F32)


def _recip(x):
    r = pl.reciprocal(x, approx=True)
    return r * (2.0 - x * r)


def _add(a, b):
    return b if a is None else a + b


def _sub(a, b):
    return -b if a is None else a - b


def _vregs(x):
    return [x[r:r + 8] for r in range(0, x.shape[0], 8)]


def _cat(vs):
    return jnp.concatenate(vs, axis=0)


def _share(tasks, k, n):
    return tasks[k * len(tasks) // n:(k + 1) * len(tasks) // n]


def _run(tasks):
    for task in tasks:
        task()


class _Products:
    def __init__(self, events, tied):
        self.events, self.tied, self.results = events, tied, []
        self.count, self.usual, self.flushed, self.waiting = 0, 0, -1, {}

    def dot(self, x, w):
        self.results.append(_vregs(pltpu.bitcast(_dot(self.tied(x), pltpu.bitcast(w, BF16)), F32)))
        return self.results[-1]

    def tick(self):
        self.count += 1
        _run(self.events.pop(self.count - 1, []))

    def now(self, x, w):
        self.tick()
        r = self.dot(x(), w[...])
        self.passed(1)
        return r

    def soon(self, x, w, use):
        self.waiting.setdefault(x.shape[0], []).append([x, w[...], [use]])

    def after(self, rows, task):
        if self.waiting.get(rows):
            self.waiting[rows][-1][2].append(lambda r: task())
        else:
            task()

    def passed(self, n, last=False):
        self.usual += n
        for rows in sorted(self.waiting, reverse=True):
            queue = self.waiting[rows]
            while queue and (last or (len(queue) >= 4 and self.usual % 4 == 0
                                      and (self.flushed < self.usual or len(queue) >= 8 or rows >= L))):
                for x, w, uses in queue[:4]:
                    r = self.dot(x, w)
                    for use in uses:
                        use(r)
                del queue[:4]
                if rows < L:
                    self.flushed = self.usual


def _block_diag(t0, t1, t2):
    lane = lax.broadcasted_iota(jnp.int32, (L, 128), 1)
    zero = jnp.zeros((L, 128), F32)
    halves = [jnp.where(lane < 64, t1, 0.0), jnp.where(lane >= 64, t1, 0.0)]
    return [_cat(x).astype(BF16) for x in ([t0, zero], halves, [zero, t2])]


def _kernel(ax_hbm, awqkv_hbm, awo_hbm, bx_hbm, mem_hbm, wq_hbm, wk_hbm, wv_hbm, wo_hbm,
            out_hbm,
            ax, awqkv, awo, tmp, wqkv_p, wo_p, x_s, qkv0, qkv1, oa0, oa1, outa,
            bx, mem, raw, wq_c0, wq_c1, wq_s, wo_c, wo_s, wl_c0, wl_c1, wl_s, mem_s, f_one, f_sum, f_dif, f_mix, cols0, cols1, part, att, keep, out_a, out_b,
            sem_a, sem_x, sem_w, sem_wo, sem_o):
    cp = pltpu.make_async_copy
    outb = ax

    def rows_copy(src, dst, r0, r1, sem):
        return cp(src.at[pl.ds(r0, r1 - r0), :], dst.at[pl.ds(r0, r1 - r0), :], sem)

    c_wqkv = [cp(awqkv_hbm.at[:, pl.ds(j * D, D)], awqkv.at[j], sem_a.at[j]) for j in range(3)]
    c_awo = cp(awo_hbm, awo, sem_a.at[3])
    c_mem = cp(mem_hbm, mem, sem_a.at[4])

    c_bx = rows_copy(bx_hbm, bx, 2 * TB, S, sem_x.at[1, 1])

    def c_x(j, k):
        return cp((ax_hbm, bx_hbm)[j].at[_ds(k, 2 * TB), :], (ax, bx)[j].at[_ds(k, 2 * TB), :], sem_x.at[k, j])

    def by_tile(src, dst, rows, sem):
        return [cp(src.at[:, pl.ds(k * 128, 128)], dst.bitcast(BF16).at[k, rows], sem) for k in range(LT)]

    def tiles(t, n):
        return pl.ds(t * 128 if isinstance(t, int) else pl.multiple_of(t * 128, 128), n * 128)

    def get_wo(t, n):
        start(by_tile(wo_hbm.at[tiles(t, n)], wo_c, tiles(t, n), sem_wo))

    def get_w(t, n, batch):
        for j, w in enumerate((wk_hbm, wq_hbm, wv_hbm)):
            start(by_tile(w.at[tiles(t, n)], raw, tiles(j * NF + t, n), sem_w.at[batch]))

    def got_w(n, batch):
        cp(raw.at[:, 0:n * 192], raw.at[:, 0:n * 192], sem_w.at[batch]).wait()

    def c_out(j, rows):
        return cp((outa, outb)[j].at[rows, :], out_hbm.at[rows, pl.ds(j * D, D)], sem_o.at[j])

    def start(copies):
        for c in copies:
            c.start()

    def wait(copies):
        for c in copies:
            c.wait()

    def permute_rows(dst, base):
        for d in range(AD):
            for t in range(LT):
                dst[pl.ds((base + d * AH) // 2, AH // 2), t * 128:(t + 1) * 128] = pltpu.bitcast(
                    tmp[t, pl.ds(d, AH, stride=AD), :].astype(BF16), U32)

    def prep_wqkv(j):
        for t in range(LT):
            tmp[t] = awqkv[j, t * 128:(t + 1) * 128, :].astype(F32).T
        permute_rows(wqkv_p, j * D)

    def prep_wo():
        for t in range(LT):
            tmp[t] = awo[:, t * 128:(t + 1) * 128].astype(F32)
        permute_rows(wo_p, 0)

    qkv, oa = (qkv0, qkv1), (oa0, oa1)
    wq, wo = (wq_c0, wq_c1, wl_c0, wl_c1, wl_s, wq_s), (wo_c, wo_s)

    ties, step = [], [None]

    def tied(x):
        head = x[0:8, 0:128]
        while ties:
            ref = ties.pop()
            ref[...] = pltpu.bitcast(head, ref.dtype)
            head = pltpu.bitcast(ref[...], x.dtype)
        if x.shape[1] > 128:
            head = jnp.concatenate([head, x[0:8, 128:]], axis=1)
        return _cat([head, x[8:]]) if x.shape[0] > 8 else head

    def a_proj(i, b, c):
        if c == 0:
            x_s[b] = ax[_ds(i, TB), :].astype(F32)
        w = pltpu.bitcast(wqkv_p[c * 64:(c + 1) * 64, :], BF16)
        r = lax.dot_general(tied(x_s[b]), w, NT, preferred_element_type=F32)
        qkv[b][c, HALO:] = r
        if c >= LT and isinstance(i, int) and i == 0:
            qkv[b][c, 0:HALO] = jnp.broadcast_to(r[0:1, :], (HALO, 128))
        elif c >= LT:
            qkv[b][c, 0:HALO] = qkv[1 - b][c, TB:]
        return r

    def a_attention(b, first_block=False):
        state = {}

        def window(c, r0, w):
            lo = HALO + r0 - ADIL * w
            return qkv[b][LT + c, lo:lo + RC]

        def logits(r0):
            q = [qkv[b][t, HALO + r0:HALO + r0 + RC] for t in range(LT)]
            state[r0] = []
            for w in range(AW):
                a = functools.reduce(jnp.add, [q[t] * window(t, r0, w) for t in range(LT)])
                a = functools.reduce(jnp.add, [a] + [pltpu.roll(a, d, 1) for d in range(AH, 128, AH)])
                if first_block and r0 < ADIL * w:
                    pos = lax.broadcasted_iota(jnp.int32, (RC, 128), 0) + r0
                    a = jnp.where(pos >= ADIL * w, a, MASKED * AD ** 0.5)
                state[r0].append(a)

        def mix(r0):
            lg = state.pop(r0)
            m = functools.reduce(jnp.maximum, lg)
            e = [jnp.exp2((a - m) * (AD ** -0.5 * LOG2E)) for a in lg]
            inv = _recip(functools.reduce(jnp.add, e))
            for t in range(LT):
                o = e[0] * window(LT + t, r0, 0)
                for w in range(1, AW):
                    o = o + e[w] * window(LT + t, r0, w)
                oa[b][t, r0:r0 + RC] = o * inv

        n = TB // RC
        return [functools.partial(f, (k - lag) * RC) for k in range(n + 1)
                for lag, f in ((0, logits), (1, mix)) if 0 <= k - lag < n]

    def a_out(i, b, c):
        lanes = slice(c * 128, (c + 1) * 128)
        x = jnp.concatenate([oa[b][k] for k in range(LT)], axis=1)
        r = _dot(tied(x), pltpu.bitcast(wo_p[:, lanes], BF16))
        outa[_ds(i, TB), lanes] = r.astype(BF16)
        return r

    def paced(tasks, ref, results):
        for n, task in enumerate(tasks):
            x = pltpu.bitcast(results[n * len(results) // len(tasks)], ref.dtype)
            if ref.shape[0] == LT:
                ref[zero, ref.shape[1] - 8:] = x
            else:
                ref[ref.shape[0] - 1 + zero, 0:8] = x
            task()

    def tie(ref):
        ties.append(ref.at[ref.shape[0] - 1 + zero, 8:16])

    def a_stage(i, b, turn, combine):
        turn = [functools.partial(_run, turn[n:n + 2]) for n in range(0, len(turn), 2)]
        side = [(a_attention(1 - b), 0, 13, 2 + 1, qkv[1 - b], oa[1 - b]),
                (turn, 12, 4 * LT, 4, raw, wq[1 - b]),
                (combine[:40], 0, 13, 2, wq[b], wq_s),
                (combine[40:], 13, 4 * LT, 2, wq[b], wq_s)]
        rs = []
        for c in range(4 * LT):
            rs.append(_vregs(a_proj(i, b, c) if c < 3 * LT else a_out(i - 1, 1 - b, c - 3 * LT)))
            for tasks, c0, c1, lag, src, dst in side:
                if c0 <= c < c1:
                    if len(rs) < lag:
                        _run(_share(tasks, c - c0, c1 - c0))
                    else:
                        paced(_share(tasks, c - c0, c1 - c0), src, rs[-lag])
                    tie(dst)

    def w_turn(g, dst, shift=0):
        def turn(c, k):
            col = c + 10 * shift
            t = (col * 171) >> 9
            x = pltpu.bitcast(raw[k, _ds((col - 3 * t) * NF + t, 64)], BF16)
            g.tile(dst, ("cell", c, k), shift)[...] = pltpu.bitcast(x.T, U32)
        return [functools.partial(turn, c, k) for c, _ in g.us + g.ws for k in range(LT)]

    def w_combine(g, dst, shift=0):
        minus, plus = {}, {}

        def get(r, c, k):
            cell = g.tile(dst, ("cell", c, k), shift).at[r // 2:r // 2 + 8]
            return pltpu.bitcast(cell[...], BF16).astype(F32)

        def put(r, x, *name):
            g.tile(dst, name, shift)[r // 2:r // 2 + 8] = pltpu.bitcast(x.astype(BF16), U32)

        def combine(r, pairs):
            for pair in pairs:
                u, i, w, j = pair
                x, y = get(r, u, j), get(r, w, i)
                put(r, x + y, "both", u, w)
                if dst is wo:
                    x, y = y, x
                for c, d, own, other in ((u, i, x, y), (w, j, y, x)):
                    mine = [p for p in g.pairs if c in (p[0], p[2])]
                    if pair == mine[0]:
                        minus[c] = plus[c] = get(r, c, d)
                    minus[c], plus[c] = minus[c] - own, plus[c] + other
                    if pair == mine[-1]:
                        put(r, minus[c], "-", c)
                        put(r, plus[c], "+", c)
        return [functools.partial(combine, r, g.pairs[n:n + 1]) for r in range(0, 128, 16)
                for n in range(0, len(g.pairs), 1)]

    start([c_wqkv[0], c_x(0, 0), c_wqkv[1], c_wqkv[2]])

    def touch(i, carry):
        for ref in (x_s, f_one, f_sum, f_dif, f_mix, cols0, cols1, part, att, keep, out_a, out_b):
            ref[i] = jnp.zeros(ref.shape[1:], F32)
        for ref in wo[1:] + wq:
            ref[i] = jnp.zeros((64, 128), U32)
        return i
    zero = lax.shift_right_logical(lax.fori_loop(0, 2, touch, 0), 16)
    c_wqkv[0].wait()
    prep_wqkv(0)
    for j in range(2):
      c_wqkv[j + 1].wait()
      if j == 0:
          c_x(0, 0).wait()
      if j == 0:
          start([c_awo, c_x(0, 1)])
      else:
          get_w(0, 4, 0)
      prep_wqkv(j + 1)
      for n in range(2 * LT):
          a_proj(n // LT, n // LT, j * LT + n % LT)
    c_awo.wait()
    get_w(4, 6, 0)
    start([c_x(0, 2), c_mem, c_x(1, 0)])
    prep_wo()
    for n in range(2 * LT):
      a_proj(n // LT, n // LT, 2 * LT + n % LT)
    _run(a_attention(0, True))
    for c in range(LT):
      a_out(0, 0, c)

    def a_step(it, carry):
        @pl.when(it == 2)
        def _():
            got_w(10, 0)
            _run(w_turn(GQ[0], wq))

        @pl.when(it > 2)
        def _():
            got_w(7, it - 1)
        c_x(0, it).wait()

        @pl.when(it < 6)
        def _():
            get_w(3 + 7 * it, 4, it + 1)

        @pl.when(it < 7)
        def _():
            get_w(jnp.minimum(7 + 7 * it, NF - 3), 3, it + 1)

        @pl.when(it < 6)
        def _():
            c_x(0, it + 2).start()

        for n in range(3):
            @pl.when(it > 5)
            def _():
                get_wo(24 * (it - 6) + 8 * n, 8)
        for b in range(2):
            i = 2 * it + b
            a_stage(i, b, w_turn(GQ[1 - b], wq, jnp.where(i < 4, 10, 2 * it - 4 + 2 * b)),
                    w_combine(GQ[b], wq, jnp.where(i < 4, 10, 2 * it - 4)))
        ties.clear()
        return carry

    lax.fori_loop(1, NB // 2, a_step, 0)
    got_w(3, NB // 2 - 1)
    wait([c_mem, c_x(1, 0)])

    cols = (cols0, cols1)

    def tokens(s):
        return [bx[_ds(s, SEG), k * 128:(k + 1) * 128].astype(F32) for k in range(LT)]

    def qkv_group(odd, g, product, nm):
        pa, pb = (g.ws, g.us) if odd else (g.us, g.ws)
        h0 = 2 * odd

        half, same, cross = slice(8 * h0, 8 * h0 + HALF), {}, {}

        def prod(lhs, *name):
            return product.now(lhs, g.tile(wq, name))

        def direct(c):
            for _, k in [x for x in g.direct if x[0] == c]:
                r = prod(lambda: f_one[odd, k, 0:SEG + nm], "cell", c, k)
                same[c] = list(map(_add, same[c], r))

        def other(a):
            return cols1.at[a, M:L] if odd else part.at[a // 10, a % 10]

        def mixed(a, b, r):
            cross[a] = list(map(_add, cross.get(a) or _vregs(other(a)[half]), r))
            for x, h in zip(r, [h0, h0 + 1] + list(range(4, len(same[b])))):
                same[b][h] = same[b][h] + x

        def save_cross(a):
            other(a)[half] = _cat(cross.pop(a))

        def save(c, more=None):
            if nm:
                cols[odd][c, 0:nm] = _cat(same[c][4:])
            cols[1 - odd][c, M:L] = _add(more, _cat(same[c][:4]))
        parts = [pb[n:n + 3] for n in range(0, len(pb), 3)]
        for some in parts:
            for b, j in some:
                same[b] = list(prod(lambda: _cat([f_dif[odd, j]] + [f_one[odd, j, SEG:L]] * (nm > 0)), "+", b))
                direct(b)
            for a, i in pa:
                if some is parts[0]:
                    same[a] = prod(lambda: f_one[odd, i, 0:SEG + nm], "-", a)
                    x = _add(other(a)[...] if odd else None, _cat(same[a][:4]))
                    other(a)[HALF - 8 * h0:SEG - 8 * h0] = x[HALF - 8 * h0:SEG - 8 * h0]
                    cross[a] = _vregs(x[half])
                    direct(a)
                else:
                    same[a] = _vregs(cols[1 - odd][a, M:L]) + ([cols[odd][a, 0:nm]] if nm else [])
                for b, j in some:
                    if i != j:
                        product.tick()
                        product.soon(_cat([f_mix[odd, MIXES.index((i, j))]] + [f_one[odd, i, SEG:L]] * (nm > 0)),
                                     g.tile(wq, ("both", b, a) if odd else ("both", a, b)),
                                     functools.partial(mixed, a, b))
                for b, j in some:
                    if i != j:
                        r = prod(lambda: f_sum[odd, SUMS.index((min(i, j), max(i, j))), 0:SEG + nm], "cell", a, j)
                        same[a] = list(map(_add, same[a], r))
                        same[b] = list(map(_sub, same[b], r))
                save(a)
                product.after(HALF + nm, functools.partial(save_cross, a))
            for b, _ in some:
                product.after(HALF + nm, functools.partial(save, b, part[b // 10, b % 10] if odd else None))

    def out_groups(odd, gs, same, cross, product, last=False):
        h0, nh = (0, SEG * odd) if last else (2 - 2 * odd, HALF)

        def xa(c, r0=0, n=SEG):
            return att[c, M + SEG * (1 - odd) + r0:M + SEG * (1 - odd) + r0 + n]

        def xb(c, r0=0, n=SEG):
            return att[c, L + r0:L + r0 + n] if odd else keep[c, r0:r0 + n]

        def xm(c):
            return att[c, 0:M]

        def prod(g, m, x, *name):
            r = product.now(lambda: x() if last else _cat([m(), x()]), g.tile(wo, name))
            return r if last else r[1:] + r[:1]
        mix = {}

        def mixed(s, t, r):
            mix[s, t] = list(map(_add, mix.get((s, t), [None] * 4), r))

        def spend(s, t):
            for x, h in zip(mix.pop((s, t), []), list(range(h0, h0 + nh // 8)) + [4]):
                same[t][h] = _add(same[t][h], x)
                if h < 4:
                    cross[s][h] = _add(cross[s][h], x)
        sides = [(g, {d: c for c, d in (g.us if odd else g.ws)}, {d: c for c, d in (g.ws if odd else g.us)})
                 for g in gs]
        for i in range(LT):
            shared = None
            for g, pa, pb in sides:
                rs = [prod(g, lambda: xm(pb[i]), lambda: xa(pb[i]) - xb(pb[i]), "+", pb[i])] if i in pb else []
                rs += [prod(g, lambda: xm(c), lambda: xa(c), "cell", c, k) for c, k in g.direct if k == i]
                for r in rs:
                    same[i] = list(map(_add, same[i], r))
                if i in pa:
                    r = prod(g, lambda: xm(pa[i]), lambda: xa(pa[i]), "-", pa[i])
                    shared = list(map(_add, shared or [None] * 5, r))
                    if odd:
                        keep[pa[i]] = xa(pa[i])
            same[i] = list(map(_add, same[i], shared))
            cross[i] = list(map(_add, cross[i], shared))
            for j in range(i + 1, LT):
                diff = None
                for s, t in ((i, j), (j, i)):
                    for g, pa, pb in sides:
                        if s in pa and t in pb:
                            a, b = pa[s], pb[t]
                            if nh:
                                product.tick()
                                x = xa(a, 8 * h0, nh) + xb(b, 8 * h0, nh)
                                product.soon(x if last else _cat([x, xm(a)]),
                                             g.tile(wo, ("both", a, b) if odd else ("both", b, a)),
                                             functools.partial(mixed, s, t))
                            r = prod(g, lambda: xm(a) + xm(b), lambda: xa(a) + xa(b), "cell", b, s)
                            diff = list(map(_add if s == i else _sub, diff or [None] * 5, r))
                    product.after(nh if last else nh + M, functools.partial(spend, s, t))
                same[i] = list(map(_add, same[i], diff))
                same[j] = list(map(_sub, same[j], diff))

    def project_out(odd, s, product, last=False):
        same, cross = [[None] * 5 for _ in range(LT)], [[None] * 4 for _ in range(LT)]
        for gs in (GO[:3], GO[3:]):
            out_groups(odd, gs, same, cross, product, last)
        product.passed(0, True)
        for k in range(LT):
            lanes = slice(k * 128, (k + 1) * 128)
            if odd:
                out_a[k], out_b[k] = _cat(same[k][:4]), _cat(cross[k])
            else:
                outb[_ds(s - 2, SEG), lanes] = (out_a[k] + _cat(cross[k])).astype(BF16)
                outb[_ds(s - 1, SEG), lanes] = (out_b[k] + _cat(same[k][:4])).astype(BF16)
        return [x[-1] for x in same]

    def attend(odd, s, m, events):
        xa, xb = tokens(jnp.minimum(s + 1, NSEG - 1)), tokens(s if odd else jnp.minimum(s + 2, NSEG - 1))
        nm = m[0].shape[0]
        rows = slice(HALF * odd, HALF * odd + HALF)
        for k in range(LT):
            f_one[odd, k, 0:SEG + nm] = _cat([xa[k], m[k]])
            f_dif[odd, k] = xa[k] - xb[k]
        for n, (i, j) in enumerate(SUMS):
            f_sum[odd, n, 0:SEG + nm] = _cat([xa[i] + xa[j], m[i] + m[j]])
        for n, (i, j) in enumerate(MIXES):
            f_mix[odd, n] = xa[i][rows] + xb[j][rows]

        row = lax.broadcasted_iota(jnp.int32, (L, 2 * L), 0)
        col = lax.broadcasted_iota(jnp.int32, (L, 2 * L), 1)
        head0 = col < L
        visible = (row < M) | (row >= jnp.where(head0, col, col - L))
        st = {}

        def operand(j, p):
            return [cols[odd][c] for c in range(9 * p + j, 9 * p + 9, 3)]

        def whole(c, k):
            def use(r):
                st["w"] = list(map(_add, r, st["w"])) if k else r
                if k == LT - 1:
                    cols[odd][c] = _cat(st["w"])
            product.soon(f_one[odd, k, SEG:], GQ[c // 10].tile(wq, ("cell", c, k)), use)
        for n in range(LT * NC if nm > M else 0):
            events.setdefault(max(n - 2, 0), []).append(functools.partial(whole, n // LT, n % LT))

        def score(p):
            sc = []
            for q, k in zip(operand(1, p), _block_diag(*operand(0, p))):
                sc.append(_vregs(lax.dot_general(q, k, NT, preferred_element_type=F32)))
                product.passed(1)
            sc = _cat([x + y + z for x, y, z in zip(*sc)])
            st[p] = jnp.where(visible, sc, MASKED * DH ** 0.5)

        def shift(p):
            m0 = jnp.max(jnp.where(head0, st[p], -jnp.inf), axis=1, keepdims=True)
            m1 = jnp.max(jnp.where(head0, -jnp.inf, st[p]), axis=1, keepdims=True)
            st[p] = st[p] - jnp.where(head0, m0, m1)

        def normalize(p):
            e = jnp.exp2(st[p] * (DH ** -0.5 * LOG2E))
            l0 = jnp.sum(jnp.where(head0, e, 0.0), axis=1, keepdims=True)
            l1 = jnp.sum(jnp.where(head0, 0.0, e), axis=1, keepdims=True)
            st[p] = e * _recip(jnp.where(head0, l0, l1))

        def pv(p):
            for t, v in enumerate(_block_diag(*operand(2, p))):
                r = _dot(st[p], v)
                product.passed(1)
                att[3 * p + t, 0:M] = r[0:M]
                att[3 * p + t, M + SEG * odd:L + SEG * odd] = r[M:L]

        for p in range(NP):
            ready = min((9 * p + 17) // 10 * 50, LT * NC)
            for f, lag in ((score, 20), (shift, 38), (normalize, 55), (pv, 75)):
                events.setdefault(ready + lag, []).append(functools.partial(f, p))
        product = step[0] = _Products(events, tied)
        for g in GQ:
            qkv_group(odd, g, product, M if nm == M else 0)
        return product

    def spread(events, tasks, t0, t1, src=None, dst=None):
        def run(some):
            if src is None or len(step[0].results) < 25:
                _run(some)
            else:
                paced(some, src, step[0].results[-25])
            if dst is not None:
                tie(dst)
        for t in range(t0, t1):
            if _share(tasks, t - t0, t1 - t0):
                events.setdefault(t, []).append(functools.partial(run, _share(tasks, t - t0, t1 - t0)))

    events, end, W = {}, LT * NC, 330
    turn = w_turn(GQ[13], wq) + w_turn(GQ[14], wq)
    spread(events, a_attention(1), 12, W // 3, qkv1, oa1)
    spread(events, [functools.partial(_run, turn[n:n + 2]) for n in range(0, 70, 2)], W // 3, W - 40, raw)
    spread(events, w_combine(GQ[12], wq), W // 3, 2 * W // 3, wq_c0, wl_s)
    spread(events, [lambda: tie(wl_c1)] * 8, W // 3 + 20, 2 * W // 3 + 40)
    spread(events, w_combine(GQ[13], wq), 2 * W // 3 + 25, W, wl_c1, wl_s)
    spread(events, w_combine(GQ[14], wq), W + 1, W + 30, wl_c0, wl_s)

    def wo_wait():
        wait([cp(wo_c.at[:, 0:NF * 64], wo_c.at[:, 0:NF * 64], sem_wo)])
        c_bx.start()
    spread(events, [wo_wait], W, W + 1)
    spread(events, sum([w_combine(g, wo) for g in GO], []), W + 30, end + 150, wo_c, wo_s)
    spread(events, [functools.partial(a_out, NB - 1, 1, c) for c in range(LT)], end, end + LT * NF)
    product = attend(0, 0, [_cat([mem[:, k * 128:(k + 1) * 128].astype(F32), x]) for k, x in enumerate(tokens(0))],
                     events)
    product.passed(0, True)
    m = [None] * LT
    for c in range(NF):
        for k in range(LT):
            g = GO[c // 10]
            w = g.tile(wo, ("cell", c, k))
            m[k] = _add(m[k], product.now(lambda: att[c, 0:M], w)[0])
    for k in range(LT):
        mem_s[k] = m[k]

    def b_step(n, carry):
        m = project_out(1, 2 * n + 1, attend(1, 2 * n + 1, [mem_s[k] for k in range(LT)], {}))
        m = project_out(0, 2 * n + 2, attend(0, 2 * n + 2, m, {}))
        for k in range(LT):
            mem_s[k] = m[k]
        c_out(1, _ds(n, 2 * SEG)).start()
        return carry

    c_out(0, pl.ds(0, S)).start()
    c_bx.wait()
    lax.fori_loop(0, NSEG // 2 - 1, b_step, 0)
    product = attend(1, NSEG - 1, [mem_s[k] for k in range(LT)], {})
    project_out(1, NSEG - 1, product, last=True)
    project_out(0, NSEG, product, last=True)
    c_out(1, _ds(NSEG // 2 - 1, 2 * SEG)).start()
    wait([c_out(j, pl.ds(0, S)) for j in range(2)])


def pallas_concat_heads__sliding_local_dilated__memory_aug_recurrent_mem_tr__prompt_kernel(
    A_x, A_wqkv, A_wo, B_x, B_mem0, B_Wq, B_Wk, B_Wv, B_Wo, B_seg_len,
):
    assert B_seg_len == SEG
    assert A_x.shape == B_x.shape == (1, S, D) and B_mem0.shape == (1, M, D)
    assert B_Wq.shape == B_Wk.shape == B_Wv.shape == (D, H, DH) and B_Wo.shape == (H, DH, D)
    vmem, dma = pltpu.VMEM, pltpu.SemaphoreType.DMA
    call = pl.pallas_call(
        _kernel,
        out_shape=jax.ShapeDtypeStruct((S, 2 * D), BF16),
        in_specs=[pl.BlockSpec(memory_space=pl.ANY)] * 9,
        out_specs=pl.BlockSpec(memory_space=pl.ANY),
        scratch_shapes=[
            vmem((S, D), BF16),
            vmem((3, D, D), BF16),
            vmem((D, D), BF16),
            vmem((LT, D, 128), F32),
            vmem((3 * D // 2, D), U32),
            vmem((D // 2, D), U32),
            vmem((2, TB, D), F32),
            vmem((3 * LT + 1, HALO + TB, 128), F32), vmem((3 * LT + 1, HALO + TB, 128), F32),
            vmem((LT + 1, TB, 128), F32), vmem((LT + 1, TB, 128), F32),
            vmem((S, D), BF16),
            vmem((S, D), BF16),
            vmem((M, D), BF16),
            vmem((LT, NC * 64 + 8, 128), U32),
            vmem((351, 64, 128), U32), vmem((301, 64, 128), U32), vmem((481, 64, 128), U32),
            vmem((LT, NF * 64 + 8, 128), U32), vmem((4 * NF, 64, 128), U32),
            vmem((21, 64, 128), U32), vmem((51, 64, 128), U32), vmem((93, 64, 128), U32),
            vmem((LT, M, 128), F32),
            vmem((2, LT, L + SEG, 128), F32),
            vmem((2, len(SUMS), L + SEG, 128), F32),
            vmem((2, LT, SEG, 128), F32),
            vmem((2, len(MIXES), HALF, 128), F32),
            vmem((NC, L, 128), F32), vmem((NC, L, 128), F32),
            vmem((len(GQ), LT, SEG, 128), F32),
            vmem((NF, L + SEG, 128), F32),
            vmem((NF, SEG, 128), F32),
            vmem((LT, SEG, 128), F32), vmem((LT, SEG, 128), F32),
            dma((5,)), dma((NB // 2, 2)), dma((NB // 2 + 1,)), dma(()), dma((2,)),
        ],
        compiler_params=pltpu.CompilerParams(vmem_limit_bytes=127 * 1024 * 1024, disable_bounds_checks=True, disable_semaphore_checks=True),
        name="sliding_and_memory_attention",
    )

    def by_feature(w):
        return w.transpose(1, 2, 0).reshape(H * DH, D)

    out = call(A_x.reshape(S, D), A_wqkv, A_wo, B_x.reshape(S, D), B_mem0.reshape(M, D),
               by_feature(B_Wq), by_feature(B_Wk), by_feature(B_Wv), B_Wo.reshape(H * DH, D))
    return out.reshape(1, S, 2 * D)
```

```python
import functools

import jax
import jax.numpy as jnp
from jax import lax
from jax.experimental import pallas as pl
from jax.experimental.pallas import tpu as pltpu

F32, BF16, U32 = jnp.float32, jnp.bfloat16, jnp.uint32
NT = (((1,), (1,)), ((), ()))
MASKED = -1000000000.0
LOG2E = 1.4426950408889634

S, D = 2048, 640
LT = D // 128

AH, AD, AW, ADIL = 32, 20, 8, 2
HALO = 16
TB = 128
NB = S // TB
RC = 8

H, DH, M, SEG = 32, 192, 8, 32
L = M + SEG
HALF = SEG // 2
NP = H // 2
NSEG = S // SEG
NF = H * DH // 128
NC = 3 * NF
SUMS = [(i, j) for i in range(LT) for j in range(i + 1, LT)]
MIXES = [(i, j) for i in range(LT) for j in range(LT) if i != j]


class _Group:
    def __init__(self, first, u_diag, w_diag):
        self.us = [(first + n, i) for n, i in enumerate(u_diag)]
        self.ws = [(first + len(u_diag) + n, j) for n, j in enumerate(w_diag)]
        self.pairs = [(u, i, w, j) for u, i in self.us for w, j in self.ws if i != j]
        paired = [(u, j) for u, i, w, j in self.pairs] + [(w, i) for u, i, w, j in self.pairs]
        self.direct = [(c, k) for c, d in self.us + self.ws for k in range(LT)
                       if k != d and (c, k) not in paired]
        sums = [(sign, c) for sign in "-+" for c, _ in self.us + self.ws]
        self.sums = sums + [("both", u, w) for u, i, w, j in self.pairs]
        self.first = first

    def tile(self, refs, name, shift=0):
        g = self.first // 10
        if name[0] != "cell" and g > 12:
            return refs[-2].at[40 * (g - 13) + self.sums.index(name)]
        if g > 13:
            return refs[2].at[LT * (name[1] - self.first) + name[2]]
        if name[0] != "cell":
            return refs[-1].at[40 * (g + shift) + self.sums.index(name)]
        if refs[0].shape[0] == LT:
            return refs[0].at[name[2], 64 * name[1]:64 * name[1] + 64]
        n = min(len(refs) - 1, 2)
        return refs[g % n].at[50 * (g // n + shift // n) + LT * (name[1] - self.first) + name[2]]


def _groups(n, u_last, w_last):
    groups = [_Group(10 * g, range(LT), range(LT)) for g in range(n // 10)]
    return groups + [_Group(n // 10 * 10, u_last, w_last)]


GQ = _groups(NC, (0, 1), (2, 3))
GO = _groups(NF, (0, 1, 2, 3), (1, 2, 3, 4))


def _ds(i, n):
    return pl.ds(i * n if isinstance(i, int) else pl.multiple_of(i * n, n), n)


def _dot(a, b):
    return jnp.dot(a, b, preferred_element_type=F32)


def _recip(x):
    r = pl.reciprocal(x, approx=True)
    return r * (2.0 - x * r)


def _add(a, b):
    return b if a is None else a + b


def _sub(a, b):
    return -b if a is None else a - b


def _vregs(x):
    return [x[r:r + 8] for r in range(0, x.shape[0], 8)]


def _cat(vs):
    return jnp.concatenate(vs, axis=0)


def _share(tasks, k, n):
    return tasks[k * len(tasks) // n:(k + 1) * len(tasks) // n]


def _run(tasks):
    for task in tasks:
        task()


class _Products:
    def __init__(self, events, tied):
        self.events, self.tied, self.results = events, tied, []
        self.count, self.usual, self.flushed, self.waiting = 0, 0, -1, {}

    def dot(self, x, w):
        self.results.append(_vregs(pltpu.bitcast(_dot(self.tied(x), pltpu.bitcast(w, BF16)), F32)))
        return self.results[-1]

    def tick(self):
        self.count += 1
        _run(self.events.pop(self.count - 1, []))

    def now(self, x, w):
        self.tick()
        r = self.dot(x(), w[...])
        self.passed(1)
        return r

    def soon(self, x, w, use):
        self.waiting.setdefault(x.shape[0], []).append([x, w[...], [use]])

    def after(self, rows, task):
        if self.waiting.get(rows):
            self.waiting[rows][-1][2].append(lambda r: task())
        else:
            task()

    def passed(self, n, last=False):
        self.usual += n
        for rows in sorted(self.waiting, reverse=True):
            queue = self.waiting[rows]
            while queue and (last or (len(queue) >= 4 and self.usual % 4 == 0
                                      and (self.flushed < self.usual or len(queue) >= 8 or rows >= L))):
                for x, w, uses in queue[:4]:
                    r = self.dot(x, w)
                    for use in uses:
                        use(r)
                del queue[:4]
                if rows < L:
                    self.flushed = self.usual


def _block_diag(t0, t1, t2):
    lane = lax.broadcasted_iota(jnp.int32, (L, 128), 1)
    zero = jnp.zeros((L, 128), F32)
    halves = [jnp.where(lane < 64, t1, 0.0), jnp.where(lane >= 64, t1, 0.0)]
    return [_cat(x).astype(BF16) for x in ([t0, zero], halves, [zero, t2])]


def _kernel(ax_hbm, awqkv_hbm, awo_hbm, bx_hbm, mem_hbm, wq_hbm, wk_hbm, wv_hbm, wo_hbm,
            out_hbm,
            ax, awqkv, awo, tmp, wqkv_p, wo_p, x_s, qkv0, qkv1, oa0, oa1, outa,
            bx, mem, raw, wq_c0, wq_c1, wq_s, wo_c, wo_s, wl_c, wl_s, mem_s, f_one, f_sum, f_dif, f_mix, cols0, cols1, part, att, keep, out_a, out_b,
            sem_a, sem_x, sem_w, sem_wo, sem_o):
    cp = pltpu.make_async_copy
    outb = ax

    def rows_copy(src, dst, r0, r1, sem):
        return cp(src.at[pl.ds(r0, r1 - r0), :], dst.at[pl.ds(r0, r1 - r0), :], sem)

    c_wqkv = [cp(awqkv_hbm.at[:, pl.ds(j * D, D)], awqkv.at[j], sem_a.at[j]) for j in range(3)]
    c_awo = cp(awo_hbm, awo, sem_a.at[3])
    c_mem = cp(mem_hbm, mem, sem_a.at[4])

    c_bx = [rows_copy(bx_hbm, bx, r0, r1, sem_a.at[5 + n]) for n, (r0, r1) in enumerate(((0, 3 * SEG), (3 * SEG, S)))]

    def c_ax(i):
        return cp(ax_hbm.at[_ds(i, TB)], ax.at[_ds(i, TB)], sem_x.at[i])

    def by_tile(src, dst, rows, sem):
        return [cp(src.at[:, pl.ds(k * 128, 128)], dst.bitcast(BF16).at[k, rows], sem) for k in range(LT)]

    def tiles(t, n):
        return pl.ds(t * 128 if isinstance(t, int) else pl.multiple_of(t * 128, 128), n * 128)

    def get_wo(t, n, batch):
        start(by_tile(wo_hbm.at[tiles(t, n)], wo_c, tiles(t, n), sem_wo.at[batch]))

    def get_w(t, n, batch):
        for j, w in enumerate((wk_hbm, wq_hbm, wv_hbm)):
            start(by_tile(w.at[tiles(t, n)], raw, tiles(j * NF + t, n), sem_w.at[batch]))

    def got_w(n, batch):
        cp(raw.at[:, 0:n * 192], raw.at[:, 0:n * 192], sem_w.at[batch]).wait()

    def c_out(j, rows):
        return cp((outa, outb)[j].at[rows, :], out_hbm.at[rows, pl.ds(j * D, D)], sem_o.at[j])

    def start(copies):
        for c in copies:
            c.start()

    def wait(copies):
        for c in copies:
            c.wait()

    def permute_rows(dst, base):
        for d in range(AD):
            for t in range(LT):
                dst[pl.ds((base + d * AH) // 2, AH // 2), t * 128:(t + 1) * 128] = pltpu.bitcast(
                    tmp[t, pl.ds(d, AH, stride=AD), :].astype(BF16), U32)

    def prep_wqkv(j):
        for t in range(LT):
            tmp[t] = awqkv[j, t * 128:(t + 1) * 128, :].astype(F32).T
        permute_rows(wqkv_p, j * D)

    def prep_wo():
        for t in range(LT):
            tmp[t] = awo[:, t * 128:(t + 1) * 128].astype(F32)
        permute_rows(wo_p, 0)

    qkv, oa = (qkv0, qkv1), (oa0, oa1)
    sums = {id(wq_c0): (wl_s, wq_s), id(wo_c): (wo_s,)}
    wl_s, wq_s, wo_s = [r.bitcast(U32) for r in (wl_s, wq_s, wo_s)]
    wq, wo = (wq_c0, wq_c1, wl_c, wl_s, wq_s), (wo_c, wo_s)

    ties, step = [], [None]

    def tied(x):
        head = x[0:8, 0:128]
        while ties:
            ref = ties.pop()
            ref[...] = pltpu.bitcast(head, ref.dtype)
            head = pltpu.bitcast(ref[...], x.dtype)
        if x.shape[1] > 128:
            head = jnp.concatenate([head, x[0:8, 128:]], axis=1)
        return _cat([head, x[8:]]) if x.shape[0] > 8 else head

    def a_proj(i, b, c):
        if c == 0:
            x_s[b] = ax[_ds(i, TB), :].astype(F32)
        w = pltpu.bitcast(wqkv_p[c * 64:(c + 1) * 64, :], BF16)
        r = lax.dot_general(tied(x_s[b]), w, NT, preferred_element_type=F32)
        qkv[b][c, HALO:] = r
        if c >= LT and isinstance(i, int) and i == 0:
            qkv[b][c, 0:HALO] = jnp.broadcast_to(r[0:1, :], (HALO, 128))
        elif c >= LT:
            qkv[b][c, 0:HALO] = qkv[1 - b][c, TB:]
        return r

    def a_attention(b, first_block=False):
        state = {}

        def window(c, r0, w):
            lo = HALO + r0 - ADIL * w
            return qkv[b][LT + c, lo:lo + RC]

        def logits(r0, ws):
            q = [qkv[b][t, HALO + r0:HALO + r0 + RC] for t in range(LT)]
            for w in ws:
                a = functools.reduce(jnp.add, [q[t] * window(t, r0, w) for t in range(LT)])
                a = functools.reduce(jnp.add, [a] + [pltpu.roll(a, d, 1) for d in range(AH, 128, AH)])
                if first_block and r0 < ADIL * w:
                    pos = lax.broadcasted_iota(jnp.int32, (RC, 128), 0) + r0
                    a = jnp.where(pos >= ADIL * w, a, MASKED * AD ** 0.5)
                state[r0, w] = a

        def mix(r0, ts):
            if ts[0] == 0:
                lg = [state.pop((r0, w)) for w in range(AW)]
                m = functools.reduce(jnp.maximum, lg)
                state[r0] = [jnp.exp2((a - m) * (AD ** -0.5 * LOG2E)) for a in lg]
                state[r0].append(_recip(functools.reduce(jnp.add, state[r0])))
            e = state[r0]
            for t in ts:
                o = functools.reduce(jnp.add, [e[w] * window(LT + t, r0, w) for w in range(AW)])
                oa[b][t, r0:r0 + RC] = o * e[AW]

        steps = ([(0, logits, range(AW)), (1, mix, range(LT))],
                 [(0, logits, range(4)), (0, logits, range(4, 8)), (1, mix, range(1)), (1, mix, range(1, LT))],
                 [(0, logits, range(w, w + 2)) for w in range(0, 8, 2)] + [(1, mix, [t]) for t in range(LT)])[1]
        n = TB // RC
        return [functools.partial(f, (k - lag) * RC, part) for k in range(n + 1)
                for lag, f, part in steps if 0 <= k - lag < n]

    def a_out(i, b, c):
        lanes = slice(c * 128, (c + 1) * 128)
        x = jnp.concatenate([oa[b][k] for k in range(LT)], axis=1)
        r = _dot(tied(x), pltpu.bitcast(wo_p[:, lanes], BF16))
        outa[_ds(i, TB), lanes] = r.astype(BF16)
        return r

    def a_last(c, k):
        def use(r):
            x = _cat(list(map(_add, _vregs(tmp[c, 0:TB // 2 * 2]), r)) if k else r)
            if k < LT - 1:
                tmp[c, 0:TB] = x
            else:
                outa[S - TB:S, c * 128:(c + 1) * 128] = x.astype(BF16)
        step[0].soon(oa1[k], wo_p.at[k * 64:(k + 1) * 64, c * 128:(c + 1) * 128], use)

    def paced(tasks, ref, results):
        for n, task in enumerate(tasks):
            x = pltpu.bitcast(results[n * len(results) // len(tasks)], ref.dtype)
            if ref.shape[0] == LT:
                ref[zero, ref.shape[1] - 8:] = x
            else:
                ref[ref.shape[0] - 1 + zero, 0:8] = x
            task()

    def tie(ref):
        ties.append(ref.at[ref.shape[0] - 1 + zero, 8:16])

    def a_pass(i, b, c, k0, k1):
        lanes = slice(c % LT * 128, c % LT * 128 + 128)
        if c < 3 * LT:
            if c == k0 == 0:
                x_s[b] = ax[_ds(i, TB), :].astype(F32)
            w = pltpu.bitcast(wqkv_p[c * 64:(c + 1) * 64, k0 * 128:k1 * 128], BF16)
            r = lax.dot_general(tied(x_s[b, :, k0 * 128:k1 * 128]), w, NT, preferred_element_type=F32)
        else:
            x = jnp.concatenate([oa[1 - b][k] for k in range(k0, k1)], axis=1)
            r = _dot(tied(x), pltpu.bitcast(wo_p[k0 * 64:k1 * 64, lanes], BF16))
        if k1 < LT:
            tmp[c % 4, 0:TB] = r
            return _vregs(r)
        r = _cat(list(map(_add, _vregs(tmp[c % 4, 0:TB]), _vregs(r))))
        if c >= 3 * LT:
            outa[_ds(i - 1, TB), lanes] = r.astype(BF16)
        else:
            qkv[b][c, HALO:] = r
            if c >= LT:
                qkv[b][c, 0:HALO] = qkv[1 - b][c, TB:]
        return _vregs(r)

    def a_stage(i, b, turn, combine):
        turn = [functools.partial(_run, turn[n:n + 2]) for n in range(0, len(turn), 2)]
        side = [(a_attention(1 - b), 0, 17, 2 + 1, qkv[1 - b], oa[1 - b]),
                (turn, 20, 25, 99, raw, wq[b]),
                (combine[:90], 0, 17, 2, wq[1 - b], wq_s),
                (combine[90:], 17, 24, 2, wq[1 - b], wq_s)]
        rs = []
        for c in range(5 * LT):
            if c % 5 < 4:
                rs.append(a_pass(i, b, c - c // 5, 0, 4))
            else:
                rs.append([a_pass(i, b, c // 5 * 4 + n, 4, LT) for n in range(4)][0])
            for tasks, c0, c1, lag, src, dst in side:
                if c0 <= c < c1:
                    if len(rs) < lag:
                        _run(_share(tasks, c - c0, c1 - c0))
                    else:
                        paced(_share(tasks, c - c0, c1 - c0), src, rs[-lag])
                    if (tasks is not turn or 1) and (dst is not wq_s or c % 1 == 0):
                        tie(dst)

    def w_turn(g, dst, shift=0):
        def turn(c, k):
            col = c + 10 * shift
            t = (col * 171) >> 9
            x = pltpu.bitcast(raw[k, _ds((col - 3 * t) * NF + t, 64)], BF16)
            g.tile(dst, ("cell", c, k), shift)[...] = pltpu.bitcast(x.T, U32)
        return [functools.partial(turn, c, k) for c, _ in g.us + g.ws for k in range(LT)]

    def w_combine(g, dst, shift=0):
        minus, plus = {}, {}

        def get(r, c, k):
            cell = g.tile(dst, ("cell", c, k), shift).at[r // 2:r // 2 + 8]
            return pltpu.bitcast(cell[...], BF16).astype(F32)

        def put(r, x, *name):
            g.tile(sums[id(dst[0])], name, shift)[r:r + 16] = x.astype(BF16)

        def combine(r, pairs):
            for pair in pairs:
                u, i, w, j = pair
                x, y = get(r, u, j), get(r, w, i)
                put(r, x + y, "both", u, w)
                if dst is wo:
                    x, y = y, x
                for c, d, own, other in ((u, i, x, y), (w, j, y, x)):
                    mine = [p for p in g.pairs if c in (p[0], p[2])]
                    if pair == mine[0]:
                        minus[c] = plus[c] = get(r, c, d)
                    minus[c], plus[c] = minus[c] - own, plus[c] + other
                    if pair == mine[-1]:
                        put(r, minus[c], "-", c)
                        put(r, plus[c], "+", c)
        return [functools.partial(combine, r, g.pairs[n:n + 1]) for r in range(0, 128, 16)
                for n in range(0, len(g.pairs), 1)]

    start([c_wqkv[0], c_ax(0), c_ax(1), c_wqkv[1], c_wqkv[2]])

    def touch(i, carry):
        tmp[i, 0:8] = jnp.zeros((8, 128), F32)
        for ref in (x_s, f_one, f_sum, f_dif, f_mix, cols0, cols1, part, att, keep, out_a, out_b):
            ref[i] = jnp.zeros(ref.shape[1:], F32)
        for ref in wo[1:] + wq:
            ref[i] = jnp.zeros((64, 128), U32)
        for ref in (wqkv_p, wo_p):
            ref[_ds(i, 8)] = jnp.zeros((8, D), U32)
        return i
    zero = lax.shift_right_logical(lax.fori_loop(0, 2, touch, 0), 16)
    c_wqkv[0].wait()
    prep_wqkv(0)
    for j in range(2):
      c_wqkv[j + 1].wait()
      if j == 0:
          wait([c_ax(0), c_ax(1)])
      if j == 0:
          start([c_awo, c_ax(2)])
      else:
          get_w(0, 4, 2)
      prep_wqkv(j + 1)
      for n in range(2 * LT):
          a_proj(n // LT, n // LT, j * LT + n % LT)
    c_awo.wait()
    get_w(4, 3, 3)
    start([c_ax(3), c_mem, c_bx[0]])
    prep_wo()
    for n in range(2 * LT):
      a_proj(n // LT, n // LT, 2 * LT + n % LT)
    _run(a_attention(0, True))
    for c in range(LT):
      a_out(0, 0, c)

    def a_step(it, carry):
        for b in range(2):
            i = 2 * it + b
            got_w(4 - 2 * b, i)
            if b:
                @pl.when(it < 7)
                def _():
                    got_w(1, i)
            c_ax(i).wait()

            @pl.when(it < 7)
            def _():
                get_w(7 * it + 4 * b, 4 - 2 * b, i + 2)
                c_ax(i + 2).start()
            if b:
                @pl.when(it < 6)
                def _():
                    get_w(7 * it + 6, 1, i + 2)

            @pl.when(it == 7)
            def _():
                for n in range(3):
                    get_wo(15 * b + 5 * n, 5, 0)
            a_stage(i, b, w_turn(GQ[b], wq, 2 * it - 2),
                    w_combine(GQ[1 - b], wq, jnp.where(i < 3, 10, 2 * it - 4 + 2 * b)))
            ties.clear()
        return carry

    lax.fori_loop(1, NB // 2, a_step, 0)
    wait([c_mem, c_bx[0]])

    cols = (cols0, cols1)

    def tokens(s):
        return [bx[_ds(s, SEG), k * 128:(k + 1) * 128].astype(F32) for k in range(LT)]

    def qkv_group(odd, g, product, nm):
        pa, pb = (g.ws, g.us) if odd else (g.us, g.ws)
        h0 = 2 * odd

        half, same, cross = slice(8 * h0, 8 * h0 + HALF), {}, {}

        def prod(lhs, *name):
            return product.now(lhs, g.tile(wq, name))

        def direct(c):
            for _, k in [x for x in g.direct if x[0] == c]:
                r = prod(lambda: f_one[odd, k, 0:SEG + nm], "cell", c, k)
                same[c] = list(map(_add, same[c], r))

        def other(a):
            return cols1.at[a, M:L] if odd else part.at[a // 10, a % 10]

        def mixed(a, b, r):
            cross[a] = list(map(_add, cross.get(a) or _vregs(other(a)[half]), r))
            for x, h in zip(r, [h0, h0 + 1] + list(range(4, len(same[b])))):
                same[b][h] = same[b][h] + x

        def save_cross(a):
            other(a)[half] = _cat(cross.pop(a))

        def save(c, more=None):
            if nm:
                cols[odd][c, 0:nm] = _cat(same[c][4:])
            cols[1 - odd][c, M:L] = _add(more, _cat(same[c][:4]))
        parts = [pb[n:n + 3] for n in range(0, len(pb), 3)]
        for some in parts:
            for b, j in some:
                same[b] = list(prod(lambda: _cat([f_dif[odd, j]] + [f_one[odd, j, SEG:L]] * (nm > 0)), "+", b))
                direct(b)
            for a, i in pa:
                if some is parts[0]:
                    same[a] = prod(lambda: f_one[odd, i, 0:SEG + nm], "-", a)
                    x = _add(other(a)[...] if odd else None, _cat(same[a][:4]))
                    other(a)[HALF - 8 * h0:SEG - 8 * h0] = x[HALF - 8 * h0:SEG - 8 * h0]
                    cross[a] = _vregs(x[half])
                    direct(a)
                else:
                    same[a] = _vregs(cols[1 - odd][a, M:L]) + ([cols[odd][a, 0:nm]] if nm else [])
                for b, j in some:
                    if i != j:
                        product.tick()
                        product.soon(_cat([f_mix[odd, MIXES.index((i, j))]] + [f_one[odd, i, SEG:L]] * (nm > 0)),
                                     g.tile(wq, ("both", b, a) if odd else ("both", a, b)),
                                     functools.partial(mixed, a, b))
                for b, j in some:
                    if i != j:
                        r = prod(lambda: f_sum[odd, SUMS.index((min(i, j), max(i, j))), 0:SEG + nm], "cell", a, j)
                        same[a] = list(map(_add, same[a], r))
                        same[b] = list(map(_sub, same[b], r))
                save(a)
                product.after(HALF + nm, functools.partial(save_cross, a))
            for b, _ in some:
                product.after(HALF + nm, functools.partial(save, b, part[b // 10, b % 10] if odd else None))

    def out_groups(odd, gs, same, cross, product, last=False):
        h0, nh = (0, SEG * odd) if last else (2 - 2 * odd, HALF)

        def xa(c, r0=0, n=SEG):
            return att[c, M + SEG * (1 - odd) + r0:M + SEG * (1 - odd) + r0 + n]

        def xb(c, r0=0, n=SEG):
            return att[c, L + r0:L + r0 + n] if odd else keep[c, r0:r0 + n]

        def xm(c):
            return att[c, 0:M]

        def prod(g, m, x, *name):
            r = product.now(lambda: x() if last else _cat([m(), x()]), g.tile(wo, name))
            return r if last else r[1:] + r[:1]
        mix = {}

        def mixed(s, t, r):
            mix[s, t] = list(map(_add, mix.get((s, t), [None] * 4), r))

        def spend(s, t):
            for x, h in zip(mix.pop((s, t), []), list(range(h0, h0 + nh // 8)) + [4]):
                same[t][h] = _add(same[t][h], x)
                if h < 4:
                    cross[s][h] = _add(cross[s][h], x)
        sides = [(g, {d: c for c, d in (g.us if odd else g.ws)}, {d: c for c, d in (g.ws if odd else g.us)})
                 for g in gs]
        for i in range(LT):
            shared = None
            for g, pa, pb in sides:
                rs = [prod(g, lambda: xm(pb[i]), lambda: xa(pb[i]) - xb(pb[i]), "+", pb[i])] if i in pb else []
                rs += [prod(g, lambda: xm(c), lambda: xa(c), "cell", c, k) for c, k in g.direct if k == i]
                for r in rs:
                    same[i] = list(map(_add, same[i], r))
                if i in pa:
                    r = prod(g, lambda: xm(pa[i]), lambda: xa(pa[i]), "-", pa[i])
                    shared = list(map(_add, shared or [None] * 5, r))
                    if odd:
                        keep[pa[i]] = xa(pa[i])
            same[i] = list(map(_add, same[i], shared))
            cross[i] = list(map(_add, cross[i], shared))
            for j in range(i + 1, LT):
                diff = None
                for s, t in ((i, j), (j, i)):
                    for g, pa, pb in sides:
                        if s in pa and t in pb:
                            a, b = pa[s], pb[t]
                            if nh:
                                product.tick()
                                x = xa(a, 8 * h0, nh) + xb(b, 8 * h0, nh)
                                product.soon(x if last else _cat([x, xm(a)]),
                                             g.tile(wo, ("both", a, b) if odd else ("both", b, a)),
                                             functools.partial(mixed, s, t))
                            r = prod(g, lambda: xm(a) + xm(b), lambda: xa(a) + xa(b), "cell", b, s)
                            diff = list(map(_add if s == i else _sub, diff or [None] * 5, r))
                    product.after(nh if last else nh + M, functools.partial(spend, s, t))
                same[i] = list(map(_add, same[i], diff))
                same[j] = list(map(_sub, same[j], diff))

    def project_out(odd, s, product, last=False):
        same, cross = [[None] * 5 for _ in range(LT)], [[None] * 4 for _ in range(LT)]
        for gs in (GO[:3], GO[3:]):
            out_groups(odd, gs, same, cross, product, last)
        product.passed(0, True)
        for k in range(LT):
            lanes = slice(k * 128, (k + 1) * 128)
            if odd:
                out_a[k], out_b[k] = _cat(same[k][:4]), _cat(cross[k])
            else:
                outb[_ds(s - 2, SEG), lanes] = (out_a[k] + _cat(cross[k])).astype(BF16)
                outb[_ds(s - 1, SEG), lanes] = (out_b[k] + _cat(same[k][:4])).astype(BF16)
        return [x[-1] for x in same]

    def attend(odd, s, m, events, last=False):
        xa, xb = tokens(jnp.minimum(s + 1, NSEG - 1)), tokens(s if odd else jnp.minimum(s + 2, NSEG - 1))
        nm = m[0].shape[0]
        rows = slice(HALF * odd, HALF * odd + HALF)
        for k in range(LT):
            f_one[odd, k, 0:SEG + nm] = _cat([xa[k], m[k]])
            f_dif[odd, k] = xa[k] - xb[k]
        for n, (i, j) in enumerate(SUMS):
            f_sum[odd, n, 0:SEG + nm] = _cat([xa[i] + xa[j], m[i] + m[j]])
        for n, (i, j) in enumerate(MIXES):
            f_mix[odd, n] = xa[i][rows] + xb[j][rows]

        row = lax.broadcasted_iota(jnp.int32, (L, 2 * L), 0)
        col = lax.broadcasted_iota(jnp.int32, (L, 2 * L), 1)
        head0 = col < L
        visible = (row < M) | (row >= jnp.where(head0, col, col - L))
        st = {}

        def operand(j, p):
            return [cols[odd][c] for c in range(9 * p + j, 9 * p + 9, 3)]

        def whole(c, k):
            def use(r):
                st["w"] = list(map(_add, r, st["w"])) if k else r
                if k == LT - 1:
                    cols[odd][c] = _cat(st["w"])
            product.soon(f_one[odd, k, SEG:], GQ[c // 10].tile(wq, ("cell", c, k)), use)
        for n in range(LT * NC if nm > M else 0):
            events.setdefault(max(n - 2, 0), []).append(functools.partial(whole, n // LT, n % LT))

        def score(p):
            sc = []
            for q, k in zip(operand(1, p), _block_diag(*operand(0, p))):
                sc.append(_vregs(lax.dot_general(q, k, NT, preferred_element_type=F32)))
                product.passed(1)
            sc = _cat([x + y + z for x, y, z in zip(*sc)])
            st[p] = jnp.where(visible, sc, MASKED * DH ** 0.5)

        def shift(p):
            m0 = jnp.max(jnp.where(head0, st[p], -jnp.inf), axis=1, keepdims=True)
            m1 = jnp.max(jnp.where(head0, -jnp.inf, st[p]), axis=1, keepdims=True)
            st[p] = st[p] - jnp.where(head0, m0, m1)

        def normalize(p):
            e = jnp.exp2(st[p] * (DH ** -0.5 * LOG2E))
            l0 = jnp.sum(jnp.where(head0, e, 0.0), axis=1, keepdims=True)
            l1 = jnp.sum(jnp.where(head0, 0.0, e), axis=1, keepdims=True)
            st[p] = e * _recip(jnp.where(head0, l0, l1))

        def pv(p):
            for t, v in enumerate(_block_diag(*operand(2, p))):
                r = _dot(st[p], v)
                product.passed(1)
                att[3 * p + t, 0:M] = r[0:M]
                att[3 * p + t, M + SEG * odd:L + SEG * odd] = r[M:L]

        for p in range(NP):
            ready = min((9 * p + 17) // 10 * 50, LT * NC)
            for f, lag in ((score, 28), (shift, 50), (normalize, 60), (pv, 76)):
                events.setdefault(ready + lag, []).append(functools.partial(f, p))
        product = step[0] = _Products(events, tied)
        def finish(u, w):
            def use(k, r):
                st["u"] = r[0] + st["u"] if k else r[0]
                if k == LT - 1:
                    cols[odd][u, 0:M] = st["u"]
            r = [None] * 5
            for k in range(LT):
                product.tick()
                if u % 3 != 1:
                    product.soon(f_one[odd, k, SEG:L], GQ[u // 10].tile(wq, ("cell", u, k)), functools.partial(use, k))
                r = list(map(_add, r, product.now(lambda: f_one[odd, k, 0:L], GQ[w // 10].tile(wq, ("cell", w, k)))))
            cols[odd][w] = _cat(r[4:] + r[:4])
        for g in GQ:
            if last:
                for (u, _), (w, _) in zip(g.us, g.ws):
                    finish(u, w)
            else:
                qkv_group(odd, g, product, M if nm == M else 0)
        return product

    def spread(events, tasks, t0, t1, src=None, dst=None):
        def run(some):
            if src is None or len(step[0].results) < 32:
                _run(some)
            else:
                paced(some, src, step[0].results[-32])
            if dst is not None:
                tie(dst)
        for t in range(t0, t1):
            if _share(tasks, t - t0, t1 - t0):
                events.setdefault(t, []).append(functools.partial(run, _share(tasks, t - t0, t1 - t0)))

    events, end, w1, w2, wa = {}, LT * NC, 280, 570, 140

    def wo_wait(n, batch):
        cp(wo_c.at[:, 0:n * 64], wo_c.at[:, 0:n * 64], sem_wo.at[batch]).wait()
    spread(events, a_attention(1), 12, wa, qkv1, oa1)
    spread(events, w_turn(GQ[14], wq) + [lambda: [get_wo(t, 6, 1) for t in range(30, NF, 6)]], wa, wa + 1)
    spread(events, w_combine(GQ[13], wq), wa, w1, wq_c1, wl_s)
    spread(events, [lambda: wo_wait(30, 0), c_bx[1].start], w1, w1 + 1)
    spread(events, w_combine(GQ[14], wq), w1 + 12, w1 + 35, wl_c, wl_s)
    spread(events, sum([w_combine(g, wo) for g in GO[:3]], []), w1 + 35, w2, wo_c, wo_s)
    spread(events, [lambda: wo_wait(18, 1)], w2, w2 + 1)
    spread(events, sum([w_combine(g, wo) for g in GO[3:]], []), w2 + 12, end + 0, wo_c, wo_s)
    spread(events, [functools.partial(a_last, c, k) for k in range(LT) for c in range(LT)], end, end + LT * NF)
    product = attend(0, 0, [_cat([mem[:, k * 128:(k + 1) * 128].astype(F32), x]) for k, x in enumerate(tokens(0))],
                     events)
    product.passed(0, True)
    m = [None] * LT
    for c in range(NF):
        for k in range(LT):
            g = GO[c // 10]
            w = g.tile(wo, ("cell", c, k))
            m[k] = _add(m[k], product.now(lambda: att[c, 0:M], w)[0])
    product.passed(0, True)
    for k in range(LT):
        mem_s[k] = m[k]

    def two_steps(n, m):
        m = project_out(1, 2 * n + 1, attend(1, 2 * n + 1, m, {}))
        m = project_out(0, 2 * n + 2, attend(0, 2 * n + 2, m, {}))
        c_out(1, _ds(n, 2 * SEG)).start()
        return m

    def b_step(it, carry):
        m = [mem_s[k] for k in range(LT)]
        for u in range(1):
            m = two_steps(1 * it + u, m)
        for k in range(LT):
            mem_s[k] = m[k]
        return carry

    c_out(0, pl.ds(0, S)).start()
    c_bx[1].wait()
    lax.fori_loop(0, (NSEG // 2 - 1) // 1, b_step, 0)
    m = [mem_s[k] for k in range(LT)]
    if 1 > 1:
        m = two_steps(NSEG // 2 - 2, m)
    product = attend(1, NSEG - 1, m, {}, last=True)
    project_out(1, NSEG - 1, product, last=True)
    project_out(0, NSEG, product, last=True)
    c_out(1, _ds(NSEG // 2 - 1, 2 * SEG)).start()
    wait([c_out(j, pl.ds(0, S)) for j in range(2)])


def pallas_concat_heads__sliding_local_dilated__memory_aug_recurrent_mem_tr__prompt_kernel(
    A_x, A_wqkv, A_wo, B_x, B_mem0, B_Wq, B_Wk, B_Wv, B_Wo, B_seg_len,
):
    assert B_seg_len == SEG
    assert A_x.shape == B_x.shape == (1, S, D) and B_mem0.shape == (1, M, D)
    assert B_Wq.shape == B_Wk.shape == B_Wv.shape == (D, H, DH) and B_Wo.shape == (H, DH, D)
    vmem, dma = pltpu.VMEM, pltpu.SemaphoreType.DMA
    call = pl.pallas_call(
        _kernel,
        out_shape=jax.ShapeDtypeStruct((S, 2 * D), BF16),
        in_specs=[pl.BlockSpec(memory_space=pl.ANY)] * 9,
        out_specs=pl.BlockSpec(memory_space=pl.ANY),
        scratch_shapes=[
            vmem((S, D), BF16),
            vmem((3, D, D), BF16),
            vmem((D, D), BF16),
            vmem((LT, D, 128), F32),
            vmem((3 * D // 2, D), U32),
            vmem((D // 2, D), U32),
            vmem((2, TB, D), F32),
            vmem((3 * LT + 1, HALO + TB, 128), F32), vmem((3 * LT + 1, HALO + TB, 128), F32),
            vmem((LT + 1, TB, 128), F32), vmem((LT + 1, TB, 128), F32),
            vmem((S, D), BF16),
            vmem((S, D), BF16),
            vmem((M, D), BF16),
            vmem((LT, NC * 64 + 8, 128), U32),
            vmem((351, 64, 128), U32), vmem((351, 64, 128), U32), vmem((521, 128, 128), BF16),
            vmem((LT, NF * 64 + 8, 128), U32), vmem((4 * NF, 128, 128), BF16),
            vmem((21, 64, 128), U32), vmem((53, 128, 128), BF16),
            vmem((LT, M, 128), F32),
            vmem((2, LT, L + SEG, 128), F32),
            vmem((2, len(SUMS), L + SEG, 128), F32),
            vmem((2, LT, SEG, 128), F32),
            vmem((2, len(MIXES), HALF, 128), F32),
            vmem((NC, L, 128), F32), vmem((NC, L, 128), F32),
            vmem((len(GQ), LT, SEG, 128), F32),
            vmem((NF, L + SEG, 128), F32),
            vmem((NF, SEG, 128), F32),
            vmem((LT, SEG, 128), F32), vmem((LT, SEG, 128), F32),
            dma((7,)), dma((NB,)), dma((NB,)), dma((2,)), dma((2,)),
        ],
        compiler_params=pltpu.CompilerParams(vmem_limit_bytes=127 * 1024 * 1024, disable_bounds_checks=True, disable_semaphore_checks=True),
        name="sliding_and_memory_attention",
    )

    def by_feature(w):
        return w.transpose(1, 2, 0).reshape(H * DH, D)

    out = call(A_x.reshape(S, D), A_wqkv, A_wo, B_x.reshape(S, D), B_mem0.reshape(M, D),
               by_feature(B_Wq), by_feature(B_Wk), by_feature(B_Wv), B_Wo.reshape(H * DH, D))
    return out.reshape(1, S, 2 * D)
```

```python
import functools

import jax
import jax.numpy as jnp
from jax import lax
from jax.experimental import pallas as pl
from jax.experimental.pallas import tpu as pltpu

F32, BF16, U32 = jnp.float32, jnp.bfloat16, jnp.uint32
NT = (((1,), (1,)), ((), ()))
MASKED = -1000000000.0
LOG2E = 1.4426950408889634

S, D = 2048, 640
LT = D // 128

AH, AD, AW, ADIL = 32, 20, 8, 2
HALO = 16
TB = 128
NB = S // TB

H, DH, M, SEG = 32, 192, 8, 32
L = M + SEG
HALF = SEG // 2
NSEG = S // SEG
NF = H * DH // 128
SUMS = [(i, j) for i in range(LT) for j in range(i + 1, LT)]
MIXES = [(i, j) for i in range(LT) for j in range(LT) if i != j]

NG = H // 4
TILE = ((1, 2, 0), (3, 4, 5))
PIECES = ((0, 40, 80), (168, 208, 248), (384, 128, 424), (600, 296, 336), (472, 560, 512), (640, 680, 720))
CUTS = (0, L, 2 * L, 128)


class _Group:
    def __init__(self, j, first):
        u_diag, w_diag = (range(LT), range(LT)) if first + 10 <= NF else (range(4), range(1, 5))
        self.j, self.first = j, first
        self.us = [(first + n, i) for n, i in enumerate(u_diag)]
        self.ws = [(first + len(u_diag) + n, j) for n, j in enumerate(w_diag)]
        self.pairs = [(u, i, w, j) for u, i in self.us for w, j in self.ws if i != j]
        paired = [(u, j) for u, i, w, j in self.pairs] + [(w, i) for u, i, w, j in self.pairs]
        self.direct = [(c, k) for c, d in self.us + self.ws for k in range(LT)
                       if k != d and (c, k) not in paired]
        self.seat = dict(self.us + [(w, LT + j) for w, j in self.ws])


K, Q, V, O = range(4)
GQ = [_Group(j, t) for t in (0, 10, 20) for j in (K, Q, V)]
GQ += [_Group(j, t) for j, t in ((K, 30), (Q, 30), (K, 40), (Q, 40), (V, 30), (V, 40))]
GO = [_Group(O, t) for t in range(0, NF, 10)]


def _first_row(j, c, n):
    return (j * NG + c // 6) * 384 + PIECES[c % 6][n] // 2


def _ds(i, n, size=None):
    return pl.ds(i * n if isinstance(i, int) else pl.multiple_of(i * n, n), size or n)


def _dot(a, b):
    return jnp.dot(a, b, preferred_element_type=F32)


def _recip(x):
    r = pl.reciprocal(x, approx=True)
    return r * (2.0 - x * r)


def _add(a, b):
    return b if a is None else a + b


def _sub(a, b):
    return -b if a is None else a - b


def _total(xs):
    return functools.reduce(jnp.add, xs)


def _vregs(x):
    return [x[r:r + 8] for r in range(0, x.shape[0], 8)]


def _cat(xs):
    return jnp.concatenate(xs, axis=0)


def _share(tasks, k, n):
    return tasks[k * len(tasks) // n:(k + 1) * len(tasks) // n]


def _run(tasks):
    for task in tasks:
        task()


class _Products:
    def __init__(self, events, tied):
        self.events, self.tied, self.results = events, tied, []
        self.count, self.usual, self.flushed, self.waiting = 0, 0, -1, {}

    def dot(self, x, w):
        self.results.append(_vregs(_dot(self.tied(x), pltpu.bitcast(w, BF16))))
        return self.results[-1]

    def tick(self):
        self.count += 1
        _run(self.events.pop(self.count - 1, []))

    def now(self, x, w):
        self.tick()
        r = self.dot(x(), w[...])
        self.passed(1)
        return r

    def soon(self, x, w, use):
        self.waiting.setdefault(x.shape[0], []).append([x, w[...], [use]])

    def after(self, rows, task):
        if self.waiting.get(rows):
            self.waiting[rows][-1][2].append(lambda r: task())
        else:
            task()

    def passed(self, n, last=False):
        self.usual += n
        for rows in sorted(self.waiting, reverse=True):
            queue = self.waiting[rows]
            while queue and (last or (len(queue) >= 4 and self.usual % 4 == 0
                                      and (self.flushed < self.usual or len(queue) >= 8 or rows >= L))):
                for x, w, uses in queue[:4]:
                    r = self.dot(x, w)
                    for use in uses:
                        use(r)
                del queue[:4]
                if rows < L:
                    self.flushed = self.usual


def _kernel(ax_hbm, awqkv_hbm, awo_hbm, bx_hbm, mem_hbm, wq_hbm, wk_hbm, wv_hbm, wo_hbm,
            out_hbm,
            ax, awqkv, awo, tmp, wqkv_p, wo_p, x_s, qkv0, qkv1, oa0, oa1, outa,
            bx, mem, raw, cells0, cells1, cells2, raw_o, sums, sums2, sums_o,
            mem_s, f_one, f_sum, f_dif, f_mix, cols0, cols1, part, keys, hold, att, keep, out_x, out_y,
            sources, sem_a, sem_x, sem_w, sem_o):
    qkv, oa, cols = (qkv0, qkv1), (oa0, oa1), (cols0, cols1)
    outb = ax

    cp = pltpu.make_async_copy
    c_wqkv = [cp(awqkv_hbm.at[:, pl.ds(j * D, D)], awqkv.at[j], sem_a.at[j]) for j in range(3)]
    c_awo = cp(awo_hbm, awo, sem_a.at[3])
    c_mem = cp(mem_hbm, mem, sem_a.at[4])
    c_bx = [cp(bx_hbm.at[rows], bx.at[rows], sem_a.at[5 + n])
            for n, rows in enumerate((pl.ds(0, 3 * SEG), pl.ds(3 * SEG, S - 3 * SEG)))]

    def c_ax(i):
        return cp(ax_hbm.at[_ds(i, TB)], ax.at[_ds(i, TB)], sem_x.at[i])

    def c_out(j, rows):
        return cp((outa, outb)[j].at[rows, :], out_hbm.at[rows, pl.ds(j * D, D)], sem_o.at[j])

    def get_w(j, t, n, batch):
        dst, first = (raw_o, t) if j == O else (raw, j * NF + t)
        for k in range(LT):
            cp((wk_hbm, wq_hbm, wv_hbm, wo_hbm)[j].at[_ds(t, 128, 128 * n), _ds(k, 128)],
               dst.bitcast(BF16).at[k, _ds(first, 128, 128 * n)], sem_w.at[batch]).start()

    def got_w(n, batch):
        cp(raw.at[:, 0:n * 64], raw.at[:, 0:n * 64], sem_w.at[batch]).wait()

    ties = []

    def paced(tasks, ref, results):
        for n, task in enumerate(tasks):
            ref[ref.shape[0] - 1 + zero, 0:8] = pltpu.bitcast(results[n * len(results) // len(tasks)], ref.dtype)
            task()

    def tie(ref):
        ties.append(ref.at[ref.shape[0] - 1 + zero, 8:16])

    def tied(x):
        head = x[0:8, 0:128]
        while ties:
            ref = ties.pop()
            ref[...] = pltpu.bitcast(head, ref.dtype)
            head = pltpu.bitcast(ref[...], x.dtype)
        if x.shape[1] > 128:
            head = jnp.concatenate([head, x[0:8, 128:]], axis=1)
        return _cat([head, x[8:]]) if x.shape[0] > 8 else head

    def permute_rows(dst, base):
        for d in range(AD):
            for t in range(LT):
                dst[pl.ds((base + d * AH) // 2, AH // 2), t * 128:(t + 1) * 128] = pltpu.bitcast(
                    tmp[t, pl.ds(d, AH, stride=AD), :].astype(BF16), U32)

    def prep_wqkv(j):
        for t in range(LT):
            tmp[t] = awqkv[j, t * 128:(t + 1) * 128, :].astype(F32).T
        permute_rows(wqkv_p, j * D)

    def prep_wo():
        for t in range(LT):
            tmp[t] = awo[:, t * 128:(t + 1) * 128].astype(F32)
        permute_rows(wo_p, 0)

    def a_pass(i, b, c, k0=0, k1=LT):
        lanes = slice(c % LT * 128, c % LT * 128 + 128)
        if c < 3 * LT:
            if c == k0 == 0:
                x_s[b] = ax[_ds(i, TB), :].astype(F32)
            w = pltpu.bitcast(wqkv_p[c * 64:(c + 1) * 64, k0 * 128:k1 * 128], BF16)
            r = lax.dot_general(tied(x_s[b, :, k0 * 128:k1 * 128]), w, NT, preferred_element_type=F32)
        else:
            x = jnp.concatenate([oa[1 - b][k] for k in range(k0, k1)], axis=1)
            r = _dot(tied(x), pltpu.bitcast(wo_p[k0 * 64:k1 * 64, lanes], BF16))
        if k0:
            r = _cat(list(map(_add, _vregs(tmp[c % 4, 0:TB]), _vregs(r))))
        if k1 < LT:
            tmp[c % 4, 0:TB] = r
        elif c >= 3 * LT:
            outa[_ds(i - 1, TB), lanes] = r.astype(BF16)
        else:
            qkv[b][c, HALO:] = r
            if c >= LT and isinstance(i, int) and i == 0:
                qkv[b][c, 0:HALO] = jnp.broadcast_to(r[0:1, :], (HALO, 128))
            elif c >= LT:
                qkv[b][c, 0:HALO] = qkv[1 - b][c, TB:]
        return _vregs(r)

    def a_attention(b, first_block=False):
        state = {}

        def window(c, r0, w):
            return qkv[b][c, HALO + r0 - ADIL * w:HALO + r0 - ADIL * w + 8]

        def logits(r0, ws):
            q = [window(t, r0, 0) for t in range(LT)]
            for w in ws:
                a = _total([q[t] * window(LT + t, r0, w) for t in range(LT)])
                a = _total([a] + [pltpu.roll(a, d, 1) for d in range(AH, 128, AH)])
                if first_block and r0 < ADIL * w:
                    pos = lax.broadcasted_iota(jnp.int32, (8, 128), 0) + r0
                    a = jnp.where(pos >= ADIL * w, a, MASKED * AD ** 0.5)
                state[r0, w] = a

        def mix(r0, ts):
            if ts[0] == 0:
                lg = [state.pop((r0, w)) for w in range(AW)]
                m = functools.reduce(jnp.maximum, lg)
                state[r0] = [jnp.exp2((a - m) * (AD ** -0.5 * LOG2E)) for a in lg]
                state[r0].append(_recip(_total(state[r0])))
            e = state[r0]
            for t in ts:
                oa[b][t, r0:r0 + 8] = _total([e[w] * window(2 * LT + t, r0, w) for w in range(AW)]) * e[AW]

        steps = [(0, logits, range(4)), (0, logits, range(4, AW)), (8, mix, range(1)), (8, mix, range(1, LT))]
        return [functools.partial(f, r0 - lag, some) for r0 in range(0, TB + 8, 8)
                for lag, f, some in steps if 0 <= r0 - lag < TB]

    def place(j, first):
        return first // 10 * 3 + j

    def stored(g, name, at=None, as_words=True):
        n = place(g.j, g.first)
        if name[0] == "cell":
            slot = LT * g.seat[name[1]] + name[2]
            if n == 14:
                return cells2.at[slot]
            return (cells0, cells1)[n % 2].at[50 * ((n if at is None else at) >> 1) + slot]
        ref, n = (sums_o, g.first // 10) if g.j == O else (sums2, n - 13) if n >= 13 else (sums, n)
        if name[0] == "both":
            slot = 20 + MIXES.index((g.seat[name[1]], g.seat[name[2]] - LT))
        else:
            slot = 10 * "-+".index(name[0]) + g.seat[name[1]]
        return (ref.bitcast(U32) if as_words else ref).at[40 * (n if at is None else at) + slot]

    def runs(ref, k, r0, r1, r2):
        if isinstance(r0, int) and r1 == r0 + L // 2:
            return ref[k, r0:r0 + 64]
        low = lax.broadcasted_iota(jnp.int32, (8, 128), 0) < 4
        x, y = ref[k, pl.ds(r0, 24)], ref[k, pl.ds(r1 - 4, 24)]
        return _cat([x[0:16], jnp.where(low, x[16:], y[0:8]), y[8:], ref[k, pl.ds(r2, 24)]])

    def weight(g, name, at=None):
        if g.j == O and name[0] == "cell":
            return runs(raw_o, name[2], *[_first_row(0, name[1], n) for n in range(3)])
        return stored(g, name, at)

    def w_turn(g, at=None):
        def turn(c, k, *rows):
            stored(g, ("cell", c, k), at)[...] = pltpu.bitcast(pltpu.bitcast(runs(raw, k, *rows), BF16).T, U32)
        tasks = []
        for c, _ in g.us + g.ws:
            rows = [_first_row(g.j, c, n) if at is None else sources[30 * at + 3 * c + n] for n in range(3)]
            tasks += [functools.partial(turn, c, k, *rows) for k in range(LT)]
        return [functools.partial(_run, tasks[n:n + 2]) for n in range(0, len(tasks), 2)]

    def w_combine(g, at=None):
        minus, plus = {}, {}

        def get(r, c, k, optional=False):
            x = weight(g, ("cell", c, k), at)[r // 2:r // 2 + 8]
            return pltpu.bitcast(jnp.where(at < 12, x, 0) if optional else x, BF16).astype(F32)

        def put(r, x, *name):
            stored(g, name, at, as_words=False)[r:r + 16] = x.astype(BF16)

        def combine(r, pair):
            u, i, w, j = pair
            optional = at is not None and g.j == 0 and (i == LT - 1 or j == 0)
            x, y = get(r, u, j, optional), get(r, w, i, optional)
            put(r, x + y, "both", u, w)
            if g.j == O:
                x, y = y, x
            for c, d, own, other in ((u, i, x, y), (w, j, y, x)):
                mine = [p for p in g.pairs if c in (p[0], p[2])]
                if pair == mine[0]:
                    minus[c] = plus[c] = get(r, c, d)
                minus[c], plus[c] = minus[c] - own, plus[c] + other
                if pair == mine[-1]:
                    put(r, minus[c], "-", c)
                    put(r, plus[c], "+", c)
        return [functools.partial(combine, r, pair) for r in range(0, 128, 16) for pair in g.pairs]

    for c in (c_wqkv[0], c_ax(0), c_wqkv[1], c_ax(1)):
        c.start()

    def touch(i, carry):
        for ref in (x_s, f_one, f_sum, f_dif, f_mix, cols0, cols1, part, keys, hold, att, keep,
                    out_x, out_y, tmp, cells0, cells1, cells2, sums, sums2, sums_o):
            ref[(i,) + (0,) * (len(ref.shape) - 3) + (slice(0, 16),)] = jnp.zeros((16, ref.shape[-1]), ref.dtype)
        for ref in (wqkv_p, wo_p):
            ref[_ds(i, 8)] = jnp.zeros((8, D), U32)
        return i
    zero = lax.shift_right_logical(lax.fori_loop(0, 2, touch, 0), 16)

    for g in GQ:
        tiles = {seat: c for c, seat in g.seat.items()}
        for n in range(30):
            sources[30 * place(g.j, g.first) + n] = _first_row(g.j, tiles.get(n // 3, g.first), n % 3)

    c_wqkv[0].wait()
    c_wqkv[2].start()
    prep_wqkv(0)
    c_ax(0).wait()
    for c in range(LT):
        a_pass(0, 0, c)
    c_wqkv[1].wait()
    c_ax(1).wait()
    c_awo.start()
    c_ax(2).start()
    prep_wqkv(1)
    for c in range(LT):
        a_pass(1, 1, c)
    c_wqkv[2].wait()
    get_w(K, 0, 6, 2)
    get_w(K, 6, 5, 2)
    prep_wqkv(2)
    for n in range(2 * LT):
        a_pass(n // LT, n // LT, LT + n % LT)
    c_awo.wait()
    get_w(Q, 0, 6, 3)
    get_w(Q, 6, 5, 3)
    get_w(V, 0, 1, 4)
    for c in (c_ax(3), c_mem, c_bx[0]):
        c.start()
    prep_wo()
    for n in range(2 * LT):
        a_pass(n // LT, n // LT, 2 * LT + n % LT)
    _run(a_attention(0, True))
    for c in range(LT):
        a_pass(1, 1, 3 * LT + c)

    def a_step(it, carry):
        for b in range(2):
            i = 2 * it + b
            for n, needed in ((1, i < 5), (3, i < 14)):
                pl.when(needed)(functools.partial(got_w, n, i))
            got_w(7, i)
            c_ax(i).wait()
            third = (i * 43) >> 7
            for j in range(3):
                for t, n, needed in ((1, 7, i < 15), (8, 3, i < 12)):
                    pl.when(needed & (i - 3 * third == j))(functools.partial(get_w, j, 10 * third + t, n, i + 2))
            pl.when(it < NB // 2 - 1)(lambda: c_ax(i + 2).start())
            for g in ((0, 1), (2, 3, 4))[b]:
                pl.when(it == NB // 2 - 1)(functools.partial(get_w, O, 6 * g, 6, 0))
            combine = w_combine(_Group(1 - b, 0), jnp.where(i < 3, 11, i - 3))
            side = [(a_attention(1 - b), 0, 17, 3, qkv[1 - b], oa[1 - b]),
                    (w_turn(_Group(b, 0), i - 2), 20, 5 * LT, 99, raw, (cells0, cells1)[b]),
                    (combine[:90], 0, 17, 2, (cells1, cells0)[b], sums.bitcast(U32)),
                    (combine[90:], 17, 24, 2, (cells1, cells0)[b], sums.bitcast(U32))]
            rs = []
            for c in range(5 * LT):
                if c % 5 < 4:
                    rs.append(a_pass(i, b, c - c // 5, 0, 4))
                else:
                    rs.append([a_pass(i, b, c // 5 * 4 + n, 4, LT) for n in range(4)][0])
                for tasks, c0, c1, lag, src, dst in side:
                    if c0 <= c < c1:
                        if len(rs) < lag:
                            _run(_share(tasks, c - c0, c1 - c0))
                        else:
                            paced(_share(tasks, c - c0, c1 - c0), src, rs[-lag])
                        tie(dst)
            ties.clear()
        return carry

    lax.fori_loop(1, NB // 2, a_step, 0)
    got_w(7, NB)
    c_mem.wait()
    c_bx[0].wait()
    for g in range(5, NG):
        get_w(O, 6 * g, 6, 1)

    def tokens(s):
        return [bx[_ds(s, SEG), k * 128:(k + 1) * 128].astype(F32) for k in range(LT)]

    def project_group(odd, g, product, nm):
        pa, pb = (g.ws, g.us) if odd else (g.us, g.ws)
        half, same, cross = slice(HALF * odd, HALF * odd + HALF), {}, {}

        def with_memory(x, k):
            return _cat([x, f_one[odd, k, SEG:L]]) if nm else x

        def prod(lhs, *name):
            return product.now(lhs, weight(g, name))

        def direct(c):
            for _, k in [x for x in g.direct if x[0] == c]:
                r = prod(lambda: f_one[odd, k, 0:SEG + nm], "cell", c, k)
                same[c] = list(map(_add, same[c], r))

        def other(a):
            return cols1.at[g.j, a, M:L] if odd else part.at[place(g.j, a), a % 10]

        def mixed(a, b, r):
            cross[a] = list(map(_add, cross.get(a) or _vregs(other(a)[half]), r))
            for x, h in zip(r, (2 * odd, 2 * odd + 1, 4)):
                same[b][h] = same[b][h] + x

        def save_cross(a):
            other(a)[half] = _cat(cross.pop(a))

        def save(c, more=None):
            if nm:
                cols[odd][g.j, c, 0:M] = same[c][4]
            cols[1 - odd][g.j, c, M:L] = _add(more, _cat(same[c][:4]))
        for some in (pb[:-2], pb[-2:]):
            for b, j in some:
                same[b] = list(prod(lambda: with_memory(f_dif[odd, j], j), "+", b))
                direct(b)
            for a, i in pa:
                if a not in same:
                    same[a] = prod(lambda: f_one[odd, i, 0:SEG + nm], "-", a)
                    x = _add(other(a)[...] if odd else None, _cat(same[a][:4]))
                    other(a)[HALF - half.start:SEG - half.start] = x[HALF - half.start:SEG - half.start]
                    cross[a] = _vregs(x[half])
                    direct(a)
                else:
                    same[a] = _vregs(cols[1 - odd][g.j, a, M:L]) + ([cols[odd][g.j, a, 0:M]] if nm else [])
                for b, j in some:
                    if i != j:
                        product.tick()
                        product.soon(with_memory(f_mix[odd, MIXES.index((i, j))], i),
                                     weight(g, ("both", b, a) if odd else ("both", a, b)),
                                     functools.partial(mixed, a, b))
                for b, j in some:
                    if i != j:
                        r = prod(lambda: f_sum[odd, SUMS.index((min(i, j), max(i, j))), 0:SEG + nm], "cell", a, j)
                        same[a] = list(map(_add, same[a], r))
                        same[b] = list(map(_sub, same[b], r))
                save(a)
                product.after(HALF + nm, functools.partial(save_cross, a))
            for b, _ in some:
                product.after(HALF + nm, functools.partial(save, b, part[place(g.j, b), b % 10] if odd else None))

    def project_last(g, product):
        def use(u, k, r):
            cols1[g.j, u, 0:M] = r[0] + cols1[g.j, u, 0:M] if k else r[0]
        for (u, _), (w, _) in zip(g.us, g.ws):
            r = [None] * 5
            for k in range(LT):
                product.tick()
                if g.j != Q:
                    product.soon(f_one[1, k, SEG:L], weight(g, ("cell", u, k)), functools.partial(use, u, k))
                r = list(map(_add, r, product.now(lambda: f_one[1, k, 0:L], weight(g, ("cell", w, k)))))
            cols1[g.j, w] = _cat(r[4:] + r[:4])

    def out_groups(odd, gs, same, cross, product, last):
        h0, nh = (0, SEG * odd) if last else (2 - 2 * odd, HALF)
        mix = {}

        def xa(c, r0=0, n=SEG):
            return att[c, M + SEG * (1 - odd) + r0:M + SEG * (1 - odd) + r0 + n]

        def xb(c, r0=0, n=SEG):
            return att[c, L + r0:L + r0 + n] if odd else keep[c, r0:r0 + n]

        def xm(c):
            return att[c, 0:M]

        def prod(g, m, x, *name):
            r = product.now(lambda: x() if last else _cat([m(), x()]), weight(g, name))
            return r if last else r[1:] + r[:1]

        def mixed(s, t, r):
            mix[s, t] = list(map(_add, mix.get((s, t), [None] * 4), r))

        def spend(s, t):
            for x, h in zip(mix.pop((s, t), []), list(range(h0, h0 + nh // 8)) + [4]):
                same[t][h] = _add(same[t][h], x)
                if h < 4:
                    cross[s][h] = _add(cross[s][h], x)
        sides = [(g, {d: c for c, d in (g.us if odd else g.ws)}, {d: c for c, d in (g.ws if odd else g.us)})
                 for g in gs]
        for i in range(LT):
            shared = [None] * 5
            for g, pa, pb in sides:
                rs = [prod(g, lambda: xm(pb[i]), lambda: xa(pb[i]) - xb(pb[i]), "+", pb[i])] if i in pb else []
                rs += [prod(g, lambda: xm(c), lambda: xa(c), "cell", c, k) for c, k in g.direct if k == i]
                for r in rs:
                    same[i] = list(map(_add, same[i], r))
                if i in pa:
                    shared = list(map(_add, shared, prod(g, lambda: xm(pa[i]), lambda: xa(pa[i]), "-", pa[i])))
                    if odd:
                        keep[pa[i]] = xa(pa[i])
            same[i] = list(map(_add, same[i], shared))
            cross[i] = list(map(_add, cross[i], shared))
            for j in range(i + 1, LT):
                diff = [None] * 5
                for s, t in ((i, j), (j, i)):
                    for g, pa, pb in sides:
                        if s in pa and t in pb:
                            a, b = pa[s], pb[t]
                            if nh:
                                product.tick()
                                x = xa(a, 8 * h0, nh) + xb(b, 8 * h0, nh)
                                product.soon(x if last else _cat([x, xm(a)]),
                                             weight(g, ("both", a, b) if odd else ("both", b, a)),
                                             functools.partial(mixed, s, t))
                            r = prod(g, lambda: xm(a) + xm(b), lambda: xa(a) + xa(b), "cell", b, s)
                            diff = list(map(_add if s == i else _sub, diff, r))
                    product.after(nh if last else nh + M, functools.partial(spend, s, t))
                same[i] = list(map(_add, same[i], diff))
                same[j] = list(map(_sub, same[j], diff))

    def project_out(odd, s, product, last=False):
        same, cross = [[None] * 5 for _ in range(LT)], [[None] * 4 for _ in range(LT)]
        for gs in (GO[:3], GO[3:]):
            assert gs[0] is GO[0] or not product.events
            out_groups(odd, gs, same, cross, product, last)
        product.passed(0, True)
        for k in range(LT):
            lanes = slice(k * 128, (k + 1) * 128)
            if odd:
                out_x[k], out_y[k] = _cat(same[k][:4]), _cat(cross[k])
            else:
                outb[_ds(s - 2, SEG), lanes] = (out_x[k] + _cat(cross[k])).astype(BF16)
                outb[_ds(s - 1, SEG), lanes] = (out_y[k] + _cat(same[k][:4])).astype(BF16)
        return [x[-1] for x in same]

    def attend(odd, s, m, product, last=False):
        xa, xb = tokens(jnp.minimum(s + 1, NSEG - 1)), tokens(s if odd else jnp.minimum(s + 2, NSEG - 1))
        nm = M if m[0].shape[0] == M else 0
        for k in range(LT):
            f_one[odd, k, 0:SEG + m[k].shape[0]] = _cat([xa[k], m[k]])
            f_dif[odd, k] = xa[k] - xb[k]
        for n, (i, j) in enumerate(SUMS):
            f_sum[odd, n] = _cat([xa[i] + xa[j], m[i][0:M] + m[j][0:M]])
        for n, (i, j) in enumerate(MIXES):
            f_mix[odd, n] = (xa[i] + xb[j])[HALF * odd:HALF * odd + HALF]

        lane = lax.broadcasted_iota(jnp.int32, (L, 128), 1)
        zone = [(lane >= L * z) & (lane < L * z + L) for z in range(3)]
        some = [(lane >= 24 + 16 * n) & (lane < 40 + 16 * n) for n in range(2)]

        def tile(j, g, n, z):
            return cols[odd][j, 6 * g + TILE[n][z]]

        def gathered(j, g, n):
            x = jnp.where(zone[2], tile(j, g, n, 2), 0.0) if j == K else tile(j, g, n, 2)
            return jnp.where(zone[0], tile(j, g, n, 0), jnp.where(zone[1], tile(j, g, n, 1), x))

        def stack(xs):
            return _cat(xs + [jnp.zeros((8, 128), F32)])

        def by_head(x, a, of_a):
            xs = [jnp.zeros((L, 128), F32)] * 2 + [x]
            if a < 2:
                xs[a], xs[2] = jnp.where(of_a, x, 0.0), jnp.where(of_a, 0.0, x)
            return stack(xs)

        def turned(slot, x):
            keys[slot] = x.T
            return keys[slot]

        def one_pass(x, w):
            r = _dot(x, w.astype(BF16))
            product.passed(1)
            return _cat(_vregs(r))

        def done(g, n, z, o):
            att[6 * g + TILE[n][z], 0:M] = o[0:M]
            att[6 * g + TILE[n][z], M + SEG * odd:L + SEG * odd] = o[M:L]

        def alone(j, g):
            sc = {}
            for z in (2, 1, 0):
                for n in range(2):
                    w = by_head(tile(j, g, n, z), z, ~zone[z] | some[n] if z == n else ~zone[z])
                    if j == V:
                        p = hold[g, 2 + n] if z in (2, n) else jnp.where(zone[2], hold[g, 2 + n], hold[g, 2 + z])
                        done(g, n, z, one_pass(p, w))
                        continue
                    r = one_pass(tile(Q, g, n, z), turned(3 * n + z, w))
                    if z in (2, n):
                        sc[n] = _add(sc.get(n), r)
                    else:
                        sc[n], sc[z] = sc[n] + jnp.where(zone[2], r, 0.0), sc[z] + jnp.where(zone[2], 0.0, r)
            for n in sc:
                hold[g, n] = sc[n]

        def zone_scores(g):
            for n in range(2):
                turned(4 * g + 2 + n, stack([tile(K, g, n, z) for z in range(3)]))
            for n in range(2):
                hold[g, n] = one_pass(gathered(Q, g, n), turned(4 * g + 4 + n, by_head(gathered(K, g, n), n, some[n])))

        def together(g):
            for n in range(2):
                hold[g - 1, 4 + n] = one_pass(hold[g - 1, 2 + n], by_head(gathered(V, g - 1, n), n, some[n]))
                for z in range(3):
                    h = n if z == 2 else z
                    w = [jnp.where(zone[z][0:8], y, 0.0) for y in _vregs(keys[4 * g + 2 + n])]
                    w[5 * z:5 * z + 5] = [jnp.where(zone[z], 0.0, tile(V, g - 1, n, z))]
                    r = one_pass(jnp.where(zone[z], hold[g - 1, 2 + h], tile(Q, g, n, z)), _cat(w))
                    hold[g, h] = hold[g, h] + jnp.where(zone[z], r, 0.0)
                    done(g - 1, n, z, jnp.where(zone[z], hold[g - 1, 4 + n], r))

        def softmax(g):
            ahead = lane[0:8] % L - lax.broadcasted_iota(jnp.int32, (8, 128), 0)
            for n in range(2):
                x = _cat([jnp.where(ahead <= 8 * b, y, MASKED * DH ** 0.5) if b else y
                          for b, y in enumerate(_vregs(hold[g, n]))])
                top = [jnp.max(jnp.where(zone[z], x, -jnp.inf), axis=1, keepdims=True) for z in (n, 2)]
                e = jnp.exp2((x - jnp.where(zone[2], top[1], top[0])) * (DH ** -0.5 * LOG2E))
                e = [jnp.where(zone[z], e, 0.0) for z in (n, 2)]
                total = [jnp.sum(y, axis=1, keepdims=True) for y in e]
                hold[g, 2 + n] = (e[0] + e[1]) * _recip(jnp.where(zone[2], total[1], total[0]))

        def complete(j, g):
            n = max(n for n, x in enumerate(GQ) if x.j == j and x.first < 6 * g + 6)
            return sum(LT * len(x.us + x.ws) for x in GQ[:n + 1])

        def at(t, f, *args):
            product.events.setdefault(t, []).append(functools.partial(f, *args))
        t = complete(Q, 0) + 48
        at(t, alone, K, 0)
        at(t, softmax, 0)
        for g in range(1, NG):
            t = max(t + 78, complete(Q, g) + (80 if last else 70 if nm else 70), complete(V, g - 1) + 48) + (0, -6, 0, 0, 3, 3, 0, 0)[g]
            at(t - 0, zone_scores, g)
            at(t, together, g)
            at(t, softmax, g)
        at(t + 56, alone, V, NG - 1)
        for g in GQ:
            if last:
                project_last(g, product)
            else:
                project_group(odd, g, product, nm)
        return product

    first, partial = _Products({}, tied), {}

    def spread(tasks, t0, t1, src=None, dst=None):
        def run(some):
            if src is None or len(first.results) < 32:
                _run(some)
            else:
                paced(some, src, first.results[-32])
            if dst is not None:
                tie(dst)
        for t in range(t0, t1):
            if _share(tasks, t - t0, t1 - t0):
                first.events.setdefault(t, []).append(functools.partial(run, _share(tasks, t - t0, t1 - t0)))

    def plain(g, c, k):
        def use(r):
            partial[c] = list(map(_add, r, partial[c])) if k else r
            if k == LT - 1:
                cols0[g.j, c] = _cat(partial[c])
        first.soon(f_one[0, k, SEG:], weight(g, ("cell", c, k)), use)

    def a_last(c, k):
        def use(r):
            x = _cat(list(map(_add, _vregs(tmp[c, 0:TB]), r)) if k else r)
            if k < LT - 1:
                tmp[c, 0:TB] = x
            else:
                outa[S - TB:S, c * 128:(c + 1) * 128] = x.astype(BF16)
        first.soon(oa1[k], wo_p.at[k * 64:(k + 1) * 64, c * 128:(c + 1) * 128], use)

    def wo_wait(n, batch):
        got_w(6 * n, batch)
    end = 3 * NF * LT
    spread(a_attention(1), 12, 140, qkv1, oa1)
    spread(w_turn(_Group(V, 40)), 140, 140 + 1)
    spread(w_combine(_Group(Q, 40)), 140, 240, cells1, sums2.bitcast(U32))
    spread([lambda: wo_wait(5, 0), c_bx[1].start],
           270, 270 + 1)
    spread(w_combine(_Group(V, 40)), 270 + 12, 270 + 60, cells2, sums2.bitcast(U32))
    spread(sum([w_combine(g) for g in GO[:3]], []), 270 + 60, 580, raw_o, sums_o.bitcast(U32))
    spread([lambda: wo_wait(3, 1)], 580, 580 + 1)
    spread(sum([w_combine(g) for g in GO[3:]], []), 580 + 12, end + 0, raw_o, sums_o.bitcast(U32))
    spread([functools.partial(a_last, c, k) for k in range(LT) for c in range(LT)], end, end + LT * NF)
    spread([functools.partial(plain, g, c, k) for g in GQ for c, _ in g.us + g.ws for k in range(LT)], 0, end - 2)
    attend(0, 0, [_cat([mem[:, k * 128:(k + 1) * 128].astype(F32), x]) for k, x in enumerate(tokens(0))], first)
    first.passed(0, True)
    m = [None] * LT
    for c in range(NF):
        for k in range(LT):
            m[k] = _add(m[k], first.now(lambda: att[c, 0:M], weight(GO[c // 10], ("cell", c, k)))[0])
    first.passed(0, True)
    for k in range(LT):
        mem_s[k] = m[k]
    c_out(0, pl.ds(0, S)).start()
    c_bx[1].wait()

    def b_step(n, carry):
        m = [mem_s[k] for k in range(LT)]
        for odd in (1, 0):
            m = project_out(odd, 2 * n + 2 - odd, attend(odd, 2 * n + 2 - odd, m, _Products({}, tied)))
        for k in range(LT):
            mem_s[k] = m[k]
        c_out(1, _ds(n, 2 * SEG)).start()
        return carry

    lax.fori_loop(0, NSEG // 2 - 1, b_step, 0)
    final = attend(1, NSEG - 1, [mem_s[k] for k in range(LT)], _Products({}, tied), last=True)
    project_out(1, NSEG - 1, final, last=True)
    project_out(0, NSEG, final, last=True)
    c_out(1, _ds(NSEG // 2 - 1, 2 * SEG)).start()
    for j in range(2):
        c_out(j, pl.ds(0, S)).wait()


def pallas_concat_heads__sliding_local_dilated__memory_aug_recurrent_mem_tr__prompt_kernel(
    A_x, A_wqkv, A_wo, B_x, B_mem0, B_Wq, B_Wk, B_Wv, B_Wo, B_seg_len,
):
    assert B_seg_len == SEG
    assert A_x.shape == B_x.shape == (1, S, D) and B_mem0.shape == (1, M, D)
    assert B_Wq.shape == B_Wk.shape == B_Wv.shape == (D, H, DH) and B_Wo.shape == (H, DH, D)
    vmem, dma = pltpu.VMEM, pltpu.SemaphoreType.DMA
    call = pl.pallas_call(
        _kernel,
        out_shape=jax.ShapeDtypeStruct((S, 2 * D), BF16),
        in_specs=[pl.BlockSpec(memory_space=pl.ANY)] * 9,
        out_specs=pl.BlockSpec(memory_space=pl.ANY),
        scratch_shapes=[
            vmem((S, D), BF16),
            vmem((3, D, D), BF16),
            vmem((D, D), BF16),
            vmem((LT, D, 128), F32),
            vmem((3 * D // 2, D), U32),
            vmem((D // 2, D), U32),
            vmem((2, TB, D), F32),
            vmem((3 * LT + 1, HALO + TB, 128), F32), vmem((3 * LT + 1, HALO + TB, 128), F32),
            vmem((LT + 1, TB, 128), F32), vmem((LT + 1, TB, 128), F32),
            vmem((S, D), BF16),
            vmem((S, D), BF16),
            vmem((M, D), BF16),
            vmem((LT, 3 * NF * 64, 128), U32),
            vmem((351, 64, 128), U32), vmem((351, 64, 128), U32), vmem((51, 64, 128), U32),
            vmem((LT + 1, NF * 64, 128), U32),
            vmem((521, 128, 128), BF16), vmem((81, 128, 128), BF16), vmem((201, 128, 128), BF16),
            vmem((LT, M, 128), F32),
            vmem((2, LT, L + SEG, 128), F32),
            vmem((2, len(SUMS), L, 128), F32),
            vmem((2, LT, SEG, 128), F32),
            vmem((2, len(MIXES), HALF, 128), F32),
            vmem((3, NF, L, 128), F32), vmem((3, NF, L, 128), F32),
            vmem((len(GQ), LT, SEG, 128), F32),
            vmem((4 * NG + 2, 128, 128), F32),
            vmem((NG, 6, L, 128), F32),
            vmem((NF, L + SEG, 128), F32),
            vmem((NF, SEG, 128), F32),
            vmem((LT, SEG, 128), F32), vmem((LT, SEG, 128), F32),
            pltpu.SMEM((30 * len(GQ),), jnp.int32),
            dma((7,)), dma((NB,)), dma((NB + 1,)), dma((2,)),
        ],
        compiler_params=pltpu.CompilerParams(
            vmem_limit_bytes=124 * 1024 * 1024, disable_bounds_checks=True, disable_semaphore_checks=True),
        name="sliding_and_memory_attention",
    )

    def by_feature(w):
        return w.transpose(1, 2, 0).reshape(H * DH, D)

    out = call(A_x.reshape(S, D), A_wqkv, A_wo, B_x.reshape(S, D), B_mem0.reshape(M, D),
               by_feature(B_Wq), by_feature(B_Wk), by_feature(B_Wv), B_Wo.reshape(H * DH, D))
    return out.reshape(1, S, 2 * D)
```

```python
import functools

import jax
import jax.numpy as jnp
from jax import lax
from jax.experimental import pallas as pl
from jax.experimental.pallas import tpu as pltpu

F32, BF16, U32 = jnp.float32, jnp.bfloat16, jnp.uint32
NT = (((1,), (1,)), ((), ()))
MASKED = -1000000000.0
LOG2E = 1.4426950408889634

S, D = 2048, 640
LT = D // 128

AH, AD, AW, ADIL = 32, 20, 8, 2
HALO = 16
TB = 128
NB = S // TB

H, DH, M, SEG = 32, 192, 8, 32
L = M + SEG
HALF = SEG // 2
NSEG = S // SEG
NF = H * DH // 128
SUMS = [(i, j) for i in range(LT) for j in range(i + 1, LT)]
MIXES = [(i, j) for i in range(LT) for j in range(LT) if i != j]

NG = H // 4
TILE = ((1, 2, 0), (3, 4, 5))
PIECES = ((0, 40, 80), (168, 208, 248), (384, 128, 424), (600, 296, 336), (472, 560, 512), (640, 680, 720))
CUTS = (0, L, 2 * L, 128)


class _Group:
    def __init__(self, j, first):
        u_diag, w_diag = (range(LT), range(LT)) if first + 10 <= NF else (range(4), range(1, 5))
        self.j, self.first = j, first
        self.us = [(first + n, i) for n, i in enumerate(u_diag)]
        self.ws = [(first + len(u_diag) + n, j) for n, j in enumerate(w_diag)]
        self.pairs = [(u, i, w, j) for u, i in self.us for w, j in self.ws if i != j]
        paired = [(u, j) for u, i, w, j in self.pairs] + [(w, i) for u, i, w, j in self.pairs]
        self.direct = [(c, k) for c, d in self.us + self.ws for k in range(LT)
                       if k != d and (c, k) not in paired]
        self.seat = dict(self.us + [(w, LT + j) for w, j in self.ws])


K, Q, V, O = range(4)
GQ = [_Group(j, t) for t in (0, 10, 20) for j in (K, Q, V)]
GQ += [_Group(j, t) for j, t in ((K, 30), (Q, 30), (K, 40), (Q, 40), (V, 30), (V, 40))]
GO = [_Group(O, t) for t in range(0, NF, 10)]


def _first_row(j, c, n):
    return (j * NG + c // 6) * 96 + PIECES[c % 6][n] // 8


def _ds(i, n, size=None):
    return pl.ds(i * n if isinstance(i, int) else pl.multiple_of(i * n, n), size or n)


def _dot(a, b):
    return jnp.dot(a, b, preferred_element_type=F32)


def _recip(x):
    r = pl.reciprocal(x, approx=True)
    return r * (2.0 - x * r)


def _add(a, b):
    return b if a is None else a + b


def _sub(a, b):
    return -b if a is None else a - b


def _total(xs):
    return functools.reduce(jnp.add, xs)


def _vregs(x):
    return [x[r:r + 8] for r in range(0, x.shape[0], 8)]


def _cat(xs):
    return jnp.concatenate(xs, axis=0)


def _share(tasks, k, n):
    return tasks[k * len(tasks) // n:(k + 1) * len(tasks) // n]


def _run(tasks):
    for task in tasks:
        task()


class _Products:
    def __init__(self, events, tied):
        self.events, self.tied, self.results = events, tied, []
        self.count, self.usual, self.flushed, self.waiting = 0, 0, -1, {}

    def dot(self, x, w):
        self.results.append(_vregs(_dot(self.tied(x), pltpu.bitcast(w, BF16))))
        return self.results[-1]

    def tick(self):
        self.count += 1
        _run(self.events.pop(self.count - 1, []))

    def now(self, x, w):
        self.tick()
        r = self.dot(x(), w[...])
        self.passed(1)
        return r

    def soon(self, x, w, use):
        self.waiting.setdefault(x.shape[0], []).append([x, w[...], [use]])

    def after(self, rows, task):
        if self.waiting.get(rows):
            self.waiting[rows][-1][2].append(lambda r: task())
        else:
            task()

    def passed(self, n, last=False):
        self.usual += n
        for rows in sorted(self.waiting, reverse=True):
            queue = self.waiting[rows]
            while queue and (last or (len(queue) >= 4 and self.usual % 4 == 0
                                      and (self.flushed < self.usual or len(queue) >= 8 or rows >= L))):
                for x, w, uses in queue[:4]:
                    r = self.dot(x, w)
                    for use in uses:
                        use(r)
                del queue[:4]
                if rows < L:
                    self.flushed = self.usual


def _kernel(ax_hbm, awqkv_hbm, awo_hbm, bx_hbm, mem_hbm, wq_hbm, wk_hbm, wv_hbm, wo_hbm,
            out_hbm,
            ax, awqkv, awo, tmp, wqkv_p, wo_p, x_s, qkv0, qkv1, oa0, oa1, outa,
            bx, mem, raw, cells0, cells1, cells2, raw_o, sums, sums2, sums_o,
            mem_s, f_one, f_sum, f_dif, f_mix, cols0, cols1, part, keys, hold, att, keep, out_x, out_y,
            sources, sem_a, sem_x, sem_w, sem_o):
    qkv, oa, cols = (qkv0, qkv1), (oa0, oa1), (cols0, cols1)
    outb = ax

    cp = pltpu.make_async_copy
    c_wqkv = [cp(awqkv_hbm.at[:, pl.ds(j * D, D)], awqkv.at[j], sem_a.at[j]) for j in range(3)]
    c_awo = cp(awo_hbm, awo, sem_a.at[3])
    c_mem = cp(mem_hbm, mem, sem_a.at[4])
    c_bx = [cp(bx_hbm.at[rows], bx.at[rows], sem_a.at[5 + n])
            for n, rows in enumerate((pl.ds(0, 3 * SEG), pl.ds(3 * SEG, S - 3 * SEG)))]

    def c_ax(i):
        return cp(ax_hbm.at[_ds(i, TB)], ax.at[_ds(i, TB)], sem_x.at[i])

    def c_out(j, rows):
        return cp((outa, outb)[j].at[rows, :], out_hbm.at[rows, pl.ds(j * D, D)], sem_o.at[j])

    def get_w(j, t, n, batch):
        dst, first = (raw_o, t) if j == O else (raw, j * NF + t)
        for k in range(LT):
            cp((wk_hbm, wq_hbm, wv_hbm, wo_hbm)[j].at[_ds(t, 128, 128 * n), _ds(k, 128)],
               dst.at[k, _ds(first, 128, 128 * n)], sem_w.at[batch]).start()

    def got_w(dst, first, n, batch):
        box = dst.at[0:LT, _ds(first, 128, 128 * n)]
        cp(box, box, sem_w.at[batch]).wait()

    ties = []

    def spare(ref, n):
        return (ref.bitcast(U32) if ref.dtype == BF16 else ref).at[ref.shape[0] - 1 + zero, _ds(n, 8)]

    def paced(tasks, ref, results):
        for n, task in enumerate(tasks):
            spare(ref, 0)[...] = pltpu.bitcast(results[n * len(results) // len(tasks)], spare(ref, 0).dtype)
            task()

    def tie(ref):
        ties.append(spare(ref, 1))

    def tied(x):
        head = x[0:8, 0:128]
        while ties:
            ref = ties.pop()
            ref[...] = pltpu.bitcast(head, ref.dtype)
            head = pltpu.bitcast(ref[...], x.dtype)
        if x.shape[1] > 128:
            head = jnp.concatenate([head, x[0:8, 128:]], axis=1)
        return _cat([head, x[8:]]) if x.shape[0] > 8 else head

    def permute_rows(dst, base):
        for d in range(AD):
            for t in range(LT):
                dst[pl.ds((base + d * AH) // 2, AH // 2), t * 128:(t + 1) * 128] = pltpu.bitcast(
                    tmp[t, pl.ds(d, AH, stride=AD), :].astype(BF16), U32)

    def prep_wqkv(j):
        for t in range(LT):
            tmp[t] = awqkv[j, t * 128:(t + 1) * 128, :].astype(F32).T
        permute_rows(wqkv_p, j * D)

    def prep_wo():
        for t in range(LT):
            tmp[t] = awo[:, t * 128:(t + 1) * 128].astype(F32)
        permute_rows(wo_p, 0)

    def a_pass(i, b, c, k0=0, k1=LT):
        lanes = slice(c % LT * 128, c % LT * 128 + 128)
        if c < 3 * LT:
            if c == k0 == 0:
                x_s[b] = ax[_ds(i, TB), :].astype(F32)
            w = pltpu.bitcast(wqkv_p[c * 64:(c + 1) * 64, k0 * 128:k1 * 128], BF16)
            r = lax.dot_general(tied(x_s[b, :, k0 * 128:k1 * 128]), w, NT, preferred_element_type=F32)
        else:
            x = jnp.concatenate([oa[1 - b][k] for k in range(k0, k1)], axis=1)
            r = _dot(tied(x), pltpu.bitcast(wo_p[k0 * 64:k1 * 64, lanes], BF16))
        if k0:
            r = _cat(list(map(_add, _vregs(tmp[c % 4, 0:TB]), _vregs(r))))
        if k1 < LT:
            tmp[c % 4, 0:TB] = r
        elif c >= 3 * LT:
            outa[_ds(i - 1, TB), lanes] = r.astype(BF16)
        else:
            qkv[b][c, HALO:] = r
            if c >= LT and isinstance(i, int) and i == 0:
                qkv[b][c, 0:HALO] = jnp.broadcast_to(r[0:1, :], (HALO, 128))
            elif c >= LT:
                qkv[b][c, 0:HALO] = qkv[1 - b][c, TB:]
        return _vregs(r)

    def a_attention(b, first_block=False):
        state = {}

        def window(c, r0, w):
            return qkv[b][c, HALO + r0 - ADIL * w:HALO + r0 - ADIL * w + 8]

        def logits(r0, ws):
            q = [window(t, r0, 0) for t in range(LT)]
            for w in ws:
                a = _total([q[t] * window(LT + t, r0, w) for t in range(LT)])
                a = _total([a] + [pltpu.roll(a, d, 1) for d in range(AH, 128, AH)])
                if first_block and r0 < ADIL * w:
                    pos = lax.broadcasted_iota(jnp.int32, (8, 128), 0) + r0
                    a = jnp.where(pos >= ADIL * w, a, MASKED * AD ** 0.5)
                state[r0, w] = a

        def mix(r0, ts):
            if ts[0] == 0:
                lg = [state.pop((r0, w)) for w in range(AW)]
                m = functools.reduce(jnp.maximum, lg)
                state[r0] = [jnp.exp2((a - m) * (AD ** -0.5 * LOG2E)) for a in lg]
                state[r0].append(_recip(_total(state[r0])))
            e = state[r0]
            for t in ts:
                oa[b][t, r0:r0 + 8] = _total([e[w] * window(2 * LT + t, r0, w) for w in range(AW)]) * e[AW]

        steps = [(0, logits, range(4)), (0, logits, range(4, AW)), (8, mix, range(1)), (8, mix, range(1, LT))]
        return [functools.partial(f, r0 - lag, some) for r0 in range(0, TB + 8, 8)
                for lag, f, some in steps if 0 <= r0 - lag < TB]

    def place(j, first):
        return first // 10 * 3 + j

    def stored(g, name, at=None, as_words=True):
        n = place(g.j, g.first)
        if name[0] == "cell":
            slot = LT * g.seat[name[1]] + name[2]
            if n == 14:
                return cells2.at[slot]
            return (cells0, cells1)[n % 2].at[50 * ((n if at is None else at) >> 1) + slot]
        ref, n = (sums_o, g.first // 10) if g.j == O else (sums2, n - 13) if n >= 13 else (sums, n)
        if name[0] == "both":
            slot = 20 + MIXES.index((g.seat[name[1]], g.seat[name[2]] - LT))
        else:
            slot = 10 * "-+".index(name[0]) + g.seat[name[1]]
        return (ref.bitcast(U32) if as_words else ref).at[40 * (n if at is None else at) + slot]

    def runs(ref, k, r0, r1, r2):
        ref = ref.bitcast(U32)
        if isinstance(r0, int) and r1 == r0 + L // 8:
            return ref[k, _ds(r0, 4, 64)]
        low = lax.broadcasted_iota(jnp.int32, (8, 128), 0) < 4
        x, y = ref[k, _ds(r0, 4, 24)], ref[k, _ds(r1 - 1, 4, 24)]
        return _cat([x[0:16], jnp.where(low, x[16:], y[0:8]), y[8:], ref[k, _ds(r2, 4, 24)]])

    def weight(g, name, at=None):
        if g.j == O and name[0] == "cell":
            return runs(raw_o, name[2], *[_first_row(0, name[1], n) for n in range(3)])
        return stored(g, name, at)

    def w_turn(g, at=None):
        def turn(c, k, *rows):
            stored(g, ("cell", c, k), at)[...] = pltpu.bitcast(pltpu.bitcast(runs(raw, k, *rows), BF16).T, U32)
        tasks = []
        for c, _ in g.us + g.ws:
            rows = [_first_row(g.j, c, n) if at is None else sources[30 * at + 3 * c + n] for n in range(3)]
            tasks += [functools.partial(turn, c, k, *rows) for k in range(LT)]
        return [functools.partial(_run, tasks[n:n + 2]) for n in range(0, len(tasks), 2)]

    def w_combine(g, at=None):
        minus, plus = {}, {}
        pairs = sorted(g.pairs, key=lambda p: p[3] // (0 if at is None else 3)) if (0 if at is None else 3) else g.pairs

        def get(r, c, k, optional=False):
            x = weight(g, ("cell", c, k), at)[r // 2:r // 2 + 8]
            return pltpu.bitcast(jnp.where(at < 12, x, 0) if optional else x, BF16).astype(F32)

        def put(r, x, *name):
            stored(g, name, at, as_words=False)[r:r + 16] = x.astype(BF16)

        def combine(r, pair):
            u, i, w, j = pair
            optional = at is not None and g.j == 0 and (i == LT - 1 or j == 0)
            x, y = get(r, u, j, optional), get(r, w, i, optional)
            put(r, x + y, "both", u, w)
            if g.j == O:
                x, y = y, x
            for c, d, own, other in ((u, i, x, y), (w, j, y, x)):
                mine = [p for p in pairs if c in (p[0], p[2])]
                if pair == mine[0]:
                    minus[c] = plus[c] = get(r, c, d)
                minus[c], plus[c] = minus[c] - own, plus[c] + other
                if pair == mine[-1]:
                    put(r, minus[c], "-", c)
                    put(r, plus[c], "+", c)
        return [functools.partial(combine, r, pair) for r in range(0, 128, 16) for pair in pairs]

    for c in (c_wqkv[0], c_ax(0), c_wqkv[1], c_ax(1)):
        c.start()

    def touch(i, carry):
        for ref in (x_s, f_one, f_sum, f_dif, f_mix, cols0, cols1, part, keys, hold, att, keep,
                    out_x, out_y, tmp, cells0, cells1, cells2, sums, sums2, sums_o):
            ref[(i,) + (0,) * (len(ref.shape) - 3) + (slice(0, 16),)] = jnp.zeros((16, ref.shape[-1]), ref.dtype)
        for ref in (wqkv_p, wo_p):
            ref[_ds(i, 8)] = jnp.zeros((8, D), U32)
        return i
    zero = lax.shift_right_logical(lax.fori_loop(0, 2, touch, 0), 16)

    for g in GQ:
        tiles = {seat: c for c, seat in g.seat.items()}
        for n in range(30):
            sources[30 * place(g.j, g.first) + n] = _first_row(g.j, tiles.get(n // 3, g.first), n % 3)

    c_wqkv[0].wait()
    c_wqkv[2].start()
    prep_wqkv(0)
    c_ax(0).wait()
    for c in range(LT):
        a_pass(0, 0, c)
    c_wqkv[1].wait()
    c_ax(1).wait()
    c_awo.start()
    c_ax(2).start()
    prep_wqkv(1)
    for c in range(LT):
        a_pass(1, 1, c)
    c_wqkv[2].wait()
    get_w(K, 0, 6, 2)
    get_w(K, 6, 5, 2)
    prep_wqkv(2)
    for n in range(2 * LT):
        a_pass(n // LT, n // LT, LT + n % LT)
    c_awo.wait()
    get_w(Q, 0, 6, 3)
    get_w(Q, 6, 5, 3)
    get_w(V, 0, 1, 4)
    for c in (c_ax(3), c_mem, c_bx[0]):
        c.start()
    prep_wo()
    for n in range(2 * LT):
        a_pass(n // LT, n // LT, 2 * LT + n % LT)
    _run(a_attention(0, True))
    for c in range(LT):
        a_pass(1, 1, 3 * LT + c)

    def a_step(it, carry):
        for b in range(2):
            i = 2 * it + b
            third = (i * 43 - 86) >> 7
            t = (i - 2 - 3 * third) * NF + 10 * third
            pl.when(i < 5)(functools.partial(got_w, raw, t, 1, i))
            pl.when(i < 14)(functools.partial(got_w, raw, t + 8, 3, i))
            got_w(raw, t + 1, 7, i)
            c_ax(i).wait()
            third = (i * 43) >> 7
            for j in range(3):
                for t, n, needed in ((1, 7, i < 15), (8, 3, i < 12)):
                    pl.when(needed & (i - 3 * third == j))(functools.partial(get_w, j, 10 * third + t, n, i + 2))
            pl.when(it < NB // 2 - 1)(lambda: c_ax(i + 2).start())
            if b:
                pl.when(i > 12)(lambda: get_w(O, 6 * (i - 13), 6, it - 6))
                pl.when(i == 15)(lambda: get_w(O, 18, 6, 1))
            else:
                pl.when(i == 14)(lambda: get_w(O, 6, 6, 0))
            combine = w_combine(_Group(1 - b, 0), jnp.where(i < 3, 11, i - 3))
            side = [(a_attention(1 - b), 0, 17, 3, qkv[1 - b], oa[1 - b]),
                    (w_turn(_Group(b, 0), i - 2), 22, 5 * LT, 99, raw, (cells0, cells1)[b]),
                    (combine[:90], 0, 17, 2, (cells1, cells0)[b], sums),
                    (combine[90:], 17, 25, 2, (cells1, cells0)[b], sums)]
            rs = []
            for c in range(5 * LT):
                if c % 5 < 4:
                    rs.append(a_pass(i, b, c - c // 5, 0, 4))
                else:
                    rs.append([a_pass(i, b, c // 5 * 4 + n, 4, LT) for n in range(4)][0])
                for tasks, c0, c1, lag, src, dst in side:
                    if c0 <= c < c1:
                        if len(rs) < lag:
                            _run(_share(tasks, c - c0, c1 - c0))
                        else:
                            paced(_share(tasks, c - c0, c1 - c0), src, rs[-lag])
                        tie(dst)
            ties.clear()
        return carry

    lax.fori_loop(1, NB // 2, a_step, 0)
    got_w(raw, V * NF + 41, 7, NB)
    c_mem.wait()
    c_bx[0].wait()
    got_w(raw_o, 0, 12, 0)
    for t in range(24, NF, 6):
        get_w(O, t, 6, 1 if t < 30 else NB + 1)

    def tokens(s):
        return [bx[_ds(s, SEG), k * 128:(k + 1) * 128].astype(F32) for k in range(LT)]

    def project_group(odd, g, product, nm):
        pa, pb = (g.ws, g.us) if odd else (g.us, g.ws)
        half, same, cross = slice(HALF * odd, HALF * odd + HALF), {}, {}

        def with_memory(x, k):
            return _cat([x, f_one[odd, k, SEG:SEG + nm]])

        def prod(lhs, *name):
            return product.now(lhs, weight(g, name))

        def direct(c):
            for _, k in [x for x in g.direct if x[0] == c]:
                r = prod(lambda: f_one[odd, k, 0:SEG + nm], "cell", c, k)
                same[c] = list(map(_add, same[c], r))

        def other(a):
            return cols1.at[g.j, a, M:L] if odd else part.at[place(g.j, a), a % 10]

        def mixed(a, b, r):
            cross[a] = list(map(_add, cross.get(a) or _vregs(other(a)[half]), r))
            for x, h in zip(r, (2 * odd, 2 * odd + 1, *range(4, 9))):
                same[b][h] = same[b][h] + x

        def save_cross(a):
            other(a)[half] = _cat(cross.pop(a))

        def save(c, more=None):
            cols[odd][g.j, c, 0:nm] = _cat(same[c][4:])
            cols[1 - odd][g.j, c, M:L] = _add(more, _cat(same[c][:4]))
        for some in (pb[:-2], pb[-2:]):
            for b, j in some:
                same[b] = list(prod(lambda: with_memory(f_dif[odd, j], j), "+", b))
                direct(b)
            for a, i in pa:
                if a not in same:
                    same[a] = prod(lambda: f_one[odd, i, 0:SEG + nm], "-", a)
                    x = _add(other(a)[...] if odd else None, _cat(same[a][:4]))
                    other(a)[HALF - half.start:SEG - half.start] = x[HALF - half.start:SEG - half.start]
                    cross[a] = _vregs(x[half])
                    direct(a)
                else:
                    same[a] = _vregs(cols[1 - odd][g.j, a, M:L]) + _vregs(cols[odd][g.j, a, 0:nm])
                for b, j in some:
                    if i != j:
                        product.tick()
                        product.soon(with_memory(f_mix[odd, MIXES.index((i, j))], i),
                                     weight(g, ("both", b, a) if odd else ("both", a, b)),
                                     functools.partial(mixed, a, b))
                for b, j in some:
                    if i != j:
                        r = prod(lambda: f_sum[odd, SUMS.index((min(i, j), max(i, j))), 0:SEG + nm], "cell", a, j)
                        same[a] = list(map(_add, same[a], r))
                        same[b] = list(map(_sub, same[b], r))
                save(a)
                product.after(HALF + nm, functools.partial(save_cross, a))
            for b, _ in some:
                product.after(HALF + nm, functools.partial(save, b, part[place(g.j, b), b % 10] if odd else None))

    def project_last(g, product):
        def use(u, k, r):
            cols1[g.j, u, 0:M] = r[0] + cols1[g.j, u, 0:M] if k else r[0]
        for (u, _), (w, _) in zip(g.us, g.ws):
            r = [None] * 5
            for k in range(LT):
                product.tick()
                if g.j != Q:
                    product.soon(f_one[1, k, SEG:L], weight(g, ("cell", u, k)), functools.partial(use, u, k))
                r = list(map(_add, r, product.now(lambda: f_one[1, k, 0:L], weight(g, ("cell", w, k)))))
            cols1[g.j, w] = _cat(r[4:] + r[:4])

    def out_groups(odd, gs, same, cross, product, last):
        h0, nh = (0, SEG * odd) if last else (2 - 2 * odd, HALF)
        mix = {}

        def xa(c, r0=0, n=SEG):
            return att[c, M + SEG * (1 - odd) + r0:M + SEG * (1 - odd) + r0 + n]

        def xb(c, r0=0, n=SEG):
            return att[c, L + r0:L + r0 + n] if odd else keep[c, r0:r0 + n]

        def xm(c):
            return att[c, 0:M]

        def prod(g, m, x, *name):
            r = product.now(lambda: x() if last else _cat([m(), x()]), weight(g, name))
            return r if last else r[1:] + r[:1]

        def mixed(s, t, r):
            mix[s, t] = list(map(_add, mix.get((s, t), [None] * 4), r))

        def spend(s, t):
            for x, h in zip(mix.pop((s, t), []), list(range(h0, h0 + nh // 8)) + [4]):
                same[t][h] = _add(same[t][h], x)
                if h < 4:
                    cross[s][h] = _add(cross[s][h], x)
        sides = [(g, {d: c for c, d in (g.us if odd else g.ws)}, {d: c for c, d in (g.ws if odd else g.us)})
                 for g in gs]
        for i in range(LT):
            shared = [None] * 5
            for g, pa, pb in sides:
                rs = [prod(g, lambda: xm(pb[i]), lambda: xa(pb[i]) - xb(pb[i]), "+", pb[i])] if i in pb else []
                rs += [prod(g, lambda: xm(c), lambda: xa(c), "cell", c, k) for c, k in g.direct if k == i]
                for r in rs:
                    same[i] = list(map(_add, same[i], r))
                if i in pa:
                    shared = list(map(_add, shared, prod(g, lambda: xm(pa[i]), lambda: xa(pa[i]), "-", pa[i])))
                    if odd:
                        keep[pa[i]] = xa(pa[i])
            same[i] = list(map(_add, same[i], shared))
            cross[i] = list(map(_add, cross[i], shared))
            for j in range(i + 1, LT):
                diff = [None] * 5
                for s, t in ((i, j), (j, i)):
                    for g, pa, pb in sides:
                        if s in pa and t in pb:
                            a, b = pa[s], pb[t]
                            if nh:
                                product.tick()
                                x = xa(a, 8 * h0, nh) + xb(b, 8 * h0, nh)
                                product.soon(x if last else _cat([x, xm(a)]),
                                             weight(g, ("both", a, b) if odd else ("both", b, a)),
                                             functools.partial(mixed, s, t))
                            r = prod(g, lambda: xm(a) + xm(b), lambda: xa(a) + xa(b), "cell", b, s)
                            diff = list(map(_add if s == i else _sub, diff, r))
                    product.after(nh if last else nh + M, functools.partial(spend, s, t))
                same[i] = list(map(_add, same[i], diff))
                same[j] = list(map(_sub, same[j], diff))

    def project_out(odd, s, product, last=False):
        same, cross = [[None] * 5 for _ in range(LT)], [[None] * 4 for _ in range(LT)]
        for gs in (GO[:3], GO[3:]):
            assert gs[0] is GO[0] or not product.events
            out_groups(odd, gs, same, cross, product, last)
        product.passed(0, True)
        for k in range(LT):
            lanes = slice(k * 128, (k + 1) * 128)
            if odd:
                out_x[k], out_y[k] = _cat(same[k][:4]), _cat(cross[k])
            else:
                outb[_ds(s - 2, SEG), lanes] = (out_x[k] + _cat(cross[k])).astype(BF16)
                outb[_ds(s - 1, SEG), lanes] = (out_y[k] + _cat(same[k][:4])).astype(BF16)
        return [x[-1] for x in same]

    def attend(odd, s, m, product, last=False):
        xa, xb = tokens(jnp.minimum(s + 1, NSEG - 1)), tokens(s if odd else jnp.minimum(s + 2, NSEG - 1))
        nm = m[0].shape[0]
        for k in range(LT):
            f_one[odd, k, 0:SEG + m[k].shape[0]] = _cat([xa[k], m[k]])
            f_dif[odd, k] = xa[k] - xb[k]
        for n, (i, j) in enumerate(SUMS):
            f_sum[odd, n, 0:SEG + nm] = _cat([xa[i] + xa[j], m[i] + m[j]])
        for n, (i, j) in enumerate(MIXES):
            f_mix[odd, n] = (xa[i] + xb[j])[HALF * odd:HALF * odd + HALF]

        lane = lax.broadcasted_iota(jnp.int32, (L, 128), 1)
        zone = [(lane >= L * z) & (lane < L * z + L) for z in range(3)]
        some = [(lane >= 24 + 16 * n) & (lane < 40 + 16 * n) for n in range(2)]

        def tile(j, g, n, z):
            return cols[odd][j, 6 * g + TILE[n][z]]

        def gathered(j, g, n):
            x = jnp.where(zone[2], tile(j, g, n, 2), 0.0) if j == K else tile(j, g, n, 2)
            return jnp.where(zone[0], tile(j, g, n, 0), jnp.where(zone[1], tile(j, g, n, 1), x))

        def stack(xs):
            return _cat(xs + [jnp.zeros((8, 128), F32)])

        def by_head(x, a, of_a):
            xs = [jnp.zeros((L, 128), F32)] * 2 + [x]
            if a < 2:
                xs[a], xs[2] = jnp.where(of_a, x, 0.0), jnp.where(of_a, 0.0, x)
            return stack(xs)

        def turned(slot, x):
            keys[slot] = x.T
            return keys[slot]

        def one_pass(x, w):
            r = _dot(x, w.astype(BF16))
            product.passed(1)
            return _cat(_vregs(r))

        def done(g, n, z, o):
            att[6 * g + TILE[n][z], 0:M] = o[0:M]
            att[6 * g + TILE[n][z], M + SEG * odd:L + SEG * odd] = o[M:L]

        def alone(j, g):
            sc = {}
            for z in (2, 1, 0):
                for n in range(2):
                    w = by_head(tile(j, g, n, z), z, ~zone[z] | some[n] if z == n else ~zone[z])
                    if j == V:
                        p = hold[g, 2 + n] if z in (2, n) else jnp.where(zone[2], hold[g, 2 + n], hold[g, 2 + z])
                        done(g, n, z, one_pass(p, w))
                        continue
                    r = one_pass(tile(Q, g, n, z), turned(3 * n + z, w))
                    if z in (2, n):
                        sc[n] = _add(sc.get(n), r)
                    else:
                        sc[n], sc[z] = sc[n] + jnp.where(zone[2], r, 0.0), sc[z] + jnp.where(zone[2], 0.0, r)
            for n in sc:
                hold[g, n] = sc[n]

        def zone_scores(g):
            for n in range(2):
                turned(4 * g + 2 + n, stack([tile(K, g, n, z) for z in range(3)]))
            for n in range(2):
                hold[g, n] = one_pass(gathered(Q, g, n), turned(4 * g + 4 + n, by_head(gathered(K, g, n), n, some[n])))

        def together(g):
            for n in range(2):
                hold[g - 1, 4 + n] = one_pass(hold[g - 1, 2 + n], by_head(gathered(V, g - 1, n), n, some[n]))
                for z in range(3):
                    h = n if z == 2 else z
                    w = [jnp.where(zone[z][0:8], y, 0.0) for y in _vregs(keys[4 * g + 2 + n])]
                    w[5 * z:5 * z + 5] = [jnp.where(zone[z], 0.0, tile(V, g - 1, n, z))]
                    r = one_pass(jnp.where(zone[z], hold[g - 1, 2 + h], tile(Q, g, n, z)), _cat(w))
                    hold[g, h] = hold[g, h] + jnp.where(zone[z], r, 0.0)
                    done(g - 1, n, z, jnp.where(zone[z], hold[g - 1, 4 + n], r))

        def softmax(g):
            ahead = lane[0:8] % L - lax.broadcasted_iota(jnp.int32, (8, 128), 0)
            for n in range(2):
                x = _cat([jnp.where(ahead <= 8 * b, y, MASKED * DH ** 0.5) if b else y
                          for b, y in enumerate(_vregs(hold[g, n]))])
                top = [jnp.max(jnp.where(zone[z], x, -jnp.inf), axis=1, keepdims=True) for z in (n, 2)]
                e = jnp.exp2((x - jnp.where(zone[2], top[1], top[0])) * (DH ** -0.5 * LOG2E))
                e = [jnp.where(zone[z], e, 0.0) for z in (n, 2)]
                total = [jnp.sum(y, axis=1, keepdims=True) for y in e]
                hold[g, 2 + n] = (e[0] + e[1]) * _recip(jnp.where(zone[2], total[1], total[0]))

        def complete(j, g):
            n = max(n for n, x in enumerate(GQ) if x.j == j and x.first < 6 * g + 6)
            return sum(LT * len(x.us + x.ws) for x in GQ[:n + 1])

        def at(t, f, *args):
            product.events.setdefault(t, []).append(functools.partial(f, *args))
        t = complete(Q, 0) + 48
        at(t, alone, K, 0)
        at(t, softmax, 0)
        for g in range(1, NG):
            t = max(t + 78, complete(Q, g) + (80 if last else 70 if nm == M else 30), complete(V, g - 1) + 48) + (0, -6, 0, 0, 3, 3, 0, 0)[g]
            at(t - 0, zone_scores, g)
            at(t, together, g)
            at(t, softmax, g)
        at(t + 56, alone, V, NG - 1)
        for g in GQ:
            if last:
                project_last(g, product)
            else:
                project_group(odd, g, product, nm)
        return product

    first = _Products({}, tied)

    def spread(tasks, t0, t1, src=None, dst=None):
        def run(some):
            if src is None or len(first.results) < 13:
                _run(some)
            else:
                paced(some, src, first.results[-13])
            if dst is not None:
                tie(dst)
        for t in range(t0, t1):
            if _share(tasks, t - t0, t1 - t0):
                first.events.setdefault(t, []).append(functools.partial(run, _share(tasks, t - t0, t1 - t0)))

    def a_last(c, k):
        def use(r):
            x = _cat(list(map(_add, _vregs(tmp[c, 0:TB]), r)) if k else r)
            if k < LT - 1:
                tmp[c, 0:TB] = x
            else:
                outa[S - TB:S, c * 128:(c + 1) * 128] = x.astype(BF16)
        first.soon(oa1[k], wo_p.at[k * 64:(k + 1) * 64, c * 128:(c + 1) * 128], use)

    def wo_wait(t, batch):
        got_w(raw_o, t, 18, batch)
    end = 3 * NF * LT
    spread(a_attention(1), 12, 150, qkv1, oa1)
    spread(w_turn(_Group(V, 40)), 150, 150 + 1)
    spread(w_combine(_Group(Q, 40)), 150, 220, cells1, sums2)
    spread(w_combine(GO[0]), 220, 325, raw_o, sums_o)
    spread([lambda: tie(cells2)], 325 - 20, 325 - 19)
    spread(w_combine(_Group(V, 40)), 325, 390, cells2, sums2)
    spread([lambda: wo_wait(12, 1), c_bx[1].start], 390, 390 + 1)
    spread(w_combine(GO[1]) + w_combine(GO[2]), 390 + 6, 590, raw_o, sums_o)
    spread([lambda: wo_wait(30, NB + 1)], 590, 590 + 1)
    spread(w_combine(GO[3]) + w_combine(GO[4]), 590 + 6, end + 30, raw_o, sums_o)
    spread([functools.partial(a_last, c, k) for k in range(LT) for c in range(LT)], end, end + LT * NF)
    attend(0, 0, [_cat([mem[:, k * 128:(k + 1) * 128].astype(F32), x]) for k, x in enumerate(tokens(0))], first)
    first.passed(0, True)
    m = [None] * LT
    for c in range(NF):
        for k in range(LT):
            m[k] = _add(m[k], first.now(lambda: att[c, 0:M], weight(GO[c // 10], ("cell", c, k)))[0])
    first.passed(0, True)
    for k in range(LT):
        mem_s[k] = m[k]
    c_out(0, pl.ds(0, S)).start()
    c_bx[1].wait()

    def b_step(n, carry):
        m = [mem_s[k] for k in range(LT)]
        for odd in (1, 0):
            m = project_out(odd, 2 * n + 2 - odd, attend(odd, 2 * n + 2 - odd, m, _Products({}, tied)))
        for k in range(LT):
            mem_s[k] = m[k]
        c_out(1, _ds(n, 2 * SEG)).start()
        return carry

    lax.fori_loop(0, NSEG // 2 - 1, b_step, 0)
    final = attend(1, NSEG - 1, [mem_s[k] for k in range(LT)], _Products({}, tied), last=True)
    project_out(1, NSEG - 1, final, last=True)
    project_out(0, NSEG, final, last=True)
    c_out(1, _ds(NSEG // 2 - 1, 2 * SEG)).start()
    for j in range(2):
        c_out(j, pl.ds(0, S)).wait()


def pallas_concat_heads__sliding_local_dilated__memory_aug_recurrent_mem_tr__prompt_kernel(
    A_x, A_wqkv, A_wo, B_x, B_mem0, B_Wq, B_Wk, B_Wv, B_Wo, B_seg_len,
):
    assert B_seg_len == SEG
    assert A_x.shape == B_x.shape == (1, S, D) and B_mem0.shape == (1, M, D)
    assert B_Wq.shape == B_Wk.shape == B_Wv.shape == (D, H, DH) and B_Wo.shape == (H, DH, D)
    vmem, dma = pltpu.VMEM, pltpu.SemaphoreType.DMA
    call = pl.pallas_call(
        _kernel,
        out_shape=jax.ShapeDtypeStruct((S, 2 * D), BF16),
        in_specs=[pl.BlockSpec(memory_space=pl.ANY)] * 9,
        out_specs=pl.BlockSpec(memory_space=pl.ANY),
        scratch_shapes=[
            vmem((S, D), BF16),
            vmem((3, D, D), BF16),
            vmem((D, D), BF16),
            vmem((LT, D, 128), F32),
            vmem((3 * D // 2, D), U32),
            vmem((D // 2, D), U32),
            vmem((2, TB, D), F32),
            vmem((3 * LT + 1, HALO + TB, 128), F32), vmem((3 * LT + 1, HALO + TB, 128), F32),
            vmem((LT + 1, TB, 128), F32), vmem((LT + 1, TB, 128), F32),
            vmem((S, D), BF16),
            vmem((S, D), BF16),
            vmem((M, D), BF16),
            vmem((LT, 3 * NF * 128, 128), BF16),
            vmem((351, 64, 128), U32), vmem((351, 64, 128), U32), vmem((51, 64, 128), U32),
            vmem((LT + 1, NF * 128, 128), BF16),
            vmem((521, 128, 128), BF16), vmem((81, 128, 128), BF16), vmem((201, 128, 128), BF16),
            vmem((LT, M, 128), F32),
            vmem((2, LT, L + SEG, 128), F32),
            vmem((2, len(SUMS), L + SEG, 128), F32),
            vmem((2, LT, SEG, 128), F32),
            vmem((2, len(MIXES), HALF, 128), F32),
            vmem((3, NF, L, 128), F32), vmem((3, NF, L, 128), F32),
            vmem((len(GQ), LT, SEG, 128), F32),
            vmem((4 * NG + 2, 128, 128), F32),
            vmem((NG, 6, L, 128), F32),
            vmem((NF, L + SEG, 128), F32),
            vmem((NF, SEG, 128), F32),
            vmem((LT, SEG, 128), F32), vmem((LT, SEG, 128), F32),
            pltpu.SMEM((30 * len(GQ),), jnp.int32),
            dma((7,)), dma((NB,)), dma((NB + 2,)), dma((2,)),
        ],
        compiler_params=pltpu.CompilerParams(
            vmem_limit_bytes=124 * 1024 * 1024, disable_bounds_checks=True, disable_semaphore_checks=True),
        name="sliding_and_memory_attention",
    )

    def by_feature(w):
        return w.transpose(1, 2, 0).reshape(H * DH, D)

    out = call(A_x.reshape(S, D), A_wqkv, A_wo, B_x.reshape(S, D), B_mem0.reshape(M, D),
               by_feature(B_Wq), by_feature(B_Wk), by_feature(B_Wv), B_Wo.reshape(H * DH, D))
    return out.reshape(1, S, 2 * D)
```

```python
import functools

import jax
import jax.numpy as jnp
from jax import lax
from jax.experimental import pallas as pl
from jax.experimental.pallas import tpu as pltpu

F32, BF16, U32 = jnp.float32, jnp.bfloat16, jnp.uint32
NT = (((1,), (1,)), ((), ()))
MASKED = -1000000000.0
LOG2E = 1.4426950408889634

S, D = 2048, 640
LT = D // 128

AH, AD, AW, ADIL = 32, 20, 8, 2
HALO = 16
TB = 128
NB = S // TB

H, DH, M, SEG = 32, 192, 8, 32
L = M + SEG
HALF = SEG // 2
NSEG = S // SEG
NF = H * DH // 128
SUMS = [(i, j) for i in range(LT) for j in range(i + 1, LT)]
MIXES = [(i, j) for i in range(LT) for j in range(LT) if i != j]

NG = H // 4
TILE = ((1, 2, 0), (3, 4, 5))
PIECES = ((0, 40, 80), (168, 208, 248), (384, 128, 424), (600, 296, 336), (472, 560, 512), (640, 680, 720))
CUTS = (0, L, 2 * L, 128)


class _Group:
    def __init__(self, j, first):
        u_diag, w_diag = (range(LT), range(LT)) if first + 10 <= NF else (range(4), range(1, 5))
        self.j, self.first = j, first
        self.us = [(first + n, i) for n, i in enumerate(u_diag)]
        self.ws = [(first + len(u_diag) + n, j) for n, j in enumerate(w_diag)]
        self.pairs = [(u, i, w, j) for u, i in self.us for w, j in self.ws if i != j]
        paired = [(u, j) for u, i, w, j in self.pairs] + [(w, i) for u, i, w, j in self.pairs]
        self.direct = [(c, k) for c, d in self.us + self.ws for k in range(LT)
                       if k != d and (c, k) not in paired]
        self.seat = dict(self.us + [(w, LT + j) for w, j in self.ws])


K, Q, V, O = range(4)
GQ = [_Group(j, t) for t in (0, 10, 20) for j in (K, Q, V)]
GQ += [_Group(j, t) for j, t in ((K, 30), (Q, 30), (K, 40), (Q, 40), (V, 30), (V, 40))]
GO = [_Group(O, t) for t in range(0, NF, 10)]
TIMES = {"first": (148, 274, 352, 436, 510, 592, 729, 809, 860),
         "last": (125, 228, 325, 379, 452, 526, 605, 675, 735),
         1: (148, 314, 392, 470, 552, 636, 728, 799, 859),
         0: (138, 314, 390, 481, 551, 632, 728, 812, 863)}


def _first_row(j, c, n):
    return (j * NG + c // 6) * 96 + PIECES[c % 6][n] // 8


def _ds(i, n, size=None):
    return pl.ds(i * n if isinstance(i, int) else pl.multiple_of(i * n, n), size or n)


def _dot(a, b):
    return jnp.dot(a, b, preferred_element_type=F32)


def _recip(x):
    r = pl.reciprocal(x, approx=True)
    return r * (2.0 - x * r)


def _add(a, b):
    return b if a is None else a + b


def _sub(a, b):
    return -b if a is None else a - b


def _total(xs):
    return functools.reduce(jnp.add, xs)


def _vregs(x):
    return [x[r:r + 8] for r in range(0, x.shape[0], 8)]


def _cat(xs):
    return jnp.concatenate(xs, axis=0)


def _share(tasks, k, n):
    return tasks[k * len(tasks) // n:(k + 1) * len(tasks) // n]


def _run(tasks):
    for task in tasks:
        task()


class _Products:
    def __init__(self, events, tied):
        self.events, self.tied, self.results, self.ready = events, tied, [], []
        self.count, self.usual, self.flushed, self.waiting = 0, 0, -1, {}

    def dot(self, x, w):
        self.results.append(_vregs(_dot(self.tied(x), pltpu.bitcast(w, BF16))))
        return self.results[-1]

    def tick(self):
        self.count += 1
        _run(self.events.pop(self.count - 1, []))

    def now(self, x, w):
        self.tick()
        r = self.dot(x(), w[...])
        self.passed(1)
        return r

    def soon(self, x, w, use):
        self.waiting.setdefault(x.shape[0], []).append([x, w[...], [use]])

    def after(self, rows, task):
        if self.waiting.get(rows):
            self.waiting[rows][-1][2].append(lambda r: task())
        else:
            task()

    def passed(self, n, last=False):
        self.usual += n
        for rows in sorted(self.waiting, reverse=True):
            queue = self.waiting[rows]
            while queue and (last or (len(queue) >= 4 and self.usual % 4 == 0
                                      and (self.flushed < self.usual or len(queue) >= 8 or rows >= L))):
                for x, w, uses in queue[:4]:
                    r = self.dot(x, w)
                    for use in uses:
                        use(r)
                del queue[:4]
                if rows < L:
                    self.flushed = self.usual


def _kernel(ax_hbm, awqkv_hbm, awo_hbm, bx_hbm, mem_hbm, wq_hbm, wk_hbm, wv_hbm, wo_hbm,
            out_hbm,
            ax, awqkv, awo, tmp, wqkv_p, wo_p, x_s, qkv0, qkv1, oa0, oa1, outa,
            bx, mem, raw, cells0, cells1, cells2, raw_o, sums, sums2, sums_o,
            mem_s, f_one, f_sum, f_dif, f_mix, cols0, cols1, part, keys, hold, att, keep, out_x, out_y,
            sources, sem_a, sem_x, sem_w, sem_o):
    qkv, oa, cols = (qkv0, qkv1), (oa0, oa1), (cols0, cols1)
    outb = ax

    cp = pltpu.make_async_copy
    c_wqkv = [cp(awqkv_hbm.at[:, pl.ds(j * D, D)], awqkv.at[j], sem_a.at[j]) for j in range(3)]
    c_awo = cp(awo_hbm, awo, sem_a.at[3])
    c_mem = cp(mem_hbm, mem, sem_a.at[4])
    c_bx = [cp(bx_hbm.at[rows], bx.at[rows], sem_a.at[5 + n])
            for n, rows in enumerate((pl.ds(0, 3 * SEG), pl.ds(3 * SEG, S - 3 * SEG)))]

    def c_ax(i):
        return cp(ax_hbm.at[_ds(i, TB)], ax.at[_ds(i, TB)], sem_x.at[i])

    def c_out(j, rows):
        return cp((outa, outb)[j].at[rows, :], out_hbm.at[rows, pl.ds(j * D, D)], sem_o.at[j])

    def get_w(j, t, n, batch):
        dst, first = (raw_o, t) if j == O else (raw, j * NF + t)
        for k in range(LT):
            cp((wk_hbm, wq_hbm, wv_hbm, wo_hbm)[j].at[_ds(t, 128, 128 * n), _ds(k, 128)],
               dst.at[k, _ds(first, 128, 128 * n)], sem_w.at[batch]).start()

    def got_w(dst, first, n, batch):
        box = dst.at[0:LT, _ds(first, 128, 128 * n)]
        cp(box, box, sem_w.at[batch]).wait()

    ties = []

    def spare(ref, n):
        return (ref.bitcast(U32) if ref.dtype == BF16 else ref).at[ref.shape[0] - 1 + zero, _ds(n, 8)]

    def paced(tasks, ref, results):
        for n, task in enumerate(tasks):
            spare(ref, 0)[...] = pltpu.bitcast(results[n * len(results) // len(tasks)], spare(ref, 0).dtype)
            task()

    def tie(ref):
        ties.append(spare(ref, 1))

    def tied(x):
        head = x[0:8, 0:128]
        while ties:
            ref = ties.pop()
            ref[...] = pltpu.bitcast(head, ref.dtype)
            head = pltpu.bitcast(ref[...], x.dtype)
        if x.shape[1] > 128:
            head = jnp.concatenate([head, x[0:8, 128:]], axis=1)
        return _cat([head, x[8:]]) if x.shape[0] > 8 else head

    def permute_rows(dst, base):
        for d in range(AD):
            for t in range(LT):
                dst[pl.ds((base + d * AH) // 2, AH // 2), t * 128:(t + 1) * 128] = pltpu.bitcast(
                    tmp[t, pl.ds(d, AH, stride=AD), :].astype(BF16), U32)

    def prep_wqkv(j):
        for t in range(LT):
            tmp[t] = awqkv[j, t * 128:(t + 1) * 128, :].astype(F32).T
        permute_rows(wqkv_p, j * D)

    def prep_wo():
        for t in range(LT):
            tmp[t] = awo[:, t * 128:(t + 1) * 128].astype(F32)
        permute_rows(wo_p, 0)

    def a_pass(i, b, c, k0=0, k1=LT):
        lanes = slice(c % LT * 128, c % LT * 128 + 128)
        if c < 3 * LT:
            if c == k0 == 0:
                x_s[b] = ax[_ds(i, TB), :].astype(F32)
            w = pltpu.bitcast(wqkv_p[c * 64:(c + 1) * 64, k0 * 128:k1 * 128], BF16)
            r = lax.dot_general(tied(x_s[b, :, k0 * 128:k1 * 128]), w, NT, preferred_element_type=F32)
        else:
            x = jnp.concatenate([oa[1 - b][k] for k in range(k0, k1)], axis=1)
            r = _dot(tied(x), pltpu.bitcast(wo_p[k0 * 64:k1 * 64, lanes], BF16))
        if k0:
            r = _cat(list(map(_add, _vregs(tmp[c % 4, 0:TB]), _vregs(r))))
        if k1 < LT:
            tmp[c % 4, 0:TB] = r
        elif c >= 3 * LT:
            outa[_ds(i - 1, TB), lanes] = r.astype(BF16)
        else:
            qkv[b][c, HALO:] = r
            if c >= LT and isinstance(i, int) and i == 0:
                qkv[b][c, 0:HALO] = jnp.broadcast_to(r[0:1, :], (HALO, 128))
            elif c >= LT:
                qkv[b][c, 0:HALO] = qkv[1 - b][c, TB:]
        return _vregs(r)

    def a_attention(b, first_block=False):
        state = {}

        def window(c, r0, w):
            return qkv[b][c, HALO + r0 - ADIL * w:HALO + r0 - ADIL * w + 8]

        def logits(r0, ws):
            q = [window(t, r0, 0) for t in range(LT)]
            for w in ws:
                a = _total([q[t] * window(LT + t, r0, w) for t in range(LT)])
                a = _total([a] + [pltpu.roll(a, d, 1) for d in range(AH, 128, AH)])
                if first_block and r0 < ADIL * w:
                    pos = lax.broadcasted_iota(jnp.int32, (8, 128), 0) + r0
                    a = jnp.where(pos >= ADIL * w, a, MASKED * AD ** 0.5)
                state[r0, w] = a

        def mix(r0, ts):
            if ts[0] == 0:
                lg = [state.pop((r0, w)) for w in range(AW)]
                m = functools.reduce(jnp.maximum, lg)
                state[r0] = [jnp.exp2((a - m) * (AD ** -0.5 * LOG2E)) for a in lg]
                state[r0].append(_recip(_total(state[r0])))
            e = state[r0]
            for t in ts:
                oa[b][t, r0:r0 + 8] = _total([e[w] * window(2 * LT + t, r0, w) for w in range(AW)]) * e[AW]

        steps = [(0, logits, range(4)), (0, logits, range(4, AW)), (8, mix, range(1)), (8, mix, range(1, LT))]
        return [functools.partial(f, r0 - lag, some) for r0 in range(0, TB + 8, 8)
                for lag, f, some in steps if 0 <= r0 - lag < TB]

    def place(j, first):
        return first // 10 * 3 + j

    def stored(g, name, at=None, as_words=True):
        n = place(g.j, g.first)
        if name[0] == "cell":
            slot = LT * g.seat[name[1]] + name[2]
            if n == 14:
                return cells2.at[slot]
            return (cells0, cells1)[n % 2].at[50 * ((n if at is None else at) >> 1) + slot]
        ref, n = (sums_o, g.first // 10) if g.j == O else (sums2, n - 13) if n >= 13 else (sums, n)
        if name[0] == "both":
            slot = 20 + MIXES.index((g.seat[name[1]], g.seat[name[2]] - LT))
        else:
            slot = 10 * "-+".index(name[0]) + g.seat[name[1]]
        return (ref.bitcast(U32) if as_words else ref).at[40 * (n if at is None else at) + slot]

    def runs(ref, k, r0, r1, r2):
        ref = ref.bitcast(U32)
        if isinstance(r0, int) and r1 == r0 + L // 8:
            return ref[k, _ds(r0, 4, 64)]
        low = lax.broadcasted_iota(jnp.int32, (8, 128), 0) < 4
        x, y = ref[k, _ds(r0, 4, 24)], ref[k, _ds(r1 - 1, 4, 24)]
        return _cat([x[0:16], jnp.where(low, x[16:], y[0:8]), y[8:], ref[k, _ds(r2, 4, 24)]])

    def weight(g, name, at=None):
        if g.j == O and name[0] == "cell":
            return runs(raw_o, name[2], *[_first_row(0, name[1], n) for n in range(3)])
        return stored(g, name, at)

    def w_turn(g, at=None):
        def turn(c, k, *rows):
            stored(g, ("cell", c, k), at)[...] = pltpu.bitcast(pltpu.bitcast(runs(raw, k, *rows), BF16).T, U32)
        tasks = []
        for c, _ in g.us + g.ws:
            rows = [_first_row(g.j, c, n) if at is None else sources[30 * at + 3 * c + n] for n in range(3)]
            tasks += [functools.partial(turn, c, k, *rows) for k in range(LT)]
        return [functools.partial(_run, tasks[n:n + 2]) for n in range(0, len(tasks), 2)]

    def w_combine(g, at=None):
        minus, plus = {}, {}
        pairs = sorted(g.pairs, key=lambda p: p[3] // (0 if at is None else 3)) if (0 if at is None else 3) else g.pairs

        def get(r, c, k, optional=False):
            x = weight(g, ("cell", c, k), at)[r // 2:r // 2 + 8]
            return pltpu.bitcast(jnp.where(at < 12, x, 0) if optional else x, BF16).astype(F32)

        def put(r, x, *name):
            stored(g, name, at, as_words=False)[r:r + 16] = x.astype(BF16)

        def combine(r, pair):
            u, i, w, j = pair
            optional = at is not None and g.j == 0 and (i == LT - 1 or j == 0)
            x, y = get(r, u, j, optional), get(r, w, i, optional)
            put(r, x + y, "both", u, w)
            if g.j == O:
                x, y = y, x
            for c, d, own, other in ((u, i, x, y), (w, j, y, x)):
                mine = [p for p in pairs if c in (p[0], p[2])]
                if pair == mine[0]:
                    minus[c] = plus[c] = get(r, c, d)
                minus[c], plus[c] = minus[c] - own, plus[c] + other
                if pair == mine[-1]:
                    put(r, minus[c], "-", c)
                    put(r, plus[c], "+", c)
        return [functools.partial(combine, r, pair) for r in range(0, 128, 16) for pair in pairs]

    for c in (c_wqkv[0], c_ax(0), c_wqkv[1], c_ax(1)):
        c.start()

    def touch(i, carry):
        for ref in (x_s, f_one, f_sum, f_dif, f_mix, cols0, cols1, part, keys, hold, att, keep,
                    out_x, out_y, tmp, cells0, cells1, cells2, sums, sums2, sums_o):
            ref[(i,) + (0,) * (len(ref.shape) - 3) + (slice(0, 16),)] = jnp.zeros((16, ref.shape[-1]), ref.dtype)
        for ref in (wqkv_p, wo_p):
            ref[_ds(i, 8)] = jnp.zeros((8, D), U32)
        return i
    zero = lax.shift_right_logical(lax.fori_loop(0, 2, touch, 0), 16)

    for g in GQ:
        tiles = {seat: c for c, seat in g.seat.items()}
        for n in range(30):
            sources[30 * place(g.j, g.first) + n] = _first_row(g.j, tiles.get(n // 3, g.first), n % 3)

    c_wqkv[0].wait()
    c_wqkv[2].start()
    prep_wqkv(0)
    c_ax(0).wait()
    for c in range(LT):
        a_pass(0, 0, c)
    c_wqkv[1].wait()
    c_ax(1).wait()
    c_awo.start()
    c_ax(2).start()
    prep_wqkv(1)
    for c in range(LT):
        a_pass(1, 1, c)
    c_wqkv[2].wait()
    get_w(K, 0, 6, 2)
    get_w(K, 6, 5, 2)
    prep_wqkv(2)
    for n in range(2 * LT):
        a_pass(n // LT, n // LT, LT + n % LT)
    c_awo.wait()
    get_w(Q, 0, 6, 3)
    get_w(Q, 6, 5, 3)
    get_w(V, 0, 1, 4)
    for c in (c_ax(3), c_mem, c_bx[0]):
        c.start()
    prep_wo()
    for n in range(2 * LT):
        a_pass(n // LT, n // LT, 2 * LT + n % LT)
    _run(a_attention(0, True))
    for c in range(LT):
        a_pass(1, 1, 3 * LT + c)

    def a_step(it, carry):
        for b in range(2):
            i = 2 * it + b
            third = (i * 43 - 86) >> 7
            t = (i - 2 - 3 * third) * NF + 10 * third
            pl.when(i < 5)(functools.partial(got_w, raw, t, 1, i))
            pl.when(i < 14)(functools.partial(got_w, raw, t + 8, 3, i))
            got_w(raw, t + 1, 7, i)
            c_ax(i).wait()
            third = (i * 43) >> 7
            for j in range(3):
                for t, n, needed in ((1, 7, i < 15), (8, 3, i < 12)):
                    pl.when(needed & (i - 3 * third == j))(functools.partial(get_w, j, 10 * third + t, n, i + 2))
            pl.when(it < NB // 2 - 1)(lambda: c_ax(i + 2).start())
            if b:
                pl.when(i > 12)(lambda: get_w(O, 6 * (i - 13), 6, it - 6))
                pl.when(i == 15)(lambda: get_w(O, 18, 6, 1))
            else:
                pl.when(i == 14)(lambda: get_w(O, 6, 6, 0))
            combine = w_combine(_Group(1 - b, 0), jnp.where(i < 3, 11, i - 3))
            side = [(a_attention(1 - b), 0, 17, 3, qkv[1 - b], oa[1 - b]),
                    (w_turn(_Group(b, 0), i - 2), 22, 5 * LT, 99, raw, (cells0, cells1)[b]),
                    (combine[:90], 0, 17, 2, (cells1, cells0)[b], sums),
                    (combine[90:], 17, 25, 2, (cells1, cells0)[b], sums)]
            rs = []
            for c in range(5 * LT):
                if c % 5 < 4:
                    rs.append(a_pass(i, b, c - c // 5, 0, 4))
                else:
                    rs.append([a_pass(i, b, c // 5 * 4 + n, 4, LT) for n in range(4)][0])
                for tasks, c0, c1, lag, src, dst in side:
                    if c0 <= c < c1:
                        if len(rs) < lag:
                            _run(_share(tasks, c - c0, c1 - c0))
                        else:
                            paced(_share(tasks, c - c0, c1 - c0), src, rs[-lag])
                        tie(dst)
            ties.clear()
        return carry

    lax.fori_loop(1, NB // 2, a_step, 0)
    got_w(raw, V * NF + 41, 7, NB)
    c_mem.wait()
    c_bx[0].wait()
    got_w(raw_o, 0, 12, 0)
    for t in range(24, NF, 6):
        get_w(O, t, 6, 1 if t < 30 else NB + 1)

    def tokens(s):
        return [bx[_ds(s, SEG), k * 128:(k + 1) * 128].astype(F32) for k in range(LT)]

    def project_group(odd, g, product, nm):
        pa, pb = (g.ws, g.us) if odd else (g.us, g.ws)
        half, same, cross = slice(HALF * odd, HALF * odd + HALF), {}, {}

        def with_memory(x, k):
            return _cat([x, f_one[odd, k, SEG:SEG + nm]])

        def prod(lhs, *name):
            return product.now(lhs, weight(g, name))

        def direct(c):
            for _, k in [x for x in g.direct if x[0] == c]:
                r = prod(lambda: f_one[odd, k, 0:SEG + nm], "cell", c, k)
                same[c] = list(map(_add, same[c], r))

        def other(a):
            return cols1.at[g.j, a, M:L] if odd else part.at[place(g.j, a), a % 10]

        def mixed(a, b, r):
            cross[a] = list(map(_add, cross[a] if a in cross else _vregs(other(a)[half]), r))
            for x, h in zip(r, (2 * odd, 2 * odd + 1, *range(4, 9))):
                same[b][h] = same[b][h] + x

        def save_cross(a):
            other(a)[half] = _cat(cross.pop(a))

        def save(c, more=None):
            cols[odd][g.j, c, 0:nm] = _cat(same[c][4:])
            cols[1 - odd][g.j, c, M:L] = _add(more, _cat(same[c][:4]))
        for some in (pb[:-2], pb[-2:]):
            for b, j in some:
                same[b] = list(prod(lambda: with_memory(f_dif[odd, j], j), "+", b))
                direct(b)
            for a, i in pa:
                if a not in same:
                    same[a] = prod(lambda: f_one[odd, i, 0:SEG + nm], "-", a)
                    x = _add(other(a)[...] if odd else None, _cat(same[a][:4]))
                    other(a)[HALF - half.start:SEG - half.start] = x[HALF - half.start:SEG - half.start]
                    cross[a] = _vregs(x[half])
                    direct(a)
                else:
                    same[a] = _vregs(cols[1 - odd][g.j, a, M:L]) + _vregs(cols[odd][g.j, a, 0:nm])
                for b, j in some:
                    if i != j:
                        product.tick()
                        product.soon(with_memory(f_mix[odd, MIXES.index((i, j))], i),
                                     weight(g, ("both", b, a) if odd else ("both", a, b)),
                                     functools.partial(mixed, a, b))
                for b, j in some:
                    if i != j:
                        r = prod(lambda: f_sum[odd, SUMS.index((min(i, j), max(i, j))), 0:SEG + nm], "cell", a, j)
                        same[a] = list(map(_add, same[a], r))
                        same[b] = list(map(_sub, same[b], r))
                save(a)
                product.after(HALF + nm, functools.partial(save_cross, a))
            for b, _ in some:
                product.after(HALF + nm, functools.partial(save, b, part[place(g.j, b), b % 10] if odd else None))
        product.after(HALF + nm, lambda: product.ready.extend((g.j, c) for c in g.seat))

    def last_queries(g, product):
        product.passed(0, True)
        for w, i in g.ws:
            r = list(map(_add, _vregs(cols1[Q, w, M:L]), product.now(lambda: f_one[1, i, 0:SEG], weight(g, ("-", w)))))
            for u, j in g.us:
                if i != j:
                    x = product.now(lambda: f_mix[1, MIXES.index((i, j))], weight(g, ("both", u, w)))
                    r[2:] = list(map(_add, r[2:], x))
            cols1[Q, w, M:L] = _cat(r)
        product.ready += [(Q, c) for c in g.seat]

    def out_groups(odd, gs, same, cross, product, last):
        h0, nh = (0, SEG * odd) if last else (2 - 2 * odd, HALF)
        mix = {}

        def xa(c, r0=0, n=SEG):
            return att[c, M + SEG * (1 - odd) + r0:M + SEG * (1 - odd) + r0 + n]

        def xb(c, r0=0, n=SEG):
            return att[c, L + r0:L + r0 + n] if odd else keep[c, r0:r0 + n]

        def xm(c):
            return att[c, 0:M]

        def prod(g, m, x, *name):
            r = product.now(lambda: x() if last else _cat([m(), x()]), weight(g, name))
            return r if last else r[1:] + r[:1]

        def mixed(s, t, r):
            mix[s, t] = list(map(_add, mix.get((s, t), [None] * 4), r))

        def spend(s, t):
            for x, h in zip(mix.pop((s, t), []), list(range(h0, h0 + nh // 8)) + [4]):
                same[t][h] = _add(same[t][h], x)
                if h < 4:
                    cross[s][h] = _add(cross[s][h], x)
        sides = [(g, {d: c for c, d in (g.us if odd else g.ws)}, {d: c for c, d in (g.ws if odd else g.us)})
                 for g in gs]
        for i in range(LT):
            shared = [None] * 5
            for g, pa, pb in sides:
                rs = [prod(g, lambda: xm(pb[i]), lambda: xa(pb[i]) - xb(pb[i]), "+", pb[i])] if i in pb else []
                rs += [prod(g, lambda: xm(c), lambda: xa(c), "cell", c, k) for c, k in g.direct if k == i]
                for r in rs:
                    same[i] = list(map(_add, same[i], r))
                if i in pa:
                    shared = list(map(_add, shared, prod(g, lambda: xm(pa[i]), lambda: xa(pa[i]), "-", pa[i])))
                    if odd:
                        keep[pa[i]] = xa(pa[i])
            same[i] = list(map(_add, same[i], shared))
            cross[i] = list(map(_add, cross[i], shared))
            for j in range(i + 1, LT):
                diff = [None] * 5
                for s, t in ((i, j), (j, i)):
                    for g, pa, pb in sides:
                        if s in pa and t in pb:
                            a, b = pa[s], pb[t]
                            if nh:
                                product.tick()
                                x = xa(a, 8 * h0, nh) + xb(b, 8 * h0, nh)
                                product.soon(x if last else _cat([x, xm(a)]),
                                             weight(g, ("both", a, b) if odd else ("both", b, a)),
                                             functools.partial(mixed, s, t))
                            r = prod(g, lambda: xm(a) + xm(b), lambda: xa(a) + xa(b), "cell", b, s)
                            diff = list(map(_add if s == i else _sub, diff, r))
                    product.after(nh if last else nh + M, functools.partial(spend, s, t))
                same[i] = list(map(_add, same[i], diff))
                same[j] = list(map(_sub, same[j], diff))

    def project_out(odd, s, product, last=False):
        same, cross = [[None] * 5 for _ in range(LT)], [[None] * 4 for _ in range(LT)]
        for gs in (GO[:3], GO[3:]):
            assert all((O, c) in product.ready for g in gs for c in g.seat)
            out_groups(odd, gs, same, cross, product, last)
        product.passed(0, True)
        for k in range(LT):
            lanes = slice(k * 128, (k + 1) * 128)
            if odd:
                out_x[k], out_y[k] = _cat(same[k][:4]), _cat(cross[k])
            else:
                outb[_ds(s - 2, SEG), lanes] = (out_x[k] + _cat(cross[k])).astype(BF16)
                outb[_ds(s - 1, SEG), lanes] = (out_y[k] + _cat(same[k][:4])).astype(BF16)
        return [x[-1] for x in same]

    def attend(odd, s, m, product, last=False):
        xa, xb = tokens(jnp.minimum(s + 1, NSEG - 1)), tokens(s if odd else jnp.minimum(s + 2, NSEG - 1))
        nm = m[0].shape[0]
        for k in range(LT):
            f_one[odd, k, 0:SEG + m[k].shape[0]] = _cat([xa[k], m[k]])
            f_dif[odd, k] = xa[k] - xb[k]
        for n, (i, j) in enumerate(SUMS):
            f_sum[odd, n, 0:SEG + nm] = _cat([xa[i] + xa[j], m[i] + m[j]])
        for n, (i, j) in enumerate(MIXES):
            f_mix[odd, n] = (xa[i] + xb[j])[HALF * odd:HALF * odd + HALF]

        lane = lax.broadcasted_iota(jnp.int32, (L, 128), 1)
        zone = [(lane >= L * z) & (lane < L * z + L) for z in range(3)]
        some = [(lane >= 24 + 16 * n) & (lane < 40 + 16 * n) for n in range(2)]

        def tile(j, g, n, z):
            assert (j, 6 * g + TILE[n][z]) in product.ready
            return cols[odd][j, 6 * g + TILE[n][z]]

        def gathered(j, g, n):
            x = jnp.where(zone[2], tile(j, g, n, 2), 0.0) if j == K else tile(j, g, n, 2)
            return jnp.where(zone[0], tile(j, g, n, 0), jnp.where(zone[1], tile(j, g, n, 1), x))

        def stack(xs):
            return _cat(xs + [jnp.zeros((8, 128), F32)])

        def by_head(x, a, of_a):
            xs = [jnp.zeros((L, 128), F32)] * 2 + [x]
            if a < 2:
                xs[a], xs[2] = jnp.where(of_a, x, 0.0), jnp.where(of_a, 0.0, x)
            return stack(xs)

        def turned(slot, x):
            keys[slot] = x.T
            return keys[slot]

        def one_pass(x, w):
            r = _dot(x, w.astype(BF16))
            product.passed(1)
            return _cat(_vregs(r))

        def done(g, n, z, o):
            product.ready.append((O, 6 * g + TILE[n][z]))
            att[6 * g + TILE[n][z], 0:M] = o[0:M]
            att[6 * g + TILE[n][z], M + SEG * odd:L + SEG * odd] = o[M:L]

        def alone(j, g):
            sc = {}
            for z in (2, 1, 0):
                for n in range(2):
                    w = by_head(tile(j, g, n, z), z, ~zone[z] | some[n] if z == n else ~zone[z])
                    if j == V:
                        p = hold[g, 2 + n] if z in (2, n) else jnp.where(zone[2], hold[g, 2 + n], hold[g, 2 + z])
                        done(g, n, z, one_pass(p, w))
                        continue
                    r = one_pass(tile(Q, g, n, z), turned(3 * n + z, w))
                    if z in (2, n):
                        sc[n] = _add(sc.get(n), r)
                    else:
                        sc[n], sc[z] = sc[n] + jnp.where(zone[2], r, 0.0), sc[z] + jnp.where(zone[2], 0.0, r)
            for n in sc:
                hold[g, n] = sc[n]

        def together(g):
            for n in range(2):
                turned(4 * g + 2 + n, stack([tile(K, g, n, z) for z in range(3)]))
            for n in range(2):
                hold[g, n] = one_pass(gathered(Q, g, n), turned(4 * g + 4 + n, by_head(gathered(K, g, n), n, some[n])))
            for n in range(2):
                hold[g - 1, 4 + n] = one_pass(hold[g - 1, 2 + n], by_head(gathered(V, g - 1, n), n, some[n]))
                for z in range(3):
                    h = n if z == 2 else z
                    w = [jnp.where(zone[z][0:8], y, 0.0) for y in _vregs(keys[4 * g + 2 + n])]
                    w[5 * z:5 * z + 5] = [jnp.where(zone[z], 0.0, tile(V, g - 1, n, z))]
                    r = one_pass(jnp.where(zone[z], hold[g - 1, 2 + h], tile(Q, g, n, z)), _cat(w))
                    hold[g, h] = hold[g, h] + jnp.where(zone[z], r, 0.0)
                    done(g - 1, n, z, jnp.where(zone[z], hold[g - 1, 4 + n], r))

        def softmax(g):
            ahead = lane[0:8] % L - lax.broadcasted_iota(jnp.int32, (8, 128), 0)
            for n in range(2):
                x = _cat([jnp.where(ahead <= 8 * b, y, MASKED * DH ** 0.5) if b else y
                          for b, y in enumerate(_vregs(hold[g, n]))])
                top = [jnp.max(jnp.where(zone[z], x, -jnp.inf), axis=1, keepdims=True) for z in (n, 2)]
                e = jnp.exp2((x - jnp.where(zone[2], top[1], top[0])) * (DH ** -0.5 * LOG2E))
                e = [jnp.where(zone[z], e, 0.0) for z in (n, 2)]
                total = [jnp.sum(y, axis=1, keepdims=True) for y in e]
                hold[g, 2 + n] = (e[0] + e[1]) * _recip(jnp.where(zone[2], total[1], total[0]))

        for g, t in enumerate(TIMES["last" if last else "first" if nm > M else odd]):
            tasks = [functools.partial(alone, V if g else K, max(g - 1, 0)) if g % NG == 0 else functools.partial(together, g)]
            product.events.setdefault(t, []).extend(tasks + [functools.partial(softmax, g)] * (g < NG))
        for g in GQ:
            if last and g.j == Q:
                last_queries(g, product)
            else:
                project_group(odd, g, product, nm)
        return product

    first = _Products({}, tied)

    def spread(tasks, t0, t1, src=None, dst=None):
        def run(some):
            if src is None or len(first.results) < 16:
                _run(some)
            else:
                paced(some, src, first.results[-16])
            if dst is not None:
                tie(dst)
        for t in range(t0, t1):
            if _share(tasks, t - t0, t1 - t0):
                first.events.setdefault(t, []).append(functools.partial(run, _share(tasks, t - t0, t1 - t0)))

    def a_last(c, k):
        def use(r):
            x = _cat(list(map(_add, _vregs(tmp[c, 0:TB]), r)) if k else r)
            if k < LT - 1:
                tmp[c, 0:TB] = x
            else:
                outa[S - TB:S, c * 128:(c + 1) * 128] = x.astype(BF16)
        first.soon(oa1[k], wo_p.at[k * 64:(k + 1) * 64, c * 128:(c + 1) * 128], use)

    def wo_wait(t, batch):
        got_w(raw_o, t, 18, batch)
    end = 3 * NF * LT
    spread(a_attention(1), 12, 138, qkv1, oa1)
    spread(w_turn(_Group(V, 40)), 138, 138 + 1)
    spread(w_combine(_Group(Q, 40)), 138, 215, cells1, sums2)
    spread(w_combine(GO[0]), 215, 285, raw_o, sums_o)
    spread([lambda: tie(cells2)], 285 - 20, 285 - 19)
    spread(w_combine(_Group(V, 40)), 285, 375, cells2, sums2)
    spread([lambda: wo_wait(12, 1), c_bx[1].start], 375, 375 + 1)
    spread(w_combine(GO[1]) + w_combine(GO[2]), 375 + 6, 560, raw_o, sums_o)
    spread([lambda: wo_wait(30, NB + 1)], 560, 560 + 1)
    spread(w_combine(GO[3]) + w_combine(GO[4]), 560 + 6, end + 32, raw_o, sums_o)
    spread([functools.partial(a_last, c, k) for k in range(LT) for c in range(LT)], end, end + LT * NF)
    attend(0, 0, [_cat([mem[:, k * 128:(k + 1) * 128].astype(F32), x]) for k, x in enumerate(tokens(0))], first)
    first.passed(0, True)
    m = [None] * LT
    for c in range(NF):
        assert (O, c) in first.ready
        for k in range(LT):
            m[k] = _add(m[k], first.now(lambda: att[c, 0:M], weight(GO[c // 10], ("cell", c, k)))[0])
    first.passed(0, True)
    for k in range(LT):
        mem_s[k] = m[k]
    c_out(0, pl.ds(0, S)).start()
    c_bx[1].wait()

    def b_step(n, carry):
        m = [mem_s[k] for k in range(LT)]
        for odd in (1, 0):
            m = project_out(odd, 2 * n + 2 - odd, attend(odd, 2 * n + 2 - odd, m, _Products({}, tied)))
        for k in range(LT):
            mem_s[k] = m[k]
        c_out(1, _ds(n, 2 * SEG)).start()
        return carry

    lax.fori_loop(0, NSEG // 2 - 1, b_step, 0)
    final = attend(1, NSEG - 1, [mem_s[k] for k in range(LT)], _Products({}, tied), last=True)
    final.passed(0, True)
    project_out(1, NSEG - 1, final, last=True)
    project_out(0, NSEG, final, last=True)
    c_out(1, _ds(NSEG // 2 - 1, 2 * SEG)).start()
    for j in range(2):
        c_out(j, pl.ds(0, S)).wait()


def pallas_concat_heads__sliding_local_dilated__memory_aug_recurrent_mem_tr__prompt_kernel(
    A_x, A_wqkv, A_wo, B_x, B_mem0, B_Wq, B_Wk, B_Wv, B_Wo, B_seg_len,
):
    assert B_seg_len == SEG
    assert A_x.shape == B_x.shape == (1, S, D) and B_mem0.shape == (1, M, D)
    assert B_Wq.shape == B_Wk.shape == B_Wv.shape == (D, H, DH) and B_Wo.shape == (H, DH, D)
    vmem, dma = pltpu.VMEM, pltpu.SemaphoreType.DMA
    call = pl.pallas_call(
        _kernel,
        out_shape=jax.ShapeDtypeStruct((S, 2 * D), BF16),
        in_specs=[pl.BlockSpec(memory_space=pl.ANY)] * 9,
        out_specs=pl.BlockSpec(memory_space=pl.ANY),
        scratch_shapes=[
            vmem((S, D), BF16),
            vmem((3, D, D), BF16),
            vmem((D, D), BF16),
            vmem((LT, D, 128), F32),
            vmem((3 * D // 2, D), U32),
            vmem((D // 2, D), U32),
            vmem((2, TB, D), F32),
            vmem((3 * LT + 1, HALO + TB, 128), F32), vmem((3 * LT + 1, HALO + TB, 128), F32),
            vmem((LT + 1, TB, 128), F32), vmem((LT + 1, TB, 128), F32),
            vmem((S, D), BF16),
            vmem((S, D), BF16),
            vmem((M, D), BF16),
            vmem((LT, 3 * NF * 128, 128), BF16),
            vmem((351, 64, 128), U32), vmem((351, 64, 128), U32), vmem((51, 64, 128), U32),
            vmem((LT + 1, NF * 128, 128), BF16),
            vmem((521, 128, 128), BF16), vmem((81, 128, 128), BF16), vmem((201, 128, 128), BF16),
            vmem((LT, M, 128), F32),
            vmem((2, LT, L + SEG, 128), F32),
            vmem((2, len(SUMS), L + SEG, 128), F32),
            vmem((2, LT, SEG, 128), F32),
            vmem((2, len(MIXES), HALF, 128), F32),
            vmem((3, NF, L, 128), F32), vmem((3, NF, L, 128), F32),
            vmem((len(GQ), LT, SEG, 128), F32),
            vmem((4 * NG + 2, 128, 128), F32),
            vmem((NG, 6, L, 128), F32),
            vmem((NF, L + SEG, 128), F32),
            vmem((NF, SEG, 128), F32),
            vmem((LT, SEG, 128), F32), vmem((LT, SEG, 128), F32),
            pltpu.SMEM((30 * len(GQ),), jnp.int32),
            dma((7,)), dma((NB,)), dma((NB + 2,)), dma((2,)),
        ],
        compiler_params=pltpu.CompilerParams(
            vmem_limit_bytes=124 * 1024 * 1024, disable_bounds_checks=True, disable_semaphore_checks=True),
        name="sliding_and_memory_attention",
    )

    def by_feature(w):
        return w.transpose(1, 2, 0).reshape(H * DH, D)

    out = call(A_x.reshape(S, D), A_wqkv, A_wo, B_x.reshape(S, D), B_mem0.reshape(M, D),
               by_feature(B_Wq), by_feature(B_Wk), by_feature(B_Wv), B_Wo.reshape(H * DH, D))
    return out.reshape(1, S, 2 * D)
```

```python
import functools

import jax
import jax.numpy as jnp
from jax import lax
from jax.experimental import pallas as pl
from jax.experimental.pallas import tpu as pltpu

F32, BF16, U32 = jnp.float32, jnp.bfloat16, jnp.uint32
NT = (((1,), (1,)), ((), ()))
MASKED = -1000000000.0
LOG2E = 1.4426950408889634

S, D = 2048, 640
LT = D // 128

AH, AD, AW, ADIL = 32, 20, 8, 2
HALO = 16
TB = 128
NB = S // TB

H, DH, M, SEG = 32, 192, 8, 32
L = M + SEG
HALF = SEG // 2
NSEG = S // SEG
NF = H * DH // 128
SUMS = [(i, j) for i in range(LT) for j in range(i + 1, LT)]
MIXES = [(i, j) for i in range(LT) for j in range(LT) if i != j]

NG = H // 4
TILE = ((1, 2, 0), (3, 4, 5))
PIECES = ((0, 40, 80), (168, 208, 248), (384, 128, 424), (600, 296, 336), (472, 560, 512), (640, 680, 720))


class _Group:
    def __init__(self, j, first):
        u_diag, w_diag = (range(LT), range(LT)) if first + 10 <= NF else (range(4), range(1, 5))
        self.j, self.first = j, first
        self.us = [(first + n, i) for n, i in enumerate(u_diag)]
        self.ws = [(first + len(u_diag) + n, j) for n, j in enumerate(w_diag)]
        self.pairs = [(u, i, w, j) for u, i in self.us for w, j in self.ws if i != j]
        paired = [(u, j) for u, i, w, j in self.pairs] + [(w, i) for u, i, w, j in self.pairs]
        self.direct = [(c, k) for c, d in self.us + self.ws for k in range(LT)
                       if k != d and (c, k) not in paired]
        self.seat = dict(self.us + [(w, LT + j) for w, j in self.ws])


K, Q, V, O = range(4)
GQ = [_Group(j, t) for t in (0, 10, 20) for j in (K, Q, V)]
GQ += [_Group(j, t) for j, t in ((K, 30), (Q, 30), (K, 40), (Q, 40), (V, 30), (V, 40))]
GO = [_Group(O, t) for t in range(0, NF, 10)]
TIMES = {"first": (148, 274, 352, 436, 510, 592, 729, 809, 860),
         "last": (125, 228, 325, 379, 452, 526, 605, 675, 735),
         1: (148, 314, 392, 470, 552, 636, 728, 799, 859),
         0: (138, 314, 390, 481, 551, 632, 728, 812, 863)}


def _first_row(j, c, n):
    return (j * NG + c // 6) * 96 + PIECES[c % 6][n] // 8


def _ds(i, n, size=None):
    return pl.ds(i * n if isinstance(i, int) else pl.multiple_of(i * n, n), size or n)


def _dot(a, b):
    return jnp.dot(a, b, preferred_element_type=F32)


def _recip(x):
    r = pl.reciprocal(x, approx=True)
    return r * (2.0 - x * r)


def _add(a, b):
    return b if a is None else a + b


def _sub(a, b):
    return -b if a is None else a - b


def _total(xs):
    return functools.reduce(jnp.add, xs)


def _vregs(x):
    return [x[r:r + 8] for r in range(0, x.shape[0], 8)]


def _cat(xs):
    return jnp.concatenate(xs, axis=0)


def _share(tasks, k, n):
    return tasks[k * len(tasks) // n:(k + 1) * len(tasks) // n]


def _run(tasks):
    for task in tasks:
        task()


class _Products:
    def __init__(self, events, tied):
        self.events, self.tied, self.results, self.ready = events, tied, [], []
        self.count, self.usual, self.flushed, self.waiting = 0, 0, -1, {}

    def dot(self, x, w):
        self.results.append(_vregs(_dot(self.tied(x), pltpu.bitcast(w, BF16) if w.dtype == U32 else w)))
        return self.results[-1]

    def tick(self):
        self.count += 1
        _run(self.events.pop(self.count - 1, []))

    def now(self, x, w):
        self.tick()
        r = self.dot(x(), w[...])
        self.passed(1)
        return r

    def soon(self, x, w, use):
        self.waiting.setdefault(x.shape[0], []).append([x, w[...], [use]])

    def after(self, rows, task):
        if self.waiting.get(rows):
            self.waiting[rows][-1][2].append(lambda r: task())
        else:
            task()

    def passed(self, n, last=False):
        self.usual += n
        for rows in sorted(self.waiting, reverse=True):
            queue = self.waiting[rows]
            while queue and (last or (len(queue) >= 4 and self.usual % 4 == 0
                                      and (self.flushed < self.usual or len(queue) >= 8 or rows >= L))):
                for x, w, uses in queue[:4]:
                    r = self.dot(x, w)
                    for use in uses:
                        use(r)
                del queue[:4]
                if rows < L:
                    self.flushed = self.usual


def _kernel(ax_hbm, awqkv_hbm, awo_hbm, bx_hbm, mem_hbm, wq_hbm, wk_hbm, wv_hbm, wo_hbm,
            out_hbm,
            ax, awqkv, awo, tmp, wqkv_p, wo_p, x_s, qkv0, qkv1, oa0, oa1, outa,
            bx, mem, raw, cells0, cells1, cells2, raw_o, sums, sums2, sums_o,
            mem_s, f_one, f_sum, f_dif, f_mix, cols0, cols1, part, keys, hold, att, keep, out_x, out_y,
            sources, sem_a, sem_x, sem_w, sem_o):
    qkv, oa, cols = (qkv0, qkv1), (oa0, oa1), (cols0, cols1)
    outb = ax

    cp = pltpu.make_async_copy
    c_wqkv = [cp(awqkv_hbm.at[:, pl.ds(j * D, D)], awqkv.at[j], sem_a.at[j]) for j in range(3)]
    c_awo = cp(awo_hbm, awo, sem_a.at[3])
    c_mem = cp(mem_hbm, mem, sem_a.at[4])
    c_bx = [cp(bx_hbm.at[rows], bx.at[rows], sem_a.at[5 + n])
            for n, rows in enumerate((pl.ds(0, 3 * SEG), pl.ds(3 * SEG, S - 3 * SEG)))]

    def c_ax(i):
        return cp(ax_hbm.at[_ds(i, TB)], ax.at[_ds(i, TB)], sem_x.at[i])

    def c_out(j, rows):
        return cp((outa, outb)[j].at[rows, :], out_hbm.at[rows, pl.ds(j * D, D)], sem_o.at[j])

    def get_w(j, t, n, batch):
        dst, first = (raw_o, t) if j == O else (raw, j * NF + t)
        for k in range(LT):
            cp((wk_hbm, wq_hbm, wv_hbm, wo_hbm)[j].at[_ds(t, 128, 128 * n), _ds(k, 128)],
               dst.at[k, _ds(first, 128, 128 * n)], sem_w.at[batch]).start()

    def got_w(dst, first, n, batch):
        box = dst.at[0:LT, _ds(first, 128, 128 * n)]
        cp(box, box, sem_w.at[batch]).wait()

    ties = []

    def spare(ref, n):
        return ref.at[ref.shape[0] - 1 + zero, _ds(n, 16 if ref.dtype == BF16 else 8)]

    def paced(tasks, ref, results):
        for n, task in enumerate(tasks):
            spare(ref, 0)[...] = pltpu.bitcast(results[n * len(results) // len(tasks)], ref.dtype)
            task()

    def tie(ref):
        ties.append(spare(ref.bitcast(U32) if ref.dtype == BF16 else ref, 1))

    def tied(x):
        head = x[0:8, 0:128]
        while ties:
            ref = ties.pop()
            ref[...] = pltpu.bitcast(head, ref.dtype)
            head = pltpu.bitcast(ref[...], x.dtype)
        if x.shape[1] > 128:
            head = jnp.concatenate([head, x[0:8, 128:]], axis=1)
        return _cat([head, x[8:]]) if x.shape[0] > 8 else head

    def permute_rows(dst, base):
        for d in range(AD):
            for t in range(LT):
                dst[pl.ds((base + d * AH) // 2, AH // 2), t * 128:(t + 1) * 128] = pltpu.bitcast(
                    tmp[t, pl.ds(d, AH, stride=AD), :].astype(BF16), U32)

    def prep_wqkv(j):
        for t in range(LT):
            tmp[t] = awqkv[j, t * 128:(t + 1) * 128, :].astype(F32).T
        permute_rows(wqkv_p, j * D)

    def prep_wo():
        for t in range(LT):
            tmp[t] = awo[:, t * 128:(t + 1) * 128].astype(F32)
        permute_rows(wo_p, 0)

    def a_pass(i, b, c, k0=0, k1=LT):
        lanes = slice(c % LT * 128, c % LT * 128 + 128)
        if c < 3 * LT:
            if c == k0 == 0:
                x_s[b] = ax[_ds(i, TB), :].astype(F32)
            w = pltpu.bitcast(wqkv_p[c * 64:(c + 1) * 64, k0 * 128:k1 * 128], BF16)
            r = lax.dot_general(tied(x_s[b, :, k0 * 128:k1 * 128]), w, NT, preferred_element_type=F32)
        else:
            x = jnp.concatenate([oa[1 - b][k] for k in range(k0, k1)], axis=1)
            r = _dot(tied(x), pltpu.bitcast(wo_p[k0 * 64:k1 * 64, lanes], BF16))
        if k0:
            r = _cat(list(map(_add, _vregs(tmp[c % 4, 0:TB]), _vregs(r))))
        if k1 < LT:
            tmp[c % 4, 0:TB] = r
        elif c >= 3 * LT:
            outa[_ds(i - 1, TB), lanes] = r.astype(BF16)
        else:
            qkv[b][c, HALO:] = r
            if c >= LT and isinstance(i, int) and i == 0:
                qkv[b][c, 0:HALO] = jnp.broadcast_to(r[0:1, :], (HALO, 128))
            elif c >= LT:
                qkv[b][c, 0:HALO] = qkv[1 - b][c, TB:]
        return _vregs(r)

    def a_attention(b, first_block=False):
        state = {}

        def window(c, r0, w):
            return qkv[b][c, HALO + r0 - ADIL * w:HALO + r0 - ADIL * w + 8]

        def logits(r0, ws):
            q = [window(t, r0, 0) for t in range(LT)]
            for w in ws:
                a = _total([q[t] * window(LT + t, r0, w) for t in range(LT)])
                a = _total([a] + [pltpu.roll(a, d, 1) for d in range(AH, 128, AH)])
                if first_block and r0 < ADIL * w:
                    pos = lax.broadcasted_iota(jnp.int32, (8, 128), 0) + r0
                    a = jnp.where(pos >= ADIL * w, a, MASKED * AD ** 0.5)
                state[r0, w] = a

        def mix(r0, ts):
            if ts[0] == 0:
                lg = [state.pop((r0, w)) for w in range(AW)]
                m = functools.reduce(jnp.maximum, lg)
                state[r0] = [jnp.exp2((a - m) * (AD ** -0.5 * LOG2E)) for a in lg]
                state[r0].append(_recip(_total(state[r0])))
            e = state[r0]
            for t in ts:
                oa[b][t, r0:r0 + 8] = _total([e[w] * window(2 * LT + t, r0, w) for w in range(AW)]) * e[AW]

        steps = [(0, logits, range(4)), (0, logits, range(4, AW)), (8, mix, range(1)), (8, mix, range(1, LT))]
        return [functools.partial(f, r0 - lag, some) for r0 in range(0, TB + 8, 8)
                for lag, f, some in steps if 0 <= r0 - lag < TB]

    def place(j, first):
        return first // 10 * 3 + j

    def stored(g, name, at=None, as_words=True):
        n = place(g.j, g.first)
        if name[0] == "cell":
            slot = LT * g.seat[name[1]] + name[2]
            if n == 14:
                return cells2.at[slot]
            return (cells0, cells1)[n % 2].at[50 * ((n if at is None else at) >> 1) + slot]
        ref, n = (sums_o, g.first // 10) if g.j == O else (sums2, n - 13) if n >= 13 else (sums, n)
        if name[0] == "both":
            slot = 20 + MIXES.index((g.seat[name[1]], g.seat[name[2]] - LT))
        else:
            slot = 10 * "-+".index(name[0]) + g.seat[name[1]]
        return (ref.bitcast(U32) if as_words else ref).at[40 * (n if at is None else at) + slot]

    def runs(ref, k, r0, r1, r2):
        return _cat([ref[k, _ds(r, 8, n)] for r, n in ((r0, L), (r1, L), (r2, 128 - 2 * L))])

    def weight(g, name):
        if g.j == O and name[0] == "cell":
            return runs(raw_o, name[2], *[_first_row(0, name[1], n) for n in range(3)])
        return stored(g, name)

    def w_turn(g, at=None):
        def turn(c, k, *rows):
            stored(g, ("cell", c, k), at)[...] = pltpu.bitcast(runs(raw, k, *rows).T, U32)
        tasks = []
        for c, _ in g.us + g.ws:
            rows = [_first_row(g.j, c, n) if at is None else sources[30 * at + 3 * c + n] for n in range(3)]
            tasks += [functools.partial(turn, c, k, *rows) for k in range(LT)]
        return [functools.partial(_run, tasks[n:n + 2]) for n in range(0, len(tasks), 2)]

    def w_combine(g, at=None):
        minus, plus = {}, {}
        pairs = g.pairs if at is None else sorted(g.pairs, key=lambda p: p[3] // 3)

        def get(r, c, k, optional=False):
            if g.j == O:
                rows = [_first_row(0, c, min(n // 5, 2)) + n - 5 * min(n // 5, 2) for n in (r // 8, r // 8 + 1)]
                return _cat([raw_o[k, _ds(n, 8)].astype(F32) for n in rows])
            x = stored(g, ("cell", c, k), at)[r // 2:r // 2 + 8]
            return pltpu.bitcast(jnp.where(at < 12, x, 0) if optional else x, BF16).astype(F32)

        def put(r, x, *name):
            stored(g, name, at, as_words=False)[r:r + 16] = x.astype(BF16)

        def combine(r, pair):
            u, i, w, j = pair
            optional = at is not None and g.j == 0 and (i == LT - 1 or j == 0)
            x, y = get(r, u, j, optional), get(r, w, i, optional)
            put(r, x + y, "both", u, w)
            if g.j == O:
                x, y = y, x
            for c, d, own, other in ((u, i, x, y), (w, j, y, x)):
                mine = [p for p in pairs if c in (p[0], p[2])]
                if pair == mine[0]:
                    minus[c] = plus[c] = get(r, c, d)
                minus[c], plus[c] = minus[c] - own, plus[c] + other
                if pair == mine[-1]:
                    put(r, minus[c], "-", c)
                    put(r, plus[c], "+", c)
        return [functools.partial(combine, r, pair) for r in range(0, 128, 16) for pair in pairs]

    for c in (c_wqkv[0], c_ax(0), c_wqkv[1], c_ax(1)):
        c.start()

    def touch(i, carry):
        for ref in (x_s, f_one, f_sum, f_dif, f_mix, cols0, cols1, part, keys, hold, att, keep,
                    out_x, out_y, tmp, cells0, cells1, cells2, sums, sums2, sums_o):
            ref[(i,) + (0,) * (len(ref.shape) - 3) + (slice(0, 16),)] = jnp.zeros((16, ref.shape[-1]), ref.dtype)
        for ref in (wqkv_p, wo_p):
            ref[_ds(i, 8)] = jnp.zeros((8, D), U32)
        return i
    zero = lax.shift_right_logical(lax.fori_loop(0, 2, touch, 0), 16)

    for g in GQ:
        tiles = {seat: c for c, seat in g.seat.items()}
        for n in range(30):
            sources[30 * place(g.j, g.first) + n] = _first_row(g.j, tiles.get(n // 3, g.first), n % 3)

    c_wqkv[0].wait()
    c_wqkv[2].start()
    prep_wqkv(0)
    c_ax(0).wait()
    c_awo.start()
    c_ax(2).start()
    for c in range(LT):
        a_pass(0, 0, c)
    c_wqkv[1].wait()
    c_ax(1).wait()
    get_w(K, 0, 6, 2)
    prep_wqkv(1)
    for c in range(LT):
        a_pass(1, 1, c)
    c_wqkv[2].wait()
    get_w(K, 6, 5, 2)
    prep_wqkv(2)
    for n in range(2 * LT):
        a_pass(n // LT, n // LT, LT + n % LT)
    c_awo.wait()
    get_w(Q, 0, 6, 3)
    get_w(Q, 6, 5, 3)
    get_w(V, 0, 1, 4)
    for c in (c_ax(3), c_mem, c_bx[0]):
        c.start()
    prep_wo()
    for n in range(2 * LT):
        a_pass(n // LT, n // LT, 2 * LT + n % LT)
    _run(a_attention(0, True))
    for c in range(LT):
        a_pass(1, 1, 3 * LT + c)

    def a_step(it, carry):
        for b in range(2):
            i = 2 * it + b
            third = (i * 43 - 86) >> 7
            t = (i - 2 - 3 * third) * NF + 10 * third
            pl.when(i < 5)(functools.partial(got_w, raw, t, 1, i))
            pl.when(i < 14)(functools.partial(got_w, raw, t + 8, 3, i))
            got_w(raw, t + 1, 7, i)
            c_ax(i).wait()
            third = (i * 43) >> 7
            for j in range(3):
                for t, n, needed in ((1, 7, i < 15), (8, 3, i < 12)):
                    pl.when(needed & (i - 3 * third == j))(functools.partial(get_w, j, 10 * third + t, n, i + 2))
            pl.when(it < NB // 2 - 1)(lambda: c_ax(i + 2).start())
            if b:
                pl.when(i > 12)(lambda: get_w(O, 6 * (i - 13), 6, it - 6))
                pl.when(i == 15)(lambda: get_w(O, 18, 6, 1))
            else:
                pl.when(i == 14)(lambda: get_w(O, 6, 6, 0))
            combine = w_combine(_Group(1 - b, 0), jnp.where(i < 3, 11, i - 3))
            side = [(a_attention(1 - b), 0, 17, 3, qkv[1 - b], oa[1 - b]),
                    (w_turn(_Group(b, 0), i - 2), 22, 5 * LT, 99, raw, (cells0, cells1)[b]),
                    (combine[:90], 0, 17, 2, (cells1, cells0)[b], sums),
                    (combine[90:], 17, 25, 2, (cells1, cells0)[b], sums)]
            rs = []
            for c in range(5 * LT):
                if c % 5 < 4:
                    rs.append(a_pass(i, b, c - c // 5, 0, 4))
                else:
                    rs.append([a_pass(i, b, c // 5 * 4 + n, 4, LT) for n in range(4)][0])
                for tasks, c0, c1, lag, src, dst in side:
                    if c0 <= c < c1:
                        if len(rs) < lag:
                            _run(_share(tasks, c - c0, c1 - c0))
                        else:
                            paced(_share(tasks, c - c0, c1 - c0), src, rs[-lag])
                        tie(dst)
            ties.clear()
        return carry

    lax.fori_loop(1, NB // 2, a_step, 0)
    got_w(raw, V * NF + 41, 7, NB)
    c_mem.wait()
    c_bx[0].wait()
    got_w(raw_o, 0, 12, 0)
    for t in range(24, NF, 6):
        get_w(O, t, 6, 1 if t < 30 else NB + 1)

    def tokens(s):
        return [bx[_ds(s, SEG), k * 128:(k + 1) * 128].astype(F32) for k in range(LT)]

    def project_group(odd, g, product, nm):
        pa, pb = (g.ws, g.us) if odd else (g.us, g.ws)
        half, same, cross = slice(HALF * odd, HALF * odd + HALF), {}, {}

        def with_memory(x, k):
            return _cat([x, f_one[odd, k, SEG:SEG + nm]])

        def prod(lhs, *name):
            return product.now(lhs, weight(g, name))

        def direct(c):
            for _, k in [x for x in g.direct if x[0] == c]:
                r = prod(lambda: f_one[odd, k, 0:SEG + nm], "cell", c, k)
                same[c] = list(map(_add, same[c], r))

        def other(a):
            return cols1.at[g.j, a, M:L] if odd else part.at[place(g.j, a), a % 10]

        def mixed(a, b, r):
            cross[a] = list(map(_add, cross[a] if a in cross else _vregs(other(a)[half]), r))
            for x, h in zip(r, (2 * odd, 2 * odd + 1, *range(4, 9))):
                same[b][h] = same[b][h] + x

        def save_cross(a):
            other(a)[half] = _cat(cross.pop(a))

        def save(c, more=None):
            cols[odd][g.j, c, 0:nm] = _cat(same[c][4:])
            cols[1 - odd][g.j, c, M:L] = _add(more, _cat(same[c][:4]))
        for some in (pb[:-2], pb[-2:]):
            for b, j in some:
                same[b] = list(prod(lambda: with_memory(f_dif[odd, j], j), "+", b))
                direct(b)
            for a, i in pa:
                if a not in same:
                    same[a] = prod(lambda: f_one[odd, i, 0:SEG + nm], "-", a)
                    x = _add(other(a)[...] if odd else None, _cat(same[a][:4]))
                    other(a)[HALF - half.start:SEG - half.start] = x[HALF - half.start:SEG - half.start]
                    cross[a] = _vregs(x[half])
                    direct(a)
                else:
                    same[a] = _vregs(cols[1 - odd][g.j, a, M:L]) + _vregs(cols[odd][g.j, a, 0:nm])
                for b, j in some:
                    if i != j:
                        product.tick()
                        product.soon(with_memory(f_mix[odd, MIXES.index((i, j))], i),
                                     weight(g, ("both", b, a) if odd else ("both", a, b)),
                                     functools.partial(mixed, a, b))
                for b, j in some:
                    if i != j:
                        r = prod(lambda: f_sum[odd, SUMS.index((min(i, j), max(i, j))), 0:SEG + nm], "cell", a, j)
                        same[a] = list(map(_add, same[a], r))
                        same[b] = list(map(_sub, same[b], r))
                save(a)
                product.after(HALF + nm, functools.partial(save_cross, a))
            for b, _ in some:
                product.after(HALF + nm, functools.partial(save, b, part[place(g.j, b), b % 10] if odd else None))
        product.after(HALF + nm, lambda: product.ready.extend((g.j, c) for c in g.seat))

    def last_queries(g, product):
        product.passed(0, True)
        for w, i in g.ws:
            r = list(map(_add, _vregs(cols1[Q, w, M:L]), product.now(lambda: f_one[1, i, 0:SEG], weight(g, ("-", w)))))
            for u, j in g.us:
                if i != j:
                    x = product.now(lambda: f_mix[1, MIXES.index((i, j))], weight(g, ("both", u, w)))
                    r[2:] = list(map(_add, r[2:], x))
            cols1[Q, w, M:L] = _cat(r)
        product.ready += [(Q, c) for c in g.seat]

    def out_groups(odd, gs, same, cross, product, last):
        h0, nh = (0, SEG * odd) if last else (2 - 2 * odd, HALF)
        mix = {}

        def xa(c, r0=0, n=SEG):
            return att[c, M + SEG * (1 - odd) + r0:M + SEG * (1 - odd) + r0 + n]

        def xb(c, r0=0, n=SEG):
            return att[c, L + r0:L + r0 + n] if odd else keep[c, r0:r0 + n]

        def xm(c):
            return att[c, 0:M]

        def prod(g, m, x, *name):
            r = product.now(lambda: x() if last else _cat([m(), x()]), weight(g, name))
            return r if last else r[1:] + r[:1]

        def mixed(s, t, r):
            mix[s, t] = list(map(_add, mix.get((s, t), [None] * 4), r))

        def spend(s, t):
            for x, h in zip(mix.pop((s, t), []), list(range(h0, h0 + nh // 8)) + [4]):
                same[t][h] = _add(same[t][h], x)
                if h < 4:
                    cross[s][h] = _add(cross[s][h], x)
        sides = [(g, {d: c for c, d in (g.us if odd else g.ws)}, {d: c for c, d in (g.ws if odd else g.us)})
                 for g in gs]
        for i in range(LT):
            shared = [None] * 5
            for g, pa, pb in sides:
                rs = [prod(g, lambda: xm(pb[i]), lambda: xa(pb[i]) - xb(pb[i]), "+", pb[i])] if i in pb else []
                rs += [prod(g, lambda: xm(c), lambda: xa(c), "cell", c, k) for c, k in g.direct if k == i]
                for r in rs:
                    same[i] = list(map(_add, same[i], r))
                if i in pa:
                    shared = list(map(_add, shared, prod(g, lambda: xm(pa[i]), lambda: xa(pa[i]), "-", pa[i])))
                    if odd:
                        keep[pa[i]] = xa(pa[i])
            same[i] = list(map(_add, same[i], shared))
            cross[i] = list(map(_add, cross[i], shared))
            for j in range(i + 1, LT):
                diff = [None] * 5
                for s, t in ((i, j), (j, i)):
                    for g, pa, pb in sides:
                        if s in pa and t in pb:
                            a, b = pa[s], pb[t]
                            if nh:
                                product.tick()
                                x = xa(a, 8 * h0, nh) + xb(b, 8 * h0, nh)
                                product.soon(x if last else _cat([x, xm(a)]),
                                             weight(g, ("both", a, b) if odd else ("both", b, a)),
                                             functools.partial(mixed, s, t))
                            r = prod(g, lambda: xm(a) + xm(b), lambda: xa(a) + xa(b), "cell", b, s)
                            diff = list(map(_add if s == i else _sub, diff, r))
                    product.after(nh if last else nh + M, functools.partial(spend, s, t))
                same[i] = list(map(_add, same[i], diff))
                same[j] = list(map(_sub, same[j], diff))

    def project_out(odd, s, product, last=False):
        same, cross = [[None] * 5 for _ in range(LT)], [[None] * 4 for _ in range(LT)]
        for gs in (GO[:3], GO[3:]):
            assert all((O, c) in product.ready for g in gs for c in g.seat)
            out_groups(odd, gs, same, cross, product, last)
        product.passed(0, True)
        for k in range(LT):
            lanes = slice(k * 128, (k + 1) * 128)
            if odd:
                out_x[k], out_y[k] = _cat(same[k][:4]), _cat(cross[k])
            else:
                outb[_ds(s - 2, SEG), lanes] = (out_x[k] + _cat(cross[k])).astype(BF16)
                outb[_ds(s - 1, SEG), lanes] = (out_y[k] + _cat(same[k][:4])).astype(BF16)
        return [x[-1] for x in same]

    def attend(odd, s, m, product, last=False):
        xa, xb = tokens(jnp.minimum(s + 1, NSEG - 1)), tokens(s if odd else jnp.minimum(s + 2, NSEG - 1))
        nm = m[0].shape[0]
        for k in range(LT):
            f_one[odd, k, 0:SEG + m[k].shape[0]] = _cat([xa[k], m[k]])
            f_dif[odd, k] = xa[k] - xb[k]
        for n, (i, j) in enumerate(SUMS):
            f_sum[odd, n, 0:SEG + nm] = _cat([xa[i] + xa[j], m[i] + m[j]])
        for n, (i, j) in enumerate(MIXES):
            f_mix[odd, n] = (xa[i] + xb[j])[HALF * odd:HALF * odd + HALF]

        lane = lax.broadcasted_iota(jnp.int32, (L, 128), 1)
        zone = [(lane >= L * z) & (lane < L * z + L) for z in range(3)]
        some = [(lane >= 24 + 16 * n) & (lane < 40 + 16 * n) for n in range(2)]

        def tile(j, g, n, z):
            assert (j, 6 * g + TILE[n][z]) in product.ready
            return cols[odd][j, 6 * g + TILE[n][z]]

        def gathered(j, g, n):
            x = jnp.where(zone[2], tile(j, g, n, 2), 0.0) if j == K else tile(j, g, n, 2)
            return jnp.where(zone[0], tile(j, g, n, 0), jnp.where(zone[1], tile(j, g, n, 1), x))

        def stack(xs):
            return _cat(xs + [jnp.zeros((8, 128), F32)])

        def by_head(x, a, of_a):
            xs = [jnp.zeros((L, 128), F32)] * 2 + [x]
            if a < 2:
                xs[a], xs[2] = jnp.where(of_a, x, 0.0), jnp.where(of_a, 0.0, x)
            return stack(xs)

        def turned(slot, x):
            keys[slot] = x.T
            return keys[slot]

        def one_pass(x, w):
            r = _dot(x, w.astype(BF16))
            product.passed(1)
            return _cat(_vregs(r))

        def done(g, n, z, o):
            product.ready.append((O, 6 * g + TILE[n][z]))
            att[6 * g + TILE[n][z], 0:M] = o[0:M]
            att[6 * g + TILE[n][z], M + SEG * odd:L + SEG * odd] = o[M:L]

        def alone(j, g):
            sc = {}
            for z in (2, 1, 0):
                for n in range(2):
                    w = by_head(tile(j, g, n, z), z, ~zone[z] | some[n] if z == n else ~zone[z])
                    if j == V:
                        p = hold[g, 2 + n] if z in (2, n) else jnp.where(zone[2], hold[g, 2 + n], hold[g, 2 + z])
                        done(g, n, z, one_pass(p, w))
                        continue
                    r = one_pass(tile(Q, g, n, z), turned(3 * n + z, w))
                    if z in (2, n):
                        sc[n] = _add(sc.get(n), r)
                    else:
                        sc[n], sc[z] = sc[n] + jnp.where(zone[2], r, 0.0), sc[z] + jnp.where(zone[2], 0.0, r)
            for n in sc:
                hold[g, n] = sc[n]

        def together(g):
            for n in range(2):
                turned(4 * g + 2 + n, stack([tile(K, g, n, z) for z in range(3)]))
            for n in range(2):
                hold[g, n] = one_pass(gathered(Q, g, n), turned(4 * g + 4 + n, by_head(gathered(K, g, n), n, some[n])))
            for n in range(2):
                hold[g - 1, 4 + n] = one_pass(hold[g - 1, 2 + n], by_head(gathered(V, g - 1, n), n, some[n]))
                for z in range(3):
                    h = n if z == 2 else z
                    w = [jnp.where(zone[z][0:8], y, 0.0) for y in _vregs(keys[4 * g + 2 + n])]
                    w[5 * z:5 * z + 5] = [jnp.where(zone[z], 0.0, tile(V, g - 1, n, z))]
                    r = one_pass(jnp.where(zone[z], hold[g - 1, 2 + h], tile(Q, g, n, z)), _cat(w))
                    hold[g, h] = hold[g, h] + jnp.where(zone[z], r, 0.0)
                    done(g - 1, n, z, jnp.where(zone[z], hold[g - 1, 4 + n], r))

        def softmax(g):
            ahead = lane[0:8] % L - lax.broadcasted_iota(jnp.int32, (8, 128), 0)
            for n in range(2):
                x = _cat([jnp.where(ahead <= 8 * b, y, MASKED * DH ** 0.5) if b else y
                          for b, y in enumerate(_vregs(hold[g, n]))])
                top = [jnp.max(jnp.where(zone[z], x, -jnp.inf), axis=1, keepdims=True) for z in (n, 2)]
                e = jnp.exp2((x - jnp.where(zone[2], top[1], top[0])) * (DH ** -0.5 * LOG2E))
                e = [jnp.where(zone[z], e, 0.0) for z in (n, 2)]
                total = [jnp.sum(y, axis=1, keepdims=True) for y in e]
                hold[g, 2 + n] = (e[0] + e[1]) * _recip(jnp.where(zone[2], total[1], total[0]))

        for g, t in enumerate(TIMES["last" if last else "first" if nm > M else odd]):
            tasks = [functools.partial(alone, V if g else K, max(g - 1, 0)) if g % NG == 0 else functools.partial(together, g)]
            product.events.setdefault(t, []).extend(tasks + [functools.partial(softmax, g)] * (g < NG))
        for g in GQ:
            if last and g.j == Q:
                last_queries(g, product)
            else:
                project_group(odd, g, product, nm)
        return product

    first = _Products({}, tied)

    def spread(tasks, t0, t1, src=None, dst=None):
        def run(some):
            if src is None or len(first.results) < 16:
                _run(some)
            else:
                paced(some, src, first.results[-16])
            if dst is not None:
                tie(dst)
        for t in range(t0, t1):
            if _share(tasks, t - t0, t1 - t0):
                first.events.setdefault(t, []).append(functools.partial(run, _share(tasks, t - t0, t1 - t0)))

    def a_last(c, k):
        def use(r):
            x = _cat(list(map(_add, _vregs(tmp[c, 0:TB]), r)) if k else r)
            if k < LT - 1:
                tmp[c, 0:TB] = x
            else:
                outa[S - TB:S, c * 128:(c + 1) * 128] = x.astype(BF16)
        first.soon(oa1[k], wo_p.at[k * 64:(k + 1) * 64, c * 128:(c + 1) * 128], use)

    end = 3 * NF * LT
    spread(a_attention(1), 12, 138, qkv1, oa1)
    spread(w_turn(_Group(V, 40)), 138, 138 + 1)
    spread(w_combine(_Group(Q, 40)), 138, 215, cells1, sums2)
    spread(w_combine(GO[0]), 215, 285, raw_o, sums_o)
    spread([lambda: tie(cells2)], 285 - 20, 285 - 19)
    spread(w_combine(_Group(V, 40)), 285, 375, cells2, sums2)
    spread([lambda: got_w(raw_o, 12, 18, 1), c_bx[1].start], 375, 375 + 1)
    spread(w_combine(GO[1]) + w_combine(GO[2]), 375 + 6, 560, raw_o, sums_o)
    spread([lambda: got_w(raw_o, 30, 18, NB + 1)], 560, 560 + 1)
    spread(w_combine(GO[3]) + w_combine(GO[4]), 560 + 6, end + 32, raw_o, sums_o)
    spread([functools.partial(a_last, c, k) for k in range(LT) for c in range(LT)], end, end + LT * NF)
    attend(0, 0, [_cat([mem[:, k * 128:(k + 1) * 128].astype(F32), x]) for k, x in enumerate(tokens(0))], first)
    first.passed(0, True)
    m = [None] * LT
    for c in range(NF):
        assert (O, c) in first.ready
        for k in range(LT):
            m[k] = _add(m[k], first.now(lambda: att[c, 0:M], weight(GO[c // 10], ("cell", c, k)))[0])
    first.passed(0, True)
    for k in range(LT):
        mem_s[k] = m[k]
    c_out(0, pl.ds(0, S)).start()
    c_bx[1].wait()

    def b_step(n, carry):
        m = [mem_s[k] for k in range(LT)]
        for odd in (1, 0):
            m = project_out(odd, 2 * n + 2 - odd, attend(odd, 2 * n + 2 - odd, m, _Products({}, tied)))
        for k in range(LT):
            mem_s[k] = m[k]
        c_out(1, _ds(n, 2 * SEG)).start()
        return carry

    lax.fori_loop(0, NSEG // 2 - 1, b_step, 0)
    final = attend(1, NSEG - 1, [mem_s[k] for k in range(LT)], _Products({}, tied), last=True)
    final.passed(0, True)
    project_out(1, NSEG - 1, final, last=True)
    project_out(0, NSEG, final, last=True)
    c_out(1, _ds(NSEG // 2 - 1, 2 * SEG)).start()
    for j in range(2):
        c_out(j, pl.ds(0, S)).wait()


def pallas_concat_heads__sliding_local_dilated__memory_aug_recurrent_mem_tr__prompt_kernel(
    A_x, A_wqkv, A_wo, B_x, B_mem0, B_Wq, B_Wk, B_Wv, B_Wo, B_seg_len,
):
    assert B_seg_len == SEG
    assert A_x.shape == B_x.shape == (1, S, D) and B_mem0.shape == (1, M, D)
    assert B_Wq.shape == B_Wk.shape == B_Wv.shape == (D, H, DH) and B_Wo.shape == (H, DH, D)
    vmem, dma = pltpu.VMEM, pltpu.SemaphoreType.DMA
    call = pl.pallas_call(
        _kernel,
        out_shape=jax.ShapeDtypeStruct((S, 2 * D), BF16),
        in_specs=[pl.BlockSpec(memory_space=pl.ANY)] * 9,
        out_specs=pl.BlockSpec(memory_space=pl.ANY),
        scratch_shapes=[
            vmem((S, D), BF16),
            vmem((3, D, D), BF16),
            vmem((D, D), BF16),
            vmem((LT, D, 128), F32),
            vmem((3 * D // 2, D), U32),
            vmem((D // 2, D), U32),
            vmem((2, TB, D), F32),
            vmem((3 * LT + 1, HALO + TB, 128), F32), vmem((3 * LT + 1, HALO + TB, 128), F32),
            vmem((LT + 1, TB, 128), F32), vmem((LT + 1, TB, 128), F32),
            vmem((S, D), BF16),
            vmem((S, D), BF16),
            vmem((M, D), BF16),
            vmem((LT, 3 * NF * 128, 128), BF16),
            vmem((351, 64, 128), U32), vmem((351, 64, 128), U32), vmem((51, 64, 128), U32),
            vmem((LT + 1, NF * 128, 128), BF16),
            vmem((521, 128, 128), BF16), vmem((81, 128, 128), BF16), vmem((201, 128, 128), BF16),
            vmem((LT, M, 128), F32),
            vmem((2, LT, L + SEG, 128), F32),
            vmem((2, len(SUMS), L + SEG, 128), F32),
            vmem((2, LT, SEG, 128), F32),
            vmem((2, len(MIXES), HALF, 128), F32),
            vmem((3, NF, L, 128), F32), vmem((3, NF, L, 128), F32),
            vmem((len(GQ), LT, SEG, 128), F32),
            vmem((4 * NG + 2, 128, 128), F32),
            vmem((NG, 6, L, 128), F32),
            vmem((NF, L + SEG, 128), F32),
            vmem((NF, SEG, 128), F32),
            vmem((LT, SEG, 128), F32), vmem((LT, SEG, 128), F32),
            pltpu.SMEM((30 * len(GQ),), jnp.int32),
            dma((7,)), dma((NB,)), dma((NB + 2,)), dma((2,)),
        ],
        compiler_params=pltpu.CompilerParams(
            vmem_limit_bytes=124 * 1024 * 1024, disable_bounds_checks=True, disable_semaphore_checks=True),
        name="sliding_and_memory_attention",
    )

    def by_feature(w):
        return w.transpose(1, 2, 0).reshape(H * DH, D)

    out = call(A_x.reshape(S, D), A_wqkv, A_wo, B_x.reshape(S, D), B_mem0.reshape(M, D),
               by_feature(B_Wq), by_feature(B_Wk), by_feature(B_Wv), B_Wo.reshape(H * DH, D))
    return out.reshape(1, S, 2 * D)
```

```python
import functools

import jax
import jax.numpy as jnp
from jax import lax
from jax.experimental import pallas as pl
from jax.experimental.pallas import tpu as pltpu

F32, BF16, U32 = jnp.float32, jnp.bfloat16, jnp.uint32
NT = (((1,), (1,)), ((), ()))
MASKED = -1000000000.0
LOG2E = 1.4426950408889634

S, D = 2048, 640
LT = D // 128

AH, AD, AW, ADIL = 32, 20, 8, 2
HALO = 16
TB = 128
NB = S // TB

H, DH, M, SEG = 32, 192, 8, 32
L = M + SEG
HALF = SEG // 2
NSEG = S // SEG
NF = H * DH // 128
SUMS = [(i, j) for i in range(LT) for j in range(i + 1, LT)]
MIXES = [(i, j) for i in range(LT) for j in range(LT) if i != j]

NG = H // 4
TILE = ((1, 2, 0), (3, 4, 5))
PIECES = ((0, 40, 80), (168, 208, 248), (384, 128, 424), (600, 296, 336), (472, 560, 512), (640, 680, 720))


class _Group:
    def __init__(self, j, first):
        u_diag, w_diag = (range(LT), range(LT)) if first + 10 <= NF else (range(4), range(1, 5))
        self.j, self.first = j, first
        self.us = [(first + n, i) for n, i in enumerate(u_diag)]
        self.ws = [(first + len(u_diag) + n, j) for n, j in enumerate(w_diag)]
        self.pairs = [(u, i, w, j) for u, i in self.us for w, j in self.ws if i != j]
        paired = [(u, j) for u, i, w, j in self.pairs] + [(w, i) for u, i, w, j in self.pairs]
        self.direct = [(c, k) for c, d in self.us + self.ws for k in range(LT)
                       if k != d and (c, k) not in paired]
        self.seat = dict(self.us + [(w, LT + j) for w, j in self.ws])


K, Q, V, O = range(4)
GQ = [_Group(j, t) for t in (0, 10, 20) for j in (K, Q, V)]
GQ += [_Group(j, t) for j, t in ((K, 30), (Q, 30), (K, 40), (Q, 40), (V, 30), (V, 40))]
GO = [_Group(O, t) for t in range(0, NF, 10)]
TIMES = {"first": (148, 274, 352, 434, 499, 592, 729, 809, 860),
         "last": (127, 228, 325, 379, 452, 526, 605, 675, 745),
         1: (148, 314, 392, 470, 552, 636, 728, 799, 859),
         0: (137, 314, 390, 481, 551, 632, 728, 812, 863)}


def _first_row(j, c, n):
    return (j * NG + c // 6) * 96 + PIECES[c % 6][n] // 8


def _ds(i, n, size=None):
    return pl.ds(i * n if isinstance(i, int) else pl.multiple_of(i * n, n), size or n)


def _dot(a, b):
    return jnp.dot(a, b, preferred_element_type=F32)


def _recip(x):
    r = pl.reciprocal(x, approx=True)
    return r * (2.0 - x * r)


def _add(a, b):
    return b if a is None else a + b


def _sub(a, b):
    return -b if a is None else a - b


def _total(xs):
    return functools.reduce(jnp.add, xs)


def _vregs(x):
    return [x[r:r + 8] for r in range(0, x.shape[0], 8)]


def _cat(xs):
    return jnp.concatenate(xs, axis=0)


def _share(tasks, k, n):
    return tasks[k * len(tasks) // n:(k + 1) * len(tasks) // n]


def _run(tasks):
    for task in tasks:
        task()


class _Products:
    def __init__(self, events, tied):
        self.events, self.tied, self.results, self.ready = events, tied, [], []
        self.count, self.usual, self.flushed, self.waiting = 0, 0, -1, {}

    def dot(self, x, w):
        self.results.append(_vregs(_dot(self.tied(x), pltpu.bitcast(w, BF16) if w.dtype == U32 else w)))
        return self.results[-1]

    def tick(self):
        self.count += 1
        _run(self.events.pop(self.count - 1, []))

    def now(self, x, w):
        self.tick()
        r = self.dot(x(), w[...])
        self.passed(1)
        return r

    def soon(self, x, w, use):
        self.waiting.setdefault(x.shape[0], []).append([x, w[...], [use]])

    def after(self, rows, task):
        if self.waiting.get(rows):
            self.waiting[rows][-1][2].append(lambda r: task())
        else:
            task()

    def passed(self, n, last=False):
        self.usual += n
        for rows in sorted(self.waiting, reverse=True):
            queue = self.waiting[rows]
            while queue and (last or (len(queue) >= 4 and self.usual % 4 == 0
                                      and (self.flushed < self.usual or len(queue) >= 8 or rows >= L))):
                for x, w, uses in queue[:4]:
                    r = self.dot(x, w)
                    for use in uses:
                        use(r)
                del queue[:4]
                if rows < L:
                    self.flushed = self.usual


def _kernel(ax_hbm, awqkv_hbm, awo_hbm, bx_hbm, mem_hbm, wq_hbm, wk_hbm, wv_hbm, wo_hbm,
            out_hbm,
            ax, awqkv, awo, tmp, wqkv_p, wo_p, x_s, qkv0, qkv1, oa0, oa1, outa,
            bx, mem, raw, cells0, cells1, cells2, raw_o, sums, sums2, sums_o,
            mem_s, f_one, f_sum, f_dif, f_mix, cols0, cols1, part, keys, hold, att, keep, out_x, out_y,
            sources, sem_a, sem_x, sem_w, sem_o):
    qkv, oa, cols = (qkv0, qkv1), (oa0, oa1), (cols0, cols1)
    outb = ax

    cp = pltpu.make_async_copy
    c_wqkv = [cp(awqkv_hbm.at[:, pl.ds(j * D, D)], awqkv.at[j], sem_a.at[j]) for j in range(3)]
    c_awo = cp(awo_hbm, awo, sem_a.at[3])
    c_mem = cp(mem_hbm, mem, sem_a.at[4])
    c_bx = [cp(bx_hbm.at[rows], bx.at[rows], sem_a.at[5 + n])
            for n, rows in enumerate((pl.ds(0, 3 * SEG), pl.ds(3 * SEG, S - 3 * SEG)))]

    def c_ax(i):
        return cp(ax_hbm.at[_ds(i, TB)], ax.at[_ds(i, TB)], sem_x.at[i])

    def c_out(j, rows):
        return cp((outa, outb)[j].at[rows, :], out_hbm.at[rows, pl.ds(j * D, D)], sem_o.at[j])

    def get_w(j, t, n, batch):
        dst, first = (raw_o, t) if j == O else (raw, j * NF + t)
        for k in range(LT):
            cp((wk_hbm, wq_hbm, wv_hbm, wo_hbm)[j].at[_ds(t, 128, 128 * n), _ds(k, 128)],
               dst.at[k, _ds(first, 128, 128 * n)], sem_w.at[batch]).start()

    def got_w(dst, first, n, batch):
        box = dst.at[0:LT, _ds(first, 128, 128 * n)]
        cp(box, box, sem_w.at[batch]).wait()

    ties = []

    def spare(ref, n):
        return ref.at[ref.shape[0] - 1 + zero, _ds(n, 16 if ref.dtype == BF16 else 8)]

    def paced(tasks, ref, results):
        for n, task in enumerate(tasks):
            spare(ref, 0)[...] = pltpu.bitcast(results[n * len(results) // len(tasks)], ref.dtype)
            task()

    def tie(ref):
        ties.append(spare(ref.bitcast(U32) if ref.dtype == BF16 else ref, 1))

    def tied(x):
        head = x[0:8, 0:128]
        while ties:
            ref = ties.pop()
            ref[...] = pltpu.bitcast(head, ref.dtype)
            head = pltpu.bitcast(ref[...], x.dtype)
        if x.shape[1] > 128:
            head = jnp.concatenate([head, x[0:8, 128:]], axis=1)
        return _cat([head, x[8:]]) if x.shape[0] > 8 else head

    def permute_rows(dst, base):
        for d in range(AD):
            for t in range(LT):
                dst[pl.ds((base + d * AH) // 2, AH // 2), t * 128:(t + 1) * 128] = pltpu.bitcast(
                    tmp[t, pl.ds(d, AH, stride=AD), :].astype(BF16), U32)

    def prep_wqkv(j):
        for t in range(LT):
            tmp[t] = awqkv[j, t * 128:(t + 1) * 128, :].astype(F32).T
        permute_rows(wqkv_p, j * D)

    def prep_wo():
        for t in range(LT):
            tmp[t] = awo[:, t * 128:(t + 1) * 128].astype(F32)
        permute_rows(wo_p, 0)

    def a_pass(i, b, c, k0=0, k1=LT):
        lanes = slice(c % LT * 128, c % LT * 128 + 128)
        if c < 3 * LT:
            if c == k0 == 0:
                x_s[b] = ax[_ds(i, TB), :].astype(F32)
            w = pltpu.bitcast(wqkv_p[c * 64:(c + 1) * 64, k0 * 128:k1 * 128], BF16)
            r = lax.dot_general(tied(x_s[b, :, k0 * 128:k1 * 128]), w, NT, preferred_element_type=F32)
        else:
            x = jnp.concatenate([oa[1 - b][k] for k in range(k0, k1)], axis=1)
            r = _dot(tied(x), pltpu.bitcast(wo_p[k0 * 64:k1 * 64, lanes], BF16))
        if k0:
            r = _cat(list(map(_add, _vregs(tmp[c % 4, 0:TB]), _vregs(r))))
        if k1 < LT:
            tmp[c % 4, 0:TB] = r
        elif c >= 3 * LT:
            outa[_ds(i - 1, TB), lanes] = r.astype(BF16)
        else:
            qkv[b][c, HALO:] = r
            if c >= LT and isinstance(i, int) and i == 0:
                qkv[b][c, 0:HALO] = jnp.broadcast_to(r[0:1, :], (HALO, 128))
            elif c >= LT:
                qkv[b][c, 0:HALO] = qkv[1 - b][c, TB:]
        return _vregs(r)

    def a_attention(b, first_block=False):
        state = {}

        def window(c, r0, w):
            return qkv[b][c, HALO + r0 - ADIL * w:HALO + r0 - ADIL * w + 8]

        def logits(r0, ws):
            q = [window(t, r0, 0) for t in range(LT)]
            for w in ws:
                a = _total([q[t] * window(LT + t, r0, w) for t in range(LT)])
                a = _total([a] + [pltpu.roll(a, d, 1) for d in range(AH, 128, AH)])
                if first_block and r0 < ADIL * w:
                    pos = lax.broadcasted_iota(jnp.int32, (8, 128), 0) + r0
                    a = jnp.where(pos >= ADIL * w, a, MASKED * AD ** 0.5)
                state[r0, w] = a

        def mix(r0, ts):
            if ts[0] == 0:
                lg = [state.pop((r0, w)) for w in range(AW)]
                m = functools.reduce(jnp.maximum, lg)
                state[r0] = [jnp.exp2((a - m) * (AD ** -0.5 * LOG2E)) for a in lg]
                state[r0].append(_recip(_total(state[r0])))
            e = state[r0]
            for t in ts:
                oa[b][t, r0:r0 + 8] = _total([e[w] * window(2 * LT + t, r0, w) for w in range(AW)]) * e[AW]

        steps = [(0, logits, range(4)), (0, logits, range(4, AW)), (8, mix, range(1)), (8, mix, range(1, LT))]
        return [functools.partial(f, r0 - lag, some) for r0 in range(0, TB + 8, 8)
                for lag, f, some in steps if 0 <= r0 - lag < TB]

    def place(j, first):
        return first // 10 * 3 + j

    def stored(g, name, at=None, as_words=True):
        n = place(g.j, g.first)
        if name[0] == "cell":
            slot = LT * g.seat[name[1]] + name[2]
            if n == 14:
                return cells2.at[slot]
            return (cells0, cells1)[n % 2].at[50 * ((n if at is None else at) >> 1) + slot]
        ref, n = (sums_o, g.first // 10) if g.j == O else (sums2, n - 13) if n >= 13 else (sums, n)
        if name[0] == "both":
            slot = 20 + MIXES.index((g.seat[name[1]], g.seat[name[2]] - LT))
        else:
            slot = 10 * "-+".index(name[0]) + g.seat[name[1]]
        return (ref.bitcast(U32) if as_words else ref).at[40 * (n if at is None else at) + slot]

    def runs(ref, k, r0, r1, r2):
        return _cat([ref[k, _ds(r, 8, n)] for r, n in ((r0, L), (r1, L), (r2, 128 - 2 * L))])

    def weight(g, name):
        if g.j == O and name[0] == "cell":
            return runs(raw_o, name[2], *[_first_row(0, name[1], n) for n in range(3)])
        return stored(g, name)

    def w_turn(g, at=None):
        def turn(c, k, *rows):
            stored(g, ("cell", c, k), at)[...] = pltpu.bitcast(runs(raw, k, *rows).T, U32)
        tasks = []
        for c, _ in g.us + g.ws:
            rows = [_first_row(g.j, c, n) if at is None else sources[30 * at + 3 * c + n] for n in range(3)]
            tasks += [functools.partial(turn, c, k, *rows) for k in range(LT)]
        return [functools.partial(_run, tasks[n:n + 2]) for n in range(0, len(tasks), 2)]

    def w_combine(g, at=None):
        minus, plus = {}, {}
        pairs = g.pairs if at is None else sorted(g.pairs, key=lambda p: p[3] // 3)

        def get(r, c, k, optional=False):
            if g.j == O:
                rows = [_first_row(0, c, min(n // 5, 2)) + n - 5 * min(n // 5, 2) for n in (r // 8, r // 8 + 1)]
                return _cat([raw_o[k, _ds(n, 8)].astype(F32) for n in rows])
            x = stored(g, ("cell", c, k), at)[r // 2:r // 2 + 8]
            return pltpu.bitcast(jnp.where(at < 12, x, 0) if optional else x, BF16).astype(F32)

        def put(r, x, *name):
            stored(g, name, at, as_words=False)[r:r + 16] = x.astype(BF16)

        def combine(r, pair):
            u, i, w, j = pair
            optional = at is not None and g.j == 0 and (i == LT - 1 or j == 0)
            x, y = get(r, u, j, optional), get(r, w, i, optional)
            put(r, x + y, "both", u, w)
            if g.j == O:
                x, y = y, x
            for c, d, own, other in ((u, i, x, y), (w, j, y, x)):
                mine = [p for p in pairs if c in (p[0], p[2])]
                if pair == mine[0]:
                    minus[c] = plus[c] = get(r, c, d)
                minus[c], plus[c] = minus[c] - own, plus[c] + other
                if pair == mine[-1]:
                    put(r, minus[c], "-", c)
                    put(r, plus[c], "+", c)
        return [functools.partial(combine, r, pair) for r in range(0, 128, 16) for pair in pairs]

    for c in (c_wqkv[0], c_ax(0), c_wqkv[1], c_ax(1)):
        c.start()

    def touch(i, carry):
        for ref in (x_s, f_one, f_sum, f_dif, f_mix, cols0, cols1, part, keys, hold, att, keep,
                    out_x, out_y, tmp, cells0, cells1, cells2, sums, sums2, sums_o):
            ref[(i,) + (0,) * (len(ref.shape) - 3) + (slice(0, 16),)] = jnp.zeros((16, ref.shape[-1]), ref.dtype)
        for ref in (wqkv_p, wo_p):
            ref[_ds(i, 8)] = jnp.zeros((8, D), U32)
        return i
    zero = lax.shift_right_logical(lax.fori_loop(0, 2, touch, 0), 16)

    for g in GQ:
        tiles = {seat: c for c, seat in g.seat.items()}
        for n in range(30):
            sources[30 * place(g.j, g.first) + n] = _first_row(g.j, tiles.get(n // 3, g.first), n % 3)

    c_wqkv[0].wait()
    c_wqkv[2].start()
    prep_wqkv(0)
    c_ax(0).wait()
    c_awo.start()
    c_ax(2).start()
    for c in range(LT):
        a_pass(0, 0, c)
    c_wqkv[1].wait()
    c_ax(1).wait()
    get_w(K, 0, 6, 2)
    prep_wqkv(1)
    for c in range(LT):
        a_pass(1, 1, c)
    c_wqkv[2].wait()
    get_w(K, 6, 5, 2)
    prep_wqkv(2)
    for n in range(2 * LT):
        a_pass(n // LT, n // LT, LT + n % LT)
    c_awo.wait()
    get_w(Q, 0, 6, 3)
    get_w(Q, 6, 5, 3)
    get_w(V, 0, 1, 4)
    for c in (c_ax(3), c_mem, c_bx[0]):
        c.start()
    prep_wo()
    for n in range(2 * LT):
        a_pass(n // LT, n // LT, 2 * LT + n % LT)
    _run(a_attention(0, True))
    for c in range(LT):
        a_pass(1, 1, 3 * LT + c)

    def a_step(it, carry):
        for b in range(2):
            i = 2 * it + b
            third = (i * 43 - 86) >> 7
            t = (i - 2 - 3 * third) * NF + 10 * third
            pl.when(i < 5)(functools.partial(got_w, raw, t, 1, i))
            pl.when(i < 14)(functools.partial(got_w, raw, t + 8, 3, i))
            got_w(raw, t + 1, 7, i)
            c_ax(i).wait()
            third = (i * 43) >> 7
            for j in range(3):
                for t, n, needed in ((1, 7, i < 15), (8, 3, i < 12)):
                    pl.when(needed & (i - 3 * third == j))(functools.partial(get_w, j, 10 * third + t, n, i + 2))
            pl.when(it < NB // 2 - 1)(lambda: c_ax(i + 2).start())
            if b:
                pl.when(i > 12)(lambda: get_w(O, 6 * (i - 13), 6, it - 6))
                pl.when(i == 15)(lambda: get_w(O, 18, 6, 1))
            else:
                pl.when(i == 14)(lambda: get_w(O, 6, 6, 0))
            combine = w_combine(_Group(1 - b, 0), jnp.where(i < 3, 11, i - 3))
            side = [(a_attention(1 - b), 0, 17, 3, qkv[1 - b], oa[1 - b]),
                    (w_turn(_Group(b, 0), i - 2), 22, 5 * LT, 99, raw, (cells0, cells1)[b]),
                    (combine[:90], 0, 17, 2, (cells1, cells0)[b], sums),
                    (combine[90:], 17, 25, 2, (cells1, cells0)[b], sums)]
            rs = []
            for c in range(5 * LT):
                if c % 5 < 4:
                    rs.append(a_pass(i, b, c - c // 5, 0, 4))
                else:
                    rs.append([a_pass(i, b, c // 5 * 4 + n, 4, LT) for n in range(4)][0])
                for tasks, c0, c1, lag, src, dst in side:
                    if c0 <= c < c1:
                        if len(rs) < lag:
                            _run(_share(tasks, c - c0, c1 - c0))
                        else:
                            paced(_share(tasks, c - c0, c1 - c0), src, rs[-lag])
                        tie(dst)
            ties.clear()
        return carry

    lax.fori_loop(1, NB // 2, a_step, 0)
    got_w(raw, V * NF + 41, 7, NB)
    c_mem.wait()
    c_bx[0].wait()
    got_w(raw_o, 0, 12, 0)
    for t in range(24, NF, 6):
        get_w(O, t, 6, 1 if t < 30 else NB + 1)

    def tokens(s):
        return [bx[_ds(s, SEG), k * 128:(k + 1) * 128].astype(F32) for k in range(LT)]

    def project_group(odd, g, product, nm):
        pa, pb = (g.ws, g.us) if odd else (g.us, g.ws)
        half, same, cross = slice(HALF * odd, HALF * odd + HALF), {}, {}

        def with_memory(x, k):
            return _cat([x, f_one[odd, k, SEG:SEG + nm]])

        def prod(lhs, *name):
            return product.now(lhs, weight(g, name))

        def direct(c):
            for _, k in [x for x in g.direct if x[0] == c]:
                r = prod(lambda: f_one[odd, k, 0:SEG + nm], "cell", c, k)
                same[c] = list(map(_add, same[c], r))

        def other(a):
            return cols1.at[g.j, a, M:L] if odd else part.at[place(g.j, a), a % 10]

        def mixed(a, b, r):
            cross[a] = list(map(_add, cross[a] if a in cross else _vregs(other(a)[half]), r))
            for x, h in zip(r, (2 * odd, 2 * odd + 1, *range(4, 9))):
                same[b][h] = same[b][h] + x

        def save_cross(a):
            other(a)[half] = _cat(cross.pop(a))

        def save(c, more=None):
            cols[odd][g.j, c, 0:nm] = _cat(same[c][4:])
            cols[1 - odd][g.j, c, M:L] = _add(more, _cat(same[c][:4]))
        for some in (pb[:-2], pb[-2:]):
            for b, j in some:
                same[b] = list(prod(lambda: with_memory(f_dif[odd, j], j), "+", b))
                direct(b)
            for a, i in pa:
                if a not in same:
                    same[a] = prod(lambda: f_one[odd, i, 0:SEG + nm], "-", a)
                    x = _add(other(a)[...] if odd else None, _cat(same[a][:4]))
                    other(a)[HALF - half.start:SEG - half.start] = x[HALF - half.start:SEG - half.start]
                    cross[a] = _vregs(x[half])
                    direct(a)
                else:
                    same[a] = _vregs(cols[1 - odd][g.j, a, M:L]) + _vregs(cols[odd][g.j, a, 0:nm])
                for b, j in some:
                    if i != j:
                        product.tick()
                        product.soon(with_memory(f_mix[odd, MIXES.index((i, j))], i),
                                     weight(g, ("both", b, a) if odd else ("both", a, b)),
                                     functools.partial(mixed, a, b))
                for b, j in some:
                    if i != j:
                        r = prod(lambda: f_sum[odd, SUMS.index((min(i, j), max(i, j))), 0:SEG + nm], "cell", a, j)
                        same[a] = list(map(_add, same[a], r))
                        same[b] = list(map(_sub, same[b], r))
                save(a)
                product.after(HALF + nm, functools.partial(save_cross, a))
            for b, _ in some:
                product.after(HALF + nm, functools.partial(save, b, part[place(g.j, b), b % 10] if odd else None))
        product.after(HALF + nm, lambda: product.ready.extend((g.j, c) for c in g.seat))

    def last_queries(g, product):
        product.passed(0, True)
        for w, i in g.ws:
            r = list(map(_add, _vregs(cols1[Q, w, M:L]), product.now(lambda: f_one[1, i, 0:SEG], weight(g, ("-", w)))))
            for u, j in g.us:
                if i != j:
                    x = product.now(lambda: f_mix[1, MIXES.index((i, j))], weight(g, ("both", u, w)))
                    r[2:] = list(map(_add, r[2:], x))
            cols1[Q, w, M:L] = _cat(r)
        product.ready += [(Q, c) for c in g.seat]

    def out_groups(odd, gs, same, cross, product, last):
        h0, nh = (0, SEG * odd) if last else (2 - 2 * odd, HALF)
        mix = {}

        def xa(c, r0=0, n=SEG):
            return att[c, M + SEG * (1 - odd) + r0:M + SEG * (1 - odd) + r0 + n]

        def xb(c, r0=0, n=SEG):
            return att[c, L + r0:L + r0 + n] if odd else keep[c, r0:r0 + n]

        def xm(c):
            return att[c, 0:M]

        def prod(g, m, x, *name):
            r = product.now(lambda: x() if last else _cat([m(), x()]), weight(g, name))
            return r if last else r[1:] + r[:1]

        def mixed(s, t, r):
            mix[s, t] = list(map(_add, mix.get((s, t), [None] * 4), r))

        def spend(s, t):
            for x, h in zip(mix.pop((s, t), []), list(range(h0, h0 + nh // 8)) + [4]):
                same[t][h] = _add(same[t][h], x)
                if h < 4:
                    cross[s][h] = _add(cross[s][h], x)
        sides = [(g, {d: c for c, d in (g.us if odd else g.ws)}, {d: c for c, d in (g.ws if odd else g.us)})
                 for g in gs]
        for i in range(LT):
            shared = [None] * 5
            for g, pa, pb in sides:
                rs = [prod(g, lambda: xm(pb[i]), lambda: xa(pb[i]) - xb(pb[i]), "+", pb[i])] if i in pb else []
                rs += [prod(g, lambda: xm(c), lambda: xa(c), "cell", c, k) for c, k in g.direct if k == i]
                for r in rs:
                    same[i] = list(map(_add, same[i], r))
                if i in pa:
                    shared = list(map(_add, shared, prod(g, lambda: xm(pa[i]), lambda: xa(pa[i]), "-", pa[i])))
                    if odd:
                        keep[pa[i]] = xa(pa[i])
            same[i] = list(map(_add, same[i], shared))
            cross[i] = list(map(_add, cross[i], shared))
            for j in range(i + 1, LT):
                diff = [None] * 5
                for s, t in ((i, j), (j, i)):
                    for g, pa, pb in sides:
                        if s in pa and t in pb:
                            a, b = pa[s], pb[t]
                            if nh:
                                product.tick()
                                x = xa(a, 8 * h0, nh) + xb(b, 8 * h0, nh)
                                product.soon(x if last else _cat([x, xm(a)]),
                                             weight(g, ("both", a, b) if odd else ("both", b, a)),
                                             functools.partial(mixed, s, t))
                            r = prod(g, lambda: xm(a) + xm(b), lambda: xa(a) + xa(b), "cell", b, s)
                            diff = list(map(_add if s == i else _sub, diff, r))
                    product.after(nh if last else nh + M, functools.partial(spend, s, t))
                same[i] = list(map(_add, same[i], diff))
                same[j] = list(map(_sub, same[j], diff))

    def project_out(odd, s, product, last=False):
        same, cross = [[None] * 5 for _ in range(LT)], [[None] * 4 for _ in range(LT)]
        for gs in (GO[:3], GO[3:]):
            assert all((O, c) in product.ready for g in gs for c in g.seat)
            out_groups(odd, gs, same, cross, product, last)
        product.passed(0, True)
        for k in range(LT):
            lanes = slice(k * 128, (k + 1) * 128)
            if odd:
                out_x[k], out_y[k] = _cat(same[k][:4]), _cat(cross[k])
            else:
                outb[_ds(s - 2, SEG), lanes] = (out_x[k] + _cat(cross[k])).astype(BF16)
                outb[_ds(s - 1, SEG), lanes] = (out_y[k] + _cat(same[k][:4])).astype(BF16)
        return [x[-1] for x in same]

    def attend(odd, s, m, product, last=False):
        xa, xb = tokens(jnp.minimum(s + 1, NSEG - 1)), tokens(s if odd else jnp.minimum(s + 2, NSEG - 1))
        nm = m[0].shape[0]
        for k in range(LT):
            f_one[odd, k, 0:SEG + m[k].shape[0]] = _cat([xa[k], m[k]])
            f_dif[odd, k] = xa[k] - xb[k]
        for n, (i, j) in enumerate(SUMS):
            f_sum[odd, n, 0:SEG + nm] = _cat([xa[i] + xa[j], m[i] + m[j]])
        for n, (i, j) in enumerate(MIXES):
            f_mix[odd, n] = (xa[i] + xb[j])[HALF * odd:HALF * odd + HALF]

        lane = lax.broadcasted_iota(jnp.int32, (L, 128), 1)
        zone = [(lane >= L * z) & (lane < L * z + L) for z in range(3)]
        some = [(lane >= 24 + 16 * n) & (lane < 40 + 16 * n) for n in range(2)]

        def tile(j, g, n, z):
            assert (j, 6 * g + TILE[n][z]) in product.ready
            return cols[odd][j, 6 * g + TILE[n][z]]

        def gathered(j, g, n):
            x = jnp.where(zone[2], tile(j, g, n, 2), 0.0) if j == K else tile(j, g, n, 2)
            return jnp.where(zone[0], tile(j, g, n, 0), jnp.where(zone[1], tile(j, g, n, 1), x))

        def stack(xs):
            return _cat(xs + [jnp.zeros((8, 128), F32)])

        def by_head(x, a, of_a):
            xs = [jnp.zeros((L, 128), F32)] * 2 + [x]
            if a < 2:
                xs[a], xs[2] = jnp.where(of_a, x, 0.0), jnp.where(of_a, 0.0, x)
            return stack(xs)

        def turned(slot, x):
            keys[slot] = x.T
            return keys[slot]

        def one_pass(x, w):
            r = _dot(x, w.astype(BF16))
            product.passed(1)
            return _cat(_vregs(r))

        def done(g, n, z, o):
            product.ready.append((O, 6 * g + TILE[n][z]))
            att[6 * g + TILE[n][z], 0:M] = o[0:M]
            att[6 * g + TILE[n][z], M + SEG * odd:L + SEG * odd] = o[M:L]

        def alone(j, g):
            sc = {}
            for z in (2, 1, 0):
                for n in range(2):
                    w = by_head(tile(j, g, n, z), z, ~zone[z] | some[n] if z == n else ~zone[z])
                    if j == V:
                        p = hold[g, 2 + n] if z in (2, n) else jnp.where(zone[2], hold[g, 2 + n], hold[g, 2 + z])
                        done(g, n, z, one_pass(p, w))
                        continue
                    r = one_pass(tile(Q, g, n, z), turned(3 * n + z, w))
                    if z in (2, n):
                        sc[n] = _add(sc.get(n), r)
                    else:
                        sc[n], sc[z] = sc[n] + jnp.where(zone[2], r, 0.0), sc[z] + jnp.where(zone[2], 0.0, r)
            for n in sc:
                hold[g, n] = sc[n]

        def together(g):
            for n in range(2):
                turned(4 * g + 2 + n, stack([tile(K, g, n, z) for z in range(3)]))
            for n in range(2):
                hold[g, n] = one_pass(gathered(Q, g, n), turned(4 * g + 4 + n, by_head(gathered(K, g, n), n, some[n])))
            for n in range(2):
                hold[g - 1, 4 + n] = one_pass(hold[g - 1, 2 + n], by_head(gathered(V, g - 1, n), n, some[n]))
                for z in range(3):
                    h = n if z == 2 else z
                    w = [jnp.where(zone[z][0:8], y, 0.0) for y in _vregs(keys[4 * g + 2 + n])]
                    w[5 * z:5 * z + 5] = [jnp.where(zone[z], 0.0, tile(V, g - 1, n, z))]
                    r = one_pass(jnp.where(zone[z], hold[g - 1, 2 + h], tile(Q, g, n, z)), _cat(w))
                    hold[g, h] = hold[g, h] + jnp.where(zone[z], r, 0.0)
                    done(g - 1, n, z, jnp.where(zone[z], hold[g - 1, 4 + n], r))

        def softmax(g):
            ahead = lane[0:8] % L - lax.broadcasted_iota(jnp.int32, (8, 128), 0)
            for n in range(2):
                x = _cat([jnp.where(ahead <= 8 * b, y, MASKED * DH ** 0.5) if b else y
                          for b, y in enumerate(_vregs(hold[g, n]))])
                top = [jnp.max(jnp.where(zone[z], x, -jnp.inf), axis=1, keepdims=True) for z in (n, 2)]
                e = jnp.exp2((x - jnp.where(zone[2], top[1], top[0])) * (DH ** -0.5 * LOG2E))
                e = [jnp.where(zone[z], e, 0.0) for z in (n, 2)]
                total = [jnp.sum(y, axis=1, keepdims=True) for y in e]
                hold[g, 2 + n] = (e[0] + e[1]) * _recip(jnp.where(zone[2], total[1], total[0]))

        for g, t in enumerate(TIMES["last" if last else "first" if nm > M else odd]):
            tasks = [functools.partial(alone, V if g else K, max(g - 1, 0)) if g % NG == 0 else functools.partial(together, g)]
            product.events.setdefault(t, []).extend(tasks + [functools.partial(softmax, g)] * (g < NG))
        for g in GQ:
            if last and g.j == Q:
                last_queries(g, product)
            else:
                project_group(odd, g, product, nm)
        return product

    first = _Products({}, tied)

    def spread(tasks, t0, t1, src=None, dst=None):
        def run(some):
            if src is None or len(first.results) < 16:
                _run(some)
            else:
                paced(some, src, first.results[-16])
            if dst is not None:
                tie(dst)
        for t in range(t0, t1):
            if _share(tasks, t - t0, t1 - t0):
                first.events.setdefault(t, []).append(functools.partial(run, _share(tasks, t - t0, t1 - t0)))

    def a_last(c, k):
        def use(r):
            x = _cat(list(map(_add, _vregs(tmp[c, 0:TB]), r)) if k else r)
            if k < LT - 1:
                tmp[c, 0:TB] = x
            else:
                outa[S - TB:S, c * 128:(c + 1) * 128] = x.astype(BF16)
        first.soon(oa1[k], wo_p.at[k * 64:(k + 1) * 64, c * 128:(c + 1) * 128], use)

    end = 3 * NF * LT
    spread(a_attention(1), 12, 138, qkv1, oa1)
    spread(w_turn(_Group(V, 40)), 138, 138 + 1)
    spread(w_combine(_Group(Q, 40)), 138, 219, cells1, sums2)
    spread(w_combine(GO[0]), 219, 301, raw_o, sums_o)
    spread([lambda: tie(cells2)], 301 - 20, 301 - 19)
    spread(w_combine(_Group(V, 40)), 301, 378, cells2, sums2)
    spread([lambda: got_w(raw_o, 12, 18, 1), c_bx[1].start], 378, 378 + 1)
    spread(w_combine(GO[1]) + w_combine(GO[2]), 378 + 6, 564, raw_o, sums_o)
    spread([lambda: got_w(raw_o, 30, 18, NB + 1)], 564, 564 + 1)
    spread(w_combine(GO[3]) + w_combine(GO[4]), 564 + 6, end + 32, raw_o, sums_o)
    spread([functools.partial(a_last, c, k) for k in range(LT) for c in range(LT)], end, end + LT * NF)
    attend(0, 0, [_cat([mem[:, k * 128:(k + 1) * 128].astype(F32), x]) for k, x in enumerate(tokens(0))], first)
    first.passed(0, True)
    m = [None] * LT
    for c in range(NF):
        assert (O, c) in first.ready
        for k in range(LT):
            m[k] = _add(m[k], first.now(lambda: att[c, 0:M], weight(GO[c // 10], ("cell", c, k)))[0])
    first.passed(0, True)
    for k in range(LT):
        mem_s[k] = m[k]
    c_out(0, pl.ds(0, S)).start()
    c_bx[1].wait()

    def b_step(n, carry):
        m = [mem_s[k] for k in range(LT)]
        for odd in (1, 0):
            m = project_out(odd, 2 * n + 2 - odd, attend(odd, 2 * n + 2 - odd, m, _Products({}, tied)))
        for k in range(LT):
            mem_s[k] = m[k]
        c_out(1, _ds(n, 2 * SEG)).start()
        return carry

    lax.fori_loop(0, NSEG // 2 - 1, b_step, 0)
    final = attend(1, NSEG - 1, [mem_s[k] for k in range(LT)], _Products({}, tied), last=True)
    final.passed(0, True)
    project_out(1, NSEG - 1, final, last=True)
    project_out(0, NSEG, final, last=True)
    c_out(1, _ds(NSEG // 2 - 1, 2 * SEG)).start()
    for j in range(2):
        c_out(j, pl.ds(0, S)).wait()


def pallas_concat_heads__sliding_local_dilated__memory_aug_recurrent_mem_tr__prompt_kernel(
    A_x, A_wqkv, A_wo, B_x, B_mem0, B_Wq, B_Wk, B_Wv, B_Wo, B_seg_len,
):
    assert B_seg_len == SEG
    assert A_x.shape == B_x.shape == (1, S, D) and B_mem0.shape == (1, M, D)
    assert B_Wq.shape == B_Wk.shape == B_Wv.shape == (D, H, DH) and B_Wo.shape == (H, DH, D)
    vmem, dma = pltpu.VMEM, pltpu.SemaphoreType.DMA
    call = pl.pallas_call(
        _kernel,
        out_shape=jax.ShapeDtypeStruct((S, 2 * D), BF16),
        in_specs=[pl.BlockSpec(memory_space=pl.ANY)] * 9,
        out_specs=pl.BlockSpec(memory_space=pl.ANY),
        scratch_shapes=[
            vmem((S, D), BF16),
            vmem((3, D, D), BF16),
            vmem((D, D), BF16),
            vmem((LT, D, 128), F32),
            vmem((3 * D // 2, D), U32),
            vmem((D // 2, D), U32),
            vmem((2, TB, D), F32),
            vmem((3 * LT + 1, HALO + TB, 128), F32), vmem((3 * LT + 1, HALO + TB, 128), F32),
            vmem((LT + 1, TB, 128), F32), vmem((LT + 1, TB, 128), F32),
            vmem((S, D), BF16),
            vmem((S, D), BF16),
            vmem((M, D), BF16),
            vmem((LT, 3 * NF * 128, 128), BF16),
            vmem((351, 64, 128), U32), vmem((351, 64, 128), U32), vmem((51, 64, 128), U32),
            vmem((LT + 1, NF * 128, 128), BF16),
            vmem((521, 128, 128), BF16), vmem((81, 128, 128), BF16), vmem((201, 128, 128), BF16),
            vmem((LT, M, 128), F32),
            vmem((2, LT, L + SEG, 128), F32),
            vmem((2, len(SUMS), L + SEG, 128), F32),
            vmem((2, LT, SEG, 128), F32),
            vmem((2, len(MIXES), HALF, 128), F32),
            vmem((3, NF, L, 128), F32), vmem((3, NF, L, 128), F32),
            vmem((len(GQ), LT, SEG, 128), F32),
            vmem((4 * NG + 2, 128, 128), F32),
            vmem((NG, 6, L, 128), F32),
            vmem((NF, L + SEG, 128), F32),
            vmem((NF, SEG, 128), F32),
            vmem((LT, SEG, 128), F32), vmem((LT, SEG, 128), F32),
            pltpu.SMEM((30 * len(GQ),), jnp.int32),
            dma((7,)), dma((NB,)), dma((NB + 2,)), dma((2,)),
        ],
        compiler_params=pltpu.CompilerParams(
            vmem_limit_bytes=124 * 1024 * 1024, disable_bounds_checks=True, disable_semaphore_checks=True),
        name="sliding_and_memory_attention",
    )

    def by_feature(w):
        return w.transpose(1, 2, 0).reshape(H * DH, D)

    out = call(A_x.reshape(S, D), A_wqkv, A_wo, B_x.reshape(S, D), B_mem0.reshape(M, D),
               by_feature(B_Wq), by_feature(B_Wk), by_feature(B_Wv), B_Wo.reshape(H * DH, D))
    return out.reshape(1, S, 2 * D)
```

```python
import functools

import jax
import jax.numpy as jnp
from jax import lax
from jax.experimental import pallas as pl
from jax.experimental.pallas import tpu as pltpu

F32, BF16, U32 = jnp.float32, jnp.bfloat16, jnp.uint32
NT = (((1,), (1,)), ((), ()))
MASKED = -1000000000.0
LOG2E = 1.4426950408889634

S, D = 2048, 640
LT = D // 128

AH, AD, AW, ADIL = 32, 20, 8, 2
HALO = 16
TB = 128
NB = S // TB

H, DH, M, SEG = 32, 192, 8, 32
L = M + SEG
HALF = SEG // 2
NSEG = S // SEG
NF = H * DH // 128
SUMS = [(i, j) for i in range(LT) for j in range(i + 1, LT)]
MIXES = [(i, j) for i in range(LT) for j in range(LT) if i != j]

NG = H // 4
TILE = ((1, 2, 0), (3, 4, 5))
PIECES = ((0, 40, 80), (168, 208, 248), (384, 128, 424), (600, 296, 336), (472, 560, 512), (640, 680, 720))


class _Group:
    def __init__(self, j, first):
        u_diag, w_diag = (range(LT), range(LT)) if first + 10 <= NF else (range(4), range(1, 5))
        self.j, self.first = j, first
        self.us = [(first + n, i) for n, i in enumerate(u_diag)]
        self.ws = [(first + len(u_diag) + n, j) for n, j in enumerate(w_diag)]
        self.pairs = [(u, i, w, j) for u, i in self.us for w, j in self.ws if i != j]
        paired = [(u, j) for u, i, w, j in self.pairs] + [(w, i) for u, i, w, j in self.pairs]
        self.direct = [(c, k) for c, d in self.us + self.ws for k in range(LT)
                       if k != d and (c, k) not in paired]
        self.seat = dict(self.us + [(w, LT + j) for w, j in self.ws])


K, Q, V, O = range(4)
GQ = [_Group(j, t) for t in (0, 10, 20) for j in (K, Q, V)]
GQ += [_Group(j, t) for j, t in ((K, 30), (Q, 30), (K, 40), (Q, 40), (V, 30), (V, 40))]
GO = [_Group(O, t) for t in range(0, NF, 10)]
TIMES = {"first": (149, 274, 352, 434, 499, 592, 733, 809, 860),
         "last": (127, 228, 325, 379, 452, 524, 606, 675, 739),
         1: (148, 314, 392, 470, 552, 636, 728, 799, 859),
         0: (138, 314, 389, 481, 551, 633, 725, 806, 863)}


def _first_row(j, c, n):
    return (j * NG + c // 6) * 96 + PIECES[c % 6][n] // 8


def _ds(i, n, size=None):
    return pl.ds(i * n if isinstance(i, int) else pl.multiple_of(i * n, n), size or n)


def _dot(a, b):
    return jnp.dot(a, b, preferred_element_type=F32)


def _recip(x):
    r = pl.reciprocal(x, approx=True)
    return r * (2.0 - x * r)


def _add(a, b):
    return b if a is None else a + b


def _sub(a, b):
    return -b if a is None else a - b


def _total(xs):
    return functools.reduce(jnp.add, xs)


def _vregs(x):
    return [x[r:r + 8] for r in range(0, x.shape[0], 8)]


def _cat(xs):
    return jnp.concatenate(xs, axis=0)


def _share(tasks, k, n):
    return tasks[k * len(tasks) // n:(k + 1) * len(tasks) // n]


def _run(tasks):
    for task in tasks:
        task()


class _Products:
    def __init__(self, events, tied):
        self.events, self.tied, self.results, self.ready = events, tied, [], []
        self.count, self.usual, self.flushed, self.waiting = 0, 0, -1, {}

    def dot(self, x, w):
        self.results.append(_vregs(_dot(self.tied(x), pltpu.bitcast(w, BF16) if w.dtype == U32 else w)))
        return self.results[-1]

    def tick(self):
        self.count += 1
        _run(self.events.pop(self.count - 1, []))

    def now(self, x, w):
        self.tick()
        r = self.dot(x(), w[...])
        self.passed(1)
        return r

    def soon(self, x, w, use):
        self.waiting.setdefault(x.shape[0], []).append([x, w[...], [use]])

    def after(self, rows, task):
        if self.waiting.get(rows):
            self.waiting[rows][-1][2].append(lambda r: task())
        else:
            task()

    def passed(self, n, last=False):
        self.usual += n
        for rows in sorted(self.waiting, reverse=True):
            queue = self.waiting[rows]
            while queue and (last or (len(queue) >= 4 and self.usual % 4 == 0
                                      and (self.flushed < self.usual or len(queue) >= 8 or rows >= L))):
                for x, w, uses in queue[:4]:
                    r = self.dot(x, w)
                    for use in uses:
                        use(r)
                del queue[:4]
                if rows < L:
                    self.flushed = self.usual


def _kernel(ax_hbm, awqkv_hbm, awo_hbm, bx_hbm, mem_hbm, wq_hbm, wk_hbm, wv_hbm, wo_hbm,
            out_hbm,
            ax, awqkv, awo, tmp, wqkv_p, wo_p, x_s, qkv0, qkv1, oa0, oa1, outa,
            bx, mem, raw, cells0, cells1, cells2, raw_o, sums, sums2, sums_o,
            mem_s, f_one, f_sum, f_dif, f_mix, cols0, cols1, part, keys, hold, att, keep, out_x, out_y,
            sources, sem_a, sem_x, sem_w, sem_o):
    qkv, oa, cols = (qkv0, qkv1), (oa0, oa1), (cols0, cols1)
    outb = ax

    cp = pltpu.make_async_copy
    c_wqkv = [cp(awqkv_hbm.at[:, pl.ds(j * D, D)], awqkv.at[j], sem_a.at[j]) for j in range(3)]
    c_awo = cp(awo_hbm, awo, sem_a.at[3])
    c_mem = cp(mem_hbm, mem, sem_a.at[4])
    c_bx = [cp(bx_hbm.at[rows], bx.at[rows], sem_a.at[5 + n])
            for n, rows in enumerate((pl.ds(0, 3 * SEG), pl.ds(3 * SEG, S - 3 * SEG)))]

    def c_ax(i):
        return cp(ax_hbm.at[_ds(i, TB)], ax.at[_ds(i, TB)], sem_x.at[i])

    def c_out(j, rows):
        return cp((outa, outb)[j].at[rows, :], out_hbm.at[rows, pl.ds(j * D, D)], sem_o.at[j])

    def get_w(j, t, n, batch):
        dst, first = (raw_o, t) if j == O else (raw, j * NF + t)
        for k in range(LT):
            cp((wk_hbm, wq_hbm, wv_hbm, wo_hbm)[j].at[_ds(t, 128, 128 * n), _ds(k, 128)],
               dst.at[k, _ds(first, 128, 128 * n)], sem_w.at[batch]).start()

    def got_w(dst, first, n, batch):
        box = dst.at[0:LT, _ds(first, 128, 128 * n)]
        cp(box, box, sem_w.at[batch]).wait()

    ties = []

    def spare(ref, n):
        return ref.at[ref.shape[0] - 1 + zero, _ds(n, 8)]

    def paced(tasks, ref, results):
        for n, task in enumerate(tasks):
            x = results[n * len(results) // len(tasks)]
            spare(ref, 0)[...] = x.astype(BF16) if ref.dtype == BF16 else pltpu.bitcast(x, ref.dtype)
            task()

    def tie(ref):
        ties.append(spare(ref.bitcast(U32) if ref.dtype == BF16 else ref, 1))

    def tied(x):
        head = x[0:8, 0:128]
        while ties:
            ref = ties.pop()
            ref[...] = pltpu.bitcast(head, ref.dtype)
            head = pltpu.bitcast(ref[...], x.dtype)
        if x.shape[1] > 128:
            head = jnp.concatenate([head, x[0:8, 128:]], axis=1)
        return _cat([head, x[8:]]) if x.shape[0] > 8 else head

    def permute_rows(dst, base):
        for d in range(AD):
            for t in range(LT):
                dst[pl.ds((base + d * AH) // 2, AH // 2), t * 128:(t + 1) * 128] = pltpu.bitcast(
                    tmp[t, pl.ds(d, AH, stride=AD), :].astype(BF16), U32)

    def prep_wqkv(j):
        for t in range(LT):
            tmp[t] = awqkv[j, t * 128:(t + 1) * 128, :].astype(F32).T
        permute_rows(wqkv_p, j * D)

    def prep_wo():
        for t in range(LT):
            tmp[t] = awo[:, t * 128:(t + 1) * 128].astype(F32)
        permute_rows(wo_p, 0)

    def a_pass(i, b, c, k0=0, k1=LT):
        lanes = slice(c % LT * 128, c % LT * 128 + 128)
        if c < 3 * LT:
            if c == k0 == 0:
                x_s[b] = ax[_ds(i, TB), :].astype(F32)
            w = pltpu.bitcast(wqkv_p[c * 64:(c + 1) * 64, k0 * 128:k1 * 128], BF16)
            r = lax.dot_general(tied(x_s[b, :, k0 * 128:k1 * 128]), w, NT, preferred_element_type=F32)
        else:
            x = jnp.concatenate([oa[1 - b][k] for k in range(k0, k1)], axis=1)
            r = _dot(tied(x), pltpu.bitcast(wo_p[k0 * 64:k1 * 64, lanes], BF16))
        if k0:
            r = _cat(list(map(_add, _vregs(tmp[c % 4, 0:TB]), _vregs(r))))
        if k1 < LT:
            tmp[c % 4, 0:TB] = r
        elif c >= 3 * LT:
            outa[_ds(i - 1, TB), lanes] = r.astype(BF16)
        else:
            qkv[b][c, HALO:] = r
            if c >= LT and isinstance(i, int) and i == 0:
                qkv[b][c, 0:HALO] = jnp.broadcast_to(r[0:1, :], (HALO, 128))
            elif c >= LT:
                qkv[b][c, 0:HALO] = qkv[1 - b][c, TB:]
        return _vregs(r)

    def a_attention(b, first_block=False):
        state = {}

        def window(c, r0, w):
            return qkv[b][c, HALO + r0 - ADIL * w:HALO + r0 - ADIL * w + 8]

        def logits(r0, ws):
            q = [window(t, r0, 0) for t in range(LT)]
            for w in ws:
                a = _total([q[t] * window(LT + t, r0, w) for t in range(LT)])
                a = _total([a] + [pltpu.roll(a, d, 1) for d in range(AH, 128, AH)])
                if first_block and r0 < ADIL * w:
                    pos = lax.broadcasted_iota(jnp.int32, (8, 128), 0) + r0
                    a = jnp.where(pos >= ADIL * w, a, MASKED * AD ** 0.5)
                state[r0, w] = a

        def mix(r0, ts):
            if ts[0] == 0:
                lg = [state.pop((r0, w)) for w in range(AW)]
                m = functools.reduce(jnp.maximum, lg)
                state[r0] = [jnp.exp2((a - m) * (AD ** -0.5 * LOG2E)) for a in lg]
                state[r0].append(_recip(_total(state[r0])))
            e = state[r0]
            for t in ts:
                oa[b][t, r0:r0 + 8] = _total([e[w] * window(2 * LT + t, r0, w) for w in range(AW)]) * e[AW]

        steps = [(0, logits, range(4)), (0, logits, range(4, AW)), (8, mix, range(1)), (8, mix, range(1, LT))]
        return [functools.partial(f, r0 - lag, some) for r0 in range(0, TB + 8, 8)
                for lag, f, some in steps if 0 <= r0 - lag < TB]

    def place(j, first):
        return first // 10 * 3 + j

    def stored(g, name, at=None, as_words=True):
        n = place(g.j, g.first)
        if name[0] == "cell":
            slot = LT * g.seat[name[1]] + name[2]
            if n == 14:
                return cells2.at[slot]
            return (cells0, cells1)[n % 2].at[50 * ((n if at is None else at) >> 1) + slot]
        ref, n = (sums_o, g.first // 10) if g.j == O else (sums2, n - 13) if n >= 13 else (sums, n)
        if name[0] == "both":
            slot = 20 + MIXES.index((g.seat[name[1]], g.seat[name[2]] - LT))
        else:
            slot = 10 * "-+".index(name[0]) + g.seat[name[1]]
        return (ref.bitcast(U32) if as_words else ref).at[40 * (n if at is None else at) + slot]

    def runs(ref, k, r0, r1, r2):
        return _cat([ref[k, _ds(r, 8, n)] for r, n in ((r0, L), (r1, L), (r2, 128 - 2 * L))])

    def weight(g, name):
        if g.j == O and name[0] == "cell":
            return runs(raw_o, name[2], *[_first_row(0, name[1], n) for n in range(3)])
        return stored(g, name)

    def w_turn(g, at=None):
        def turn(c, k, *rows):
            stored(g, ("cell", c, k), at)[...] = pltpu.bitcast(runs(raw, k, *rows).T, U32)
        tasks = []
        for c, _ in g.us + g.ws:
            rows = [_first_row(g.j, c, n) if at is None else sources[30 * at + 3 * c + n] for n in range(3)]
            tasks += [functools.partial(turn, c, k, *rows) for k in range(LT)]
        return [functools.partial(_run, tasks[n:n + 2]) for n in range(0, len(tasks), 2)]

    def w_combine(g, at=None):
        minus, plus = {}, {}
        pairs = g.pairs if at is None else sorted(g.pairs, key=lambda p: p[3] // 3)

        def get(r, c, k, optional=False):
            if g.j == O:
                rows = [_first_row(0, c, min(n // 5, 2)) + n - 5 * min(n // 5, 2) for n in (r // 8, r // 8 + 1)]
                return _cat([raw_o[k, _ds(n, 8)].astype(F32) for n in rows])
            x = stored(g, ("cell", c, k), at)[r // 2:r // 2 + 8]
            return pltpu.bitcast(jnp.where(at < 12, x, 0) if optional else x, BF16).astype(F32)

        def put(r, x, *name):
            stored(g, name, at, as_words=False)[r:r + 16] = x.astype(BF16)

        def combine(r, pair):
            u, i, w, j = pair
            optional = at is not None and g.j == 0 and (i == LT - 1 or j == 0)
            x, y = get(r, u, j, optional), get(r, w, i, optional)
            put(r, x + y, "both", u, w)
            if g.j == O:
                x, y = y, x
            for c, d, own, other in ((u, i, x, y), (w, j, y, x)):
                mine = [p for p in pairs if c in (p[0], p[2])]
                if pair == mine[0]:
                    minus[c] = plus[c] = get(r, c, d)
                minus[c], plus[c] = minus[c] - own, plus[c] + other
                if pair == mine[-1]:
                    put(r, minus[c], "-", c)
                    put(r, plus[c], "+", c)
        return [functools.partial(combine, r, pair) for r in range(0, 128, 16) for pair in pairs]

    for c in (c_wqkv[0], c_ax(0), c_wqkv[1], c_ax(1)):
        c.start()

    def touch(i, carry):
        for ref in (x_s, f_one, f_sum, f_dif, f_mix, cols0, cols1, part, keys, hold, att, keep,
                    out_x, out_y, tmp, cells0, cells1, cells2, sums, sums2, sums_o):
            ref[(i,) + (0,) * (len(ref.shape) - 3) + (slice(0, 16),)] = jnp.zeros((16, ref.shape[-1]), ref.dtype)
        for ref in (wqkv_p, wo_p):
            ref[_ds(i, 8)] = jnp.zeros((8, D), U32)
        return i
    zero = lax.shift_right_logical(lax.fori_loop(0, 2, touch, 0), 16)

    for g in GQ:
        tiles = {seat: c for c, seat in g.seat.items()}
        for n in range(30):
            sources[30 * place(g.j, g.first) + n] = _first_row(g.j, tiles.get(n // 3, g.first), n % 3)

    c_wqkv[0].wait()
    c_wqkv[2].start()
    prep_wqkv(0)
    c_ax(0).wait()
    c_awo.start()
    c_ax(2).start()
    for c in range(LT):
        a_pass(0, 0, c)
    c_wqkv[1].wait()
    c_ax(1).wait()
    get_w(K, 0, 6, 2)
    prep_wqkv(1)
    for c in range(LT):
        a_pass(1, 1, c)
    c_wqkv[2].wait()
    get_w(K, 6, 5, 2)
    prep_wqkv(2)
    for n in range(2 * LT):
        a_pass(n // LT, n // LT, LT + n % LT)
    c_awo.wait()
    get_w(Q, 0, 6, 3)
    get_w(Q, 6, 5, 3)
    get_w(V, 0, 1, 4)
    for c in (c_ax(3), c_mem, c_bx[0]):
        c.start()
    prep_wo()
    for n in range(2 * LT):
        a_pass(n // LT, n // LT, 2 * LT + n % LT)
    _run(a_attention(0, True))
    for c in range(LT):
        a_pass(1, 1, 3 * LT + c)

    def a_step(it, carry):
        for b in range(2):
            i = 2 * it + b
            third = (i * 43 - 86) >> 7
            t = (i - 2 - 3 * third) * NF + 10 * third
            pl.when(i < 5)(functools.partial(got_w, raw, t, 1, i))
            pl.when(i < 14)(functools.partial(got_w, raw, t + 8, 3, i))
            got_w(raw, t + 1, 7, i)
            c_ax(i).wait()
            third = (i * 43) >> 7
            for j in range(3):
                for t, n, needed in ((1, 7, i < 15), (8, 3, i < 12)):
                    pl.when(needed & (i - 3 * third == j))(functools.partial(get_w, j, 10 * third + t, n, i + 2))
            pl.when(it < NB // 2 - 1)(lambda: c_ax(i + 2).start())
            if b:
                pl.when(i > 12)(lambda: get_w(O, 6 * (i - 13), 6, it - 6))
                pl.when(i == 15)(lambda: get_w(O, 18, 6, 1))
            else:
                pl.when(i == 14)(lambda: get_w(O, 6, 6, 0))
            combine = w_combine(_Group(1 - b, 0), jnp.where(i < 3, 11, i - 3))
            side = [(a_attention(1 - b), 0, 17, 3, qkv[1 - b], oa[1 - b]),
                    (w_turn(_Group(b, 0), i - 2), 22, 5 * LT, 99, raw, (cells0, cells1)[b]),
                    (combine[:90], 0, 17, 2, (cells1, cells0)[b], sums),
                    (combine[90:], 17, 25, 2, (cells1, cells0)[b], sums)]
            rs = []
            for c in range(5 * LT):
                if c % 5 < 4:
                    rs.append(a_pass(i, b, c - c // 5, 0, 4))
                else:
                    rs.append([a_pass(i, b, c // 5 * 4 + n, 4, LT) for n in range(4)][0])
                for tasks, c0, c1, lag, src, dst in side:
                    if c0 <= c < c1:
                        if len(rs) < lag:
                            _run(_share(tasks, c - c0, c1 - c0))
                        else:
                            paced(_share(tasks, c - c0, c1 - c0), src, rs[-lag])
                        tie(dst)
            ties.clear()
        return carry

    lax.fori_loop(1, NB // 2, a_step, 0)
    got_w(raw, V * NF + 41, 7, NB)
    c_mem.wait()
    c_bx[0].wait()
    got_w(raw_o, 0, 12, 0)
    for t in range(24, NF, 6):
        get_w(O, t, 6, 1 if t < 30 else NB + 1)

    def tokens(s):
        return [bx[_ds(s, SEG), k * 128:(k + 1) * 128].astype(F32) for k in range(LT)]

    def project_group(odd, g, product, nm):
        pa, pb = (g.ws, g.us) if odd else (g.us, g.ws)
        half, same, cross = slice(HALF * odd, HALF * odd + HALF), {}, {}

        def with_memory(x, k):
            return _cat([x, f_one[odd, k, SEG:SEG + nm]])

        def prod(lhs, *name):
            return product.now(lhs, weight(g, name))

        def direct(c):
            for _, k in [x for x in g.direct if x[0] == c]:
                r = prod(lambda: f_one[odd, k, 0:SEG + nm], "cell", c, k)
                same[c] = list(map(_add, same[c], r))

        def other(a):
            return cols1.at[g.j, a, M:L] if odd else part.at[place(g.j, a), a % 10]

        def mixed(a, b, r):
            cross[a] = list(map(_add, cross[a] if a in cross else _vregs(other(a)[half]), r))
            for x, h in zip(r, (2 * odd, 2 * odd + 1, *range(4, 9))):
                same[b][h] = same[b][h] + x

        def save_cross(a):
            other(a)[half] = _cat(cross.pop(a))

        def save(c, more=None):
            cols[odd][g.j, c, 0:nm] = _cat(same[c][4:])
            cols[1 - odd][g.j, c, M:L] = _add(more, _cat(same[c][:4]))
        for some in (pb[:-2], pb[-2:]):
            for b, j in some:
                same[b] = list(prod(lambda: with_memory(f_dif[odd, j], j), "+", b))
                direct(b)
            for a, i in pa:
                if a not in same:
                    same[a] = prod(lambda: f_one[odd, i, 0:SEG + nm], "-", a)
                    x = _add(other(a)[...] if odd else None, _cat(same[a][:4]))
                    other(a)[HALF - half.start:SEG - half.start] = x[HALF - half.start:SEG - half.start]
                    cross[a] = _vregs(x[half])
                    direct(a)
                else:
                    same[a] = _vregs(cols[1 - odd][g.j, a, M:L]) + _vregs(cols[odd][g.j, a, 0:nm])
                for b, j in some:
                    if i != j:
                        product.tick()
                        product.soon(with_memory(f_mix[odd, MIXES.index((i, j))], i),
                                     weight(g, ("both", b, a) if odd else ("both", a, b)),
                                     functools.partial(mixed, a, b))
                for b, j in some:
                    if i != j:
                        r = prod(lambda: f_sum[odd, SUMS.index((min(i, j), max(i, j))), 0:SEG + nm], "cell", a, j)
                        same[a] = list(map(_add, same[a], r))
                        same[b] = list(map(_sub, same[b], r))
                save(a)
                product.after(HALF + nm, functools.partial(save_cross, a))
            for b, _ in some:
                product.after(HALF + nm, functools.partial(save, b, part[place(g.j, b), b % 10] if odd else None))
        product.after(HALF + nm, lambda: product.ready.extend((g.j, c) for c in g.seat))

    def last_queries(g, product):
        product.passed(0, True)
        for w, i in g.ws:
            r = list(map(_add, _vregs(cols1[Q, w, M:L]), product.now(lambda: f_one[1, i, 0:SEG], weight(g, ("-", w)))))
            for u, j in g.us:
                if i != j:
                    x = product.now(lambda: f_mix[1, MIXES.index((i, j))], weight(g, ("both", u, w)))
                    r[2:] = list(map(_add, r[2:], x))
            cols1[Q, w, M:L] = _cat(r)
        product.ready += [(Q, c) for c in g.seat]

    def out_groups(odd, gs, same, cross, product, last):
        h0, nh = (0, SEG * odd) if last else (2 - 2 * odd, HALF)
        mix = {}

        def xa(c, r0=0, n=SEG):
            return att[c, M + SEG * (1 - odd) + r0:M + SEG * (1 - odd) + r0 + n]

        def xb(c, r0=0, n=SEG):
            return att[c, L + r0:L + r0 + n] if odd else keep[c, r0:r0 + n]

        def xm(c):
            return att[c, 0:M]

        def prod(g, m, x, *name):
            r = product.now(lambda: x() if last else _cat([m(), x()]), weight(g, name))
            return r if last else r[1:] + r[:1]

        def mixed(s, t, r):
            mix[s, t] = list(map(_add, mix.get((s, t), [None] * 4), r))

        def spend(s, t):
            for x, h in zip(mix.pop((s, t), []), list(range(h0, h0 + nh // 8)) + [4]):
                same[t][h] = _add(same[t][h], x)
                if h < 4:
                    cross[s][h] = _add(cross[s][h], x)
        sides = [(g, {d: c for c, d in (g.us if odd else g.ws)}, {d: c for c, d in (g.ws if odd else g.us)})
                 for g in gs]
        for i in range(LT):
            shared = [None] * 5
            for g, pa, pb in sides:
                rs = [prod(g, lambda: xm(pb[i]), lambda: xa(pb[i]) - xb(pb[i]), "+", pb[i])] if i in pb else []
                rs += [prod(g, lambda: xm(c), lambda: xa(c), "cell", c, k) for c, k in g.direct if k == i]
                for r in rs:
                    same[i] = list(map(_add, same[i], r))
                if i in pa:
                    shared = list(map(_add, shared, prod(g, lambda: xm(pa[i]), lambda: xa(pa[i]), "-", pa[i])))
                    if odd:
                        keep[pa[i]] = xa(pa[i])
            same[i] = list(map(_add, same[i], shared))
            cross[i] = list(map(_add, cross[i], shared))
            for j in range(i + 1, LT):
                diff = [None] * 5
                for s, t in ((i, j), (j, i)):
                    for g, pa, pb in sides:
                        if s in pa and t in pb:
                            a, b = pa[s], pb[t]
                            if nh:
                                product.tick()
                                x = xa(a, 8 * h0, nh) + xb(b, 8 * h0, nh)
                                product.soon(x if last else _cat([x, xm(a)]),
                                             weight(g, ("both", a, b) if odd else ("both", b, a)),
                                             functools.partial(mixed, s, t))
                            r = prod(g, lambda: xm(a) + xm(b), lambda: xa(a) + xa(b), "cell", b, s)
                            diff = list(map(_add if s == i else _sub, diff, r))
                    product.after(nh if last else nh + M, functools.partial(spend, s, t))
                same[i] = list(map(_add, same[i], diff))
                same[j] = list(map(_sub, same[j], diff))

    def project_out(odd, s, product, last=False):
        same, cross = [[None] * 5 for _ in range(LT)], [[None] * 4 for _ in range(LT)]
        for gs in (GO[:3], GO[3:]):
            assert all((O, c) in product.ready for g in gs for c in g.seat)
            out_groups(odd, gs, same, cross, product, last)
        product.passed(0, True)
        for k in range(LT):
            lanes = slice(k * 128, (k + 1) * 128)
            if odd:
                out_x[k], out_y[k] = _cat(same[k][:4]), _cat(cross[k])
            else:
                outb[_ds(s - 2, SEG), lanes] = (out_x[k] + _cat(cross[k])).astype(BF16)
                outb[_ds(s - 1, SEG), lanes] = (out_y[k] + _cat(same[k][:4])).astype(BF16)
        return [x[-1] for x in same]

    def attend(odd, s, m, product, last=False):
        xa, xb = tokens(jnp.minimum(s + 1, NSEG - 1)), tokens(s if odd else jnp.minimum(s + 2, NSEG - 1))
        nm = m[0].shape[0]
        for k in range(LT):
            f_one[odd, k, 0:SEG + m[k].shape[0]] = _cat([xa[k], m[k]])
            f_dif[odd, k] = xa[k] - xb[k]
        for n, (i, j) in enumerate(SUMS):
            f_sum[odd, n, 0:SEG + nm] = _cat([xa[i] + xa[j], m[i] + m[j]])
        for n, (i, j) in enumerate(MIXES):
            f_mix[odd, n] = (xa[i] + xb[j])[HALF * odd:HALF * odd + HALF]

        lane = lax.broadcasted_iota(jnp.int32, (L, 128), 1)
        zone = [(lane >= L * z) & (lane < L * z + L) for z in range(3)]
        some = [(lane >= 24 + 16 * n) & (lane < 40 + 16 * n) for n in range(2)]

        def tile(j, g, n, z):
            assert (j, 6 * g + TILE[n][z]) in product.ready
            return cols[odd][j, 6 * g + TILE[n][z]]

        def gathered(j, g, n):
            x = jnp.where(zone[2], tile(j, g, n, 2), 0.0) if j == K else tile(j, g, n, 2)
            return jnp.where(zone[0], tile(j, g, n, 0), jnp.where(zone[1], tile(j, g, n, 1), x))

        def stack(xs):
            return _cat(xs + [jnp.zeros((8, 128), F32)])

        def by_head(x, a, of_a):
            xs = [jnp.zeros((L, 128), F32)] * 2 + [x]
            if a < 2:
                xs[a], xs[2] = jnp.where(of_a, x, 0.0), jnp.where(of_a, 0.0, x)
            return stack(xs)

        def turned(slot, x):
            keys[slot] = x.T
            return keys[slot]

        def one_pass(x, w):
            r = _dot(x, w.astype(BF16))
            product.passed(1)
            return _cat(_vregs(r))

        def done(g, n, z, o):
            product.ready.append((O, 6 * g + TILE[n][z]))
            att[6 * g + TILE[n][z], 0:M] = o[0:M]
            att[6 * g + TILE[n][z], M + SEG * odd:L + SEG * odd] = o[M:L]

        def alone(j, g):
            sc = {}
            for z in (2, 1, 0):
                for n in range(2):
                    w = by_head(tile(j, g, n, z), z, ~zone[z] | some[n] if z == n else ~zone[z])
                    if j == V:
                        p = hold[g, 2 + n] if z in (2, n) else jnp.where(zone[2], hold[g, 2 + n], hold[g, 2 + z])
                        done(g, n, z, one_pass(p, w))
                        continue
                    r = one_pass(tile(Q, g, n, z), turned(3 * n + z, w))
                    if z in (2, n):
                        sc[n] = _add(sc.get(n), r)
                    else:
                        sc[n], sc[z] = sc[n] + jnp.where(zone[2], r, 0.0), sc[z] + jnp.where(zone[2], 0.0, r)
            for n in sc:
                hold[g, n] = sc[n]

        def together(g):
            for n in range(2):
                turned(4 * g + 2 + n, stack([tile(K, g, n, z) for z in range(3)]))
            for n in range(2):
                hold[g, n] = one_pass(gathered(Q, g, n), turned(4 * g + 4 + n, by_head(gathered(K, g, n), n, some[n])))
            for n in range(2):
                hold[g - 1, 4 + n] = one_pass(hold[g - 1, 2 + n], by_head(gathered(V, g - 1, n), n, some[n]))
                for z in range(3):
                    h = n if z == 2 else z
                    w = [jnp.where(zone[z][0:8], y, 0.0) for y in _vregs(keys[4 * g + 2 + n])]
                    w[5 * z:5 * z + 5] = [jnp.where(zone[z], 0.0, tile(V, g - 1, n, z))]
                    r = one_pass(jnp.where(zone[z], hold[g - 1, 2 + h], tile(Q, g, n, z)), _cat(w))
                    hold[g, h] = hold[g, h] + jnp.where(zone[z], r, 0.0)
                    done(g - 1, n, z, jnp.where(zone[z], hold[g - 1, 4 + n], r))

        def softmax(g):
            ahead = lane[0:8] % L - lax.broadcasted_iota(jnp.int32, (8, 128), 0)
            for n in range(2):
                x = _cat([jnp.where(ahead <= 8 * b, y, MASKED * DH ** 0.5) if b else y
                          for b, y in enumerate(_vregs(hold[g, n]))])
                top = [jnp.max(jnp.where(zone[z], x, -jnp.inf), axis=1, keepdims=True) for z in (n, 2)]
                e = jnp.exp2((x - jnp.where(zone[2], top[1], top[0])) * (DH ** -0.5 * LOG2E))
                e = [jnp.where(zone[z], e, 0.0) for z in (n, 2)]
                total = [jnp.sum(y, axis=1, keepdims=True) for y in e]
                hold[g, 2 + n] = (e[0] + e[1]) * _recip(jnp.where(zone[2], total[1], total[0]))

        for g, t in enumerate(TIMES["last" if last else "first" if nm > M else odd]):
            tasks = [functools.partial(alone, V if g else K, max(g - 1, 0)) if g % NG == 0 else functools.partial(together, g)]
            product.events.setdefault(t, []).extend(tasks + [functools.partial(softmax, g)] * (g < NG))
        for g in GQ:
            if last and g.j == Q:
                last_queries(g, product)
            else:
                project_group(odd, g, product, nm)
        return product

    first = _Products({}, tied)

    def spread(tasks, t0, t1, src=None, dst=None):
        def run(some):
            if src is None or len(first.results) < 16:
                _run(some)
            else:
                paced(some, src, first.results[-16])
            if dst is not None:
                tie(dst)
        for t in range(t0, t1):
            if _share(tasks, t - t0, t1 - t0):
                first.events.setdefault(t, []).append(functools.partial(run, _share(tasks, t - t0, t1 - t0)))

    def a_last(c, k):
        def use(r):
            x = _cat(list(map(_add, _vregs(tmp[c, 0:TB]), r)) if k else r)
            if k < LT - 1:
                tmp[c, 0:TB] = x
            else:
                outa[S - TB:S, c * 128:(c + 1) * 128] = x.astype(BF16)
        first.soon(oa1[k], wo_p.at[k * 64:(k + 1) * 64, c * 128:(c + 1) * 128], use)

    end = 3 * NF * LT
    spread(a_attention(1), 12, 138, qkv1, oa1)
    spread(w_turn(_Group(V, 40)), 138, 138 + 1)
    spread(w_combine(_Group(Q, 40)), 138, 223, cells1, sums2)
    spread(w_combine(GO[0]), 223, 311, raw_o, sums_o)
    spread([lambda: tie(cells2)], 311 - 20, 311 - 19)
    spread(w_combine(_Group(V, 40)), 311, 378, cells2, sums2)
    spread([lambda: got_w(raw_o, 12, 18, 1), c_bx[1].start], 378, 378 + 1)
    spread(w_combine(GO[1]) + w_combine(GO[2]), 378 + 6, 572, raw_o, sums_o)
    spread([lambda: got_w(raw_o, 30, 18, NB + 1)], 572, 572 + 1)
    spread(w_combine(GO[3]) + w_combine(GO[4]), 572 + 6, end + 32, raw_o, sums_o)
    spread([functools.partial(a_last, c, k) for k in range(LT) for c in range(LT)], end, end + LT * NF)
    attend(0, 0, [_cat([mem[:, k * 128:(k + 1) * 128].astype(F32), x]) for k, x in enumerate(tokens(0))], first)
    first.passed(0, True)
    m = [None] * LT
    for c in range(NF):
        assert (O, c) in first.ready
        for k in range(LT):
            m[k] = _add(m[k], first.now(lambda: att[c, 0:M], weight(GO[c // 10], ("cell", c, k)))[0])
    first.passed(0, True)
    for k in range(LT):
        mem_s[k] = m[k]
    c_out(0, pl.ds(0, S)).start()
    c_bx[1].wait()

    def b_step(n, carry):
        m = [mem_s[k] for k in range(LT)]
        for odd in (1, 0):
            m = project_out(odd, 2 * n + 2 - odd, attend(odd, 2 * n + 2 - odd, m, _Products({}, tied)))
        for k in range(LT):
            mem_s[k] = m[k]
        c_out(1, _ds(n, 2 * SEG)).start()
        return carry

    lax.fori_loop(0, NSEG // 2 - 1, b_step, 0)
    final = attend(1, NSEG - 1, [mem_s[k] for k in range(LT)], _Products({}, tied), last=True)
    final.passed(0, True)
    project_out(1, NSEG - 1, final, last=True)
    project_out(0, NSEG, final, last=True)
    c_out(1, _ds(NSEG // 2 - 1, 2 * SEG)).start()
    for j in range(2):
        c_out(j, pl.ds(0, S)).wait()


def pallas_concat_heads__sliding_local_dilated__memory_aug_recurrent_mem_tr__prompt_kernel(
    A_x, A_wqkv, A_wo, B_x, B_mem0, B_Wq, B_Wk, B_Wv, B_Wo, B_seg_len,
):
    assert B_seg_len == SEG
    assert A_x.shape == B_x.shape == (1, S, D) and B_mem0.shape == (1, M, D)
    assert B_Wq.shape == B_Wk.shape == B_Wv.shape == (D, H, DH) and B_Wo.shape == (H, DH, D)
    vmem, dma = pltpu.VMEM, pltpu.SemaphoreType.DMA
    call = pl.pallas_call(
        _kernel,
        out_shape=jax.ShapeDtypeStruct((S, 2 * D), BF16),
        in_specs=[pl.BlockSpec(memory_space=pl.ANY)] * 9,
        out_specs=pl.BlockSpec(memory_space=pl.ANY),
        scratch_shapes=[
            vmem((S, D), BF16),
            vmem((3, D, D), BF16),
            vmem((D, D), BF16),
            vmem((LT, D, 128), F32),
            vmem((3 * D // 2, D), U32),
            vmem((D // 2, D), U32),
            vmem((2, TB, D), F32),
            vmem((3 * LT + 1, HALO + TB, 128), F32), vmem((3 * LT + 1, HALO + TB, 128), F32),
            vmem((LT + 1, TB, 128), F32), vmem((LT + 1, TB, 128), F32),
            vmem((S, D), BF16),
            vmem((S, D), BF16),
            vmem((M, D), BF16),
            vmem((LT, 3 * NF * 128, 128), BF16),
            vmem((351, 64, 128), U32), vmem((351, 64, 128), U32), vmem((51, 64, 128), U32),
            vmem((LT + 1, NF * 128, 128), BF16),
            vmem((521, 128, 128), BF16), vmem((81, 128, 128), BF16), vmem((201, 128, 128), BF16),
            vmem((LT, M, 128), F32),
            vmem((2, LT, L + SEG, 128), F32),
            vmem((2, len(SUMS), L + SEG, 128), F32),
            vmem((2, LT, SEG, 128), F32),
            vmem((2, len(MIXES), HALF, 128), F32),
            vmem((3, NF, L, 128), F32), vmem((3, NF, L, 128), F32),
            vmem((len(GQ), LT, SEG, 128), F32),
            vmem((4 * NG + 2, 128, 128), F32),
            vmem((NG, 6, L, 128), F32),
            vmem((NF, L + SEG, 128), F32),
            vmem((NF, SEG, 128), F32),
            vmem((LT, SEG, 128), F32), vmem((LT, SEG, 128), F32),
            pltpu.SMEM((30 * len(GQ),), jnp.int32),
            dma((7,)), dma((NB,)), dma((NB + 2,)), dma((2,)),
        ],
        compiler_params=pltpu.CompilerParams(
            vmem_limit_bytes=124 * 1024 * 1024, disable_bounds_checks=True, disable_semaphore_checks=True),
        name="sliding_and_memory_attention",
    )

    def by_feature(w):
        return w.transpose(1, 2, 0).reshape(H * DH, D)

    out = call(A_x.reshape(S, D), A_wqkv, A_wo, B_x.reshape(S, D), B_mem0.reshape(M, D),
               by_feature(B_Wq), by_feature(B_Wk), by_feature(B_Wv), B_Wo.reshape(H * DH, D))
    return out.reshape(1, S, 2 * D)
```

```python
import functools

import jax
import jax.numpy as jnp
from jax import lax
from jax.experimental import pallas as pl
from jax.experimental.pallas import tpu as pltpu

F32, BF16, U32 = jnp.float32, jnp.bfloat16, jnp.uint32
NT = (((1,), (1,)), ((), ()))
MASKED = -1000000000.0
LOG2E = 1.4426950408889634

S, D = 2048, 640
LT = D // 128

AH, AD, AW, ADIL = 32, 20, 8, 2
HALO = 16
TB = 128
NB = S // TB

H, DH, M, SEG = 32, 192, 8, 32
L = M + SEG
HALF = SEG // 2
NSEG = S // SEG
NF = H * DH // 128
SUMS = [(i, j) for i in range(LT) for j in range(i + 1, LT)]
MIXES = [(i, j) for i in range(LT) for j in range(LT) if i != j]

NG = H // 4
TILE = ((1, 2, 0), (3, 4, 5))
PIECES = ((0, 40, 80), (168, 208, 248), (384, 128, 424), (600, 296, 336), (472, 560, 512), (640, 680, 720))


class _Group:
    def __init__(self, j, first):
        u_diag, w_diag = (range(LT), range(LT)) if first + 10 <= NF else (range(4), range(1, 5))
        self.j, self.first = j, first
        self.us = [(first + n, i) for n, i in enumerate(u_diag)]
        self.ws = [(first + len(u_diag) + n, j) for n, j in enumerate(w_diag)]
        self.pairs = [(u, i, w, j) for u, i in self.us for w, j in self.ws if i != j]
        paired = [(u, j) for u, i, w, j in self.pairs] + [(w, i) for u, i, w, j in self.pairs]
        self.direct = [(c, k) for c, d in self.us + self.ws for k in range(LT)
                       if k != d and (c, k) not in paired]
        self.seat = dict(self.us + [(w, LT + j) for w, j in self.ws])


K, Q, V, O = range(4)
GQ = [_Group(j, t) for t in (0, 10, 20) for j in (K, Q, V)]
GQ += [_Group(j, t) for j, t in ((K, 30), (Q, 30), (K, 40), (Q, 40), (V, 30), (V, 40))]
GO = [_Group(O, t) for t in range(0, NF, 10)]
TIMES = {"first": (149, 274, 352, 434, 499, 592, 733, 809, 860),
         "last": (127, 228, 325, 379, 452, 524, 606, 675, 739),
         1: (148, 314, 392, 470, 552, 636, 728, 799, 859),
         0: (138, 314, 389, 481, 551, 633, 725, 806, 863)}


def _first_row(j, c, n):
    return (j * NG + c // 6) * 96 + PIECES[c % 6][n] // 8


def _ds(i, n, size=None):
    return pl.ds(i * n if isinstance(i, int) else pl.multiple_of(i * n, n), size or n)


def _dot(a, b):
    return jnp.dot(a, b, preferred_element_type=F32)


def _recip(x):
    r = pl.reciprocal(x, approx=True)
    return r * (2.0 - x * r)


def _add(a, b):
    return b if a is None else a + b


def _sub(a, b):
    return -b if a is None else a - b


def _total(xs):
    return functools.reduce(jnp.add, xs)


def _vregs(x):
    return [x[r:r + 8] for r in range(0, x.shape[0], 8)]


def _cat(xs):
    return jnp.concatenate(xs, axis=0)


def _share(tasks, k, n):
    return tasks[k * len(tasks) // n:(k + 1) * len(tasks) // n]


def _run(tasks):
    for task in tasks:
        task()


class _Products:
    def __init__(self, events, tied):
        self.events, self.tied, self.results, self.ready = events, tied, [], []
        self.count, self.usual, self.flushed, self.waiting = 0, 0, -1, {}

    def dot(self, x, w):
        self.results.append(_vregs(_dot(self.tied(x), pltpu.bitcast(w, BF16) if w.dtype == U32 else w)))
        return self.results[-1]

    def tick(self):
        self.count += 1
        _run(self.events.pop(self.count - 1, []))

    def now(self, x, w):
        self.tick()
        r = self.dot(x(), w[...])
        self.passed(1)
        return r

    def soon(self, x, w, use):
        self.waiting.setdefault(x.shape[0], []).append([x, w[...], [use]])

    def after(self, rows, task):
        if self.waiting.get(rows):
            self.waiting[rows][-1][2].append(lambda r: task())
        else:
            task()

    def passed(self, n, last=False):
        self.usual += n
        for rows in sorted(self.waiting, reverse=True):
            queue = self.waiting[rows]
            while queue and (last or (len(queue) >= 4 and self.usual % 4 == 0
                                      and (self.flushed < self.usual or len(queue) >= 8 or rows >= L))):
                for x, w, uses in queue[:4]:
                    r = self.dot(x, w)
                    for use in uses:
                        use(r)
                del queue[:4]
                if rows < L:
                    self.flushed = self.usual


def _kernel(ax_hbm, awqkv_hbm, awo_hbm, bx_hbm, mem_hbm, wq_hbm, wk_hbm, wv_hbm, wo_hbm,
            out_hbm,
            ax, awqkv, awo, tmp, wqkv_p, wo_p, x_s, qkv0, qkv1, oa0, oa1, outa,
            bx, mem, raw, cells0, cells1, cells2, raw_o, sums, sums2, sums_o,
            mem_s, f_one, f_sum, f_dif, f_mix, cols0, cols1, part, keys, hold, att, keep, out_x, out_y,
            sources, sem_a, sem_x, sem_w, sem_o):
    qkv, oa, cols = (qkv0, qkv1), (oa0, oa1), (cols0, cols1)
    outb = ax

    cp = pltpu.make_async_copy
    c_wqkv = [cp(awqkv_hbm.at[:, pl.ds(j * D, D)], awqkv.at[j], sem_a.at[j]) for j in range(3)]
    c_awo = cp(awo_hbm, awo, sem_a.at[3])
    c_mem = cp(mem_hbm, mem, sem_a.at[4])
    c_bx = [cp(bx_hbm.at[rows], bx.at[rows], sem_a.at[5 + n])
            for n, rows in enumerate((pl.ds(0, 3 * SEG), pl.ds(3 * SEG, S - 3 * SEG)))]

    def c_ax(i):
        return cp(ax_hbm.at[_ds(i, TB)], ax.at[_ds(i, TB)], sem_x.at[i])

    def c_out(j, rows):
        return cp((outa, outb)[j].at[rows, :], out_hbm.at[rows, pl.ds(j * D, D)], sem_o.at[j])

    def get_w(j, t, n, batch):
        dst, first = (raw_o, t) if j == O else (raw, j * NF + t)
        for k in range(LT):
            cp((wk_hbm, wq_hbm, wv_hbm, wo_hbm)[j].at[_ds(t, 128, 128 * n), _ds(k, 128)],
               dst.at[k, _ds(first, 128, 128 * n)], sem_w.at[batch]).start()

    def got_w(dst, first, n, batch):
        box = dst.at[0:LT, _ds(first, 128, 128 * n)]
        cp(box, box, sem_w.at[batch]).wait()

    ties = []

    def spare(ref, n):
        return ref.at[ref.shape[0] - 1 + zero, _ds(n, 8)]

    def paced(tasks, ref, results):
        for n, task in enumerate(tasks):
            x = results[n * len(results) // len(tasks)]
            spare(ref, 0)[...] = x.astype(BF16) if ref.dtype == BF16 else pltpu.bitcast(x, ref.dtype)
            task()

    def tie(ref):
        ties.append(spare(ref.bitcast(U32) if ref.dtype == BF16 else ref, 1))

    def tied(x):
        head = x[0:8, 0:128]
        while ties:
            ref = ties.pop()
            ref[...] = pltpu.bitcast(head, ref.dtype)
            head = pltpu.bitcast(ref[...], x.dtype)
        if x.shape[1] > 128:
            head = jnp.concatenate([head, x[0:8, 128:]], axis=1)
        return _cat([head, x[8:]]) if x.shape[0] > 8 else head

    def permute_rows(dst, base):
        for d in range(AD):
            for t in range(LT):
                dst[pl.ds((base + d * AH) // 2, AH // 2), t * 128:(t + 1) * 128] = pltpu.bitcast(
                    tmp[t, pl.ds(d, AH, stride=AD), :].astype(BF16), U32)

    def prep_wqkv(j):
        for t in range(LT):
            tmp[t] = awqkv[j, t * 128:(t + 1) * 128, :].astype(F32).T
        permute_rows(wqkv_p, j * D)

    def prep_wo():
        for t in range(LT):
            tmp[t] = awo[:, t * 128:(t + 1) * 128].astype(F32)
        permute_rows(wo_p, 0)

    def a_pass(i, b, c, k0=0, k1=LT):
        lanes = slice(c % LT * 128, c % LT * 128 + 128)
        if c < 3 * LT:
            if c == k0 == 0:
                x_s[b] = pltpu.bitcast(ax[_ds(i, TB), :], U32)
            w = pltpu.bitcast(wqkv_p[c * 64:(c + 1) * 64, k0 * 128:k1 * 128], BF16)
            r = lax.dot_general(pltpu.bitcast(tied(x_s[b, :, k0 * 128:k1 * 128]), BF16), w, NT, preferred_element_type=F32)
        else:
            x = jnp.concatenate([oa[1 - b][k] for k in range(k0, k1)], axis=1)
            r = _dot(tied(x), pltpu.bitcast(wo_p[k0 * 64:k1 * 64, lanes], BF16))
        if k0:
            r = _cat(list(map(_add, _vregs(tmp[c % 4, 0:TB]), _vregs(r))))
        if k1 < LT:
            tmp[c % 4, 0:TB] = r
        elif c >= 3 * LT:
            outa[_ds(i - 1, TB), lanes] = r.astype(BF16)
        else:
            qkv[b][c, HALO:] = r
            if c >= LT and isinstance(i, int) and i == 0:
                qkv[b][c, 0:HALO] = jnp.broadcast_to(r[0:1, :], (HALO, 128))
            elif c >= LT:
                qkv[b][c, 0:HALO] = qkv[1 - b][c, TB:]
        return _vregs(r)

    def a_attention(b, first_block=False):
        state = {}

        def window(c, r0, w):
            return qkv[b][c, HALO + r0 - ADIL * w:HALO + r0 - ADIL * w + 8]

        def logits(r0, ws):
            q = [window(t, r0, 0) for t in range(LT)]
            for w in ws:
                a = _total([q[t] * window(LT + t, r0, w) for t in range(LT)])
                a = _total([a] + [pltpu.roll(a, d, 1) for d in range(AH, 128, AH)])
                if first_block and r0 < ADIL * w:
                    pos = lax.broadcasted_iota(jnp.int32, (8, 128), 0) + r0
                    a = jnp.where(pos >= ADIL * w, a, MASKED * AD ** 0.5)
                state[r0, w] = a

        def mix(r0, ts):
            if ts[0] == 0:
                lg = [state.pop((r0, w)) for w in range(AW)]
                m = functools.reduce(jnp.maximum, lg)
                state[r0] = [jnp.exp2((a - m) * (AD ** -0.5 * LOG2E)) for a in lg]
                state[r0].append(_recip(_total(state[r0])))
            e = state[r0]
            for t in ts:
                oa[b][t, r0:r0 + 8] = _total([e[w] * window(2 * LT + t, r0, w) for w in range(AW)]) * e[AW]

        steps = [(0, logits, range(4)), (0, logits, range(4, AW)), (8, mix, range(1)), (8, mix, range(1, LT))]
        return [functools.partial(f, r0 - lag, some) for r0 in range(0, TB + 8, 8)
                for lag, f, some in steps if 0 <= r0 - lag < TB]

    def place(j, first):
        return first // 10 * 3 + j

    def stored(g, name, at=None, as_words=True):
        n = place(g.j, g.first)
        if name[0] == "cell":
            slot = LT * g.seat[name[1]] + name[2]
            if n == 14:
                return cells2.at[slot]
            return (cells0, cells1)[n % 2].at[50 * ((n if at is None else at) >> 1) + slot]
        ref, n = (sums_o, g.first // 10) if g.j == O else (sums2, n - 13) if n >= 13 else (sums, n)
        if name[0] == "both":
            slot = 20 + MIXES.index((g.seat[name[1]], g.seat[name[2]] - LT))
        else:
            slot = 10 * "-+".index(name[0]) + g.seat[name[1]]
        return (ref.bitcast(U32) if as_words else ref).at[40 * (n if at is None else at) + slot]

    def runs(ref, k, r0, r1, r2):
        return _cat([ref[k, _ds(r, 8, n)] for r, n in ((r0, L), (r1, L), (r2, 128 - 2 * L))])

    def weight(g, name):
        if g.j == O and name[0] == "cell":
            return runs(raw_o, name[2], *[_first_row(0, name[1], n) for n in range(3)])
        return stored(g, name)

    def w_turn(g, at=None):
        def turn(c, k, *rows):
            stored(g, ("cell", c, k), at)[...] = pltpu.bitcast(runs(raw, k, *rows).T, U32)
        tasks = []
        for c, _ in g.us + g.ws:
            rows = [_first_row(g.j, c, n) if at is None else sources[30 * at + 3 * c + n] for n in range(3)]
            tasks += [functools.partial(turn, c, k, *rows) for k in range(LT)]
        return [functools.partial(_run, tasks[n:n + 2]) for n in range(0, len(tasks), 2)]

    def w_combine(g, at=None):
        minus, plus = {}, {}
        pairs = g.pairs if at is None else sorted(g.pairs, key=lambda p: p[3] // 3)

        def get(r, c, k, optional=False):
            if g.j == O:
                rows = [_first_row(0, c, min(n // 5, 2)) + n - 5 * min(n // 5, 2) for n in (r // 8, r // 8 + 1)]
                return _cat([raw_o[k, _ds(n, 8)].astype(F32) for n in rows])
            x = stored(g, ("cell", c, k), at)[r // 2:r // 2 + 8]
            return pltpu.bitcast(jnp.where(at < 12, x, 0) if optional else x, BF16).astype(F32)

        def put(r, x, *name):
            stored(g, name, at, as_words=False)[r:r + 16] = x.astype(BF16)

        def combine(r, pair):
            u, i, w, j = pair
            optional = at is not None and g.j == 0 and (i == LT - 1 or j == 0)
            x, y = get(r, u, j, optional), get(r, w, i, optional)
            put(r, x + y, "both", u, w)
            if g.j == O:
                x, y = y, x
            for c, d, own, other in ((u, i, x, y), (w, j, y, x)):
                mine = [p for p in pairs if c in (p[0], p[2])]
                if pair == mine[0]:
                    minus[c] = plus[c] = get(r, c, d)
                minus[c], plus[c] = minus[c] - own, plus[c] + other
                if pair == mine[-1]:
                    put(r, minus[c], "-", c)
                    put(r, plus[c], "+", c)
        return [functools.partial(combine, r, pair) for r in range(0, 128, 16) for pair in pairs]

    for c in (c_wqkv[0], c_ax(0), c_wqkv[1], c_ax(1)):
        c.start()

    def touch(i, carry):
        for ref in (x_s, f_one, f_sum, f_dif, f_mix, cols0, cols1, part, keys, hold, att, keep,
                    out_x, out_y, tmp, cells0, cells1, cells2, sums, sums2, sums_o):
            ref[(i,) + (0,) * (len(ref.shape) - 3) + (slice(0, 16),)] = jnp.zeros((16, ref.shape[-1]), ref.dtype)
        for ref in (wqkv_p, wo_p):
            ref[_ds(i, 8)] = jnp.zeros((8, D), U32)
        return i
    zero = lax.shift_right_logical(lax.fori_loop(0, 2, touch, 0), 16)

    for g in GQ:
        tiles = {seat: c for c, seat in g.seat.items()}
        for n in range(30):
            sources[30 * place(g.j, g.first) + n] = _first_row(g.j, tiles.get(n // 3, g.first), n % 3)

    c_wqkv[0].wait()
    c_wqkv[2].start()
    prep_wqkv(0)
    c_ax(0).wait()
    c_awo.start()
    c_ax(2).start()
    for c in range(LT):
        a_pass(0, 0, c)
    c_wqkv[1].wait()
    c_ax(1).wait()
    get_w(K, 0, 6, 2)
    prep_wqkv(1)
    for c in range(LT):
        a_pass(1, 1, c)
    c_wqkv[2].wait()
    get_w(K, 6, 5, 2)
    prep_wqkv(2)
    for n in range(2 * LT):
        a_pass(n // LT, n // LT, LT + n % LT)
    c_awo.wait()
    get_w(Q, 0, 6, 3)
    get_w(Q, 6, 5, 3)
    get_w(V, 0, 1, 4)
    for c in (c_ax(3), c_mem, c_bx[0]):
        c.start()
    prep_wo()
    for n in range(2 * LT):
        a_pass(n // LT, n // LT, 2 * LT + n % LT)
    _run(a_attention(0, True))
    for c in range(LT):
        a_pass(1, 1, 3 * LT + c)

    def a_step(it, carry):
        for b in range(2):
            i = 2 * it + b
            third = (i * 43 - 86) >> 7
            t = (i - 2 - 3 * third) * NF + 10 * third
            pl.when(i < 5)(functools.partial(got_w, raw, t, 1, i))
            pl.when(i < 14)(functools.partial(got_w, raw, t + 8, 3, i))
            got_w(raw, t + 1, 7, i)
            c_ax(i).wait()
            third = (i * 43) >> 7
            for j in range(3):
                for t, n, needed in ((1, 7, i < 15), (8, 3, i < 12)):
                    pl.when(needed & (i - 3 * third == j))(functools.partial(get_w, j, 10 * third + t, n, i + 2))
            pl.when(it < NB // 2 - 1)(lambda: c_ax(i + 2).start())
            pl.when(i >= 12)(lambda: get_w(O, 6 * (i - 12), 6, it - 6))
            combine = w_combine(_Group(1 - b, 0), jnp.where(i < 3, 11, i - 3))
            side = [(a_attention(1 - b), 0, 17, 3, qkv[1 - b], oa[1 - b]),
                    (w_turn(_Group(b, 0), i - 2), 22, 5 * LT, 99, raw, (cells0, cells1)[b]),
                    (combine[:90], 0, 17, 2, (cells1, cells0)[b], sums),
                    (combine[90:], 17, 25, 2, (cells1, cells0)[b], sums)]
            rs = []
            for c in range(5 * LT):
                if c % 5 < 4:
                    rs.append(a_pass(i, b, c - c // 5, 0, 4))
                else:
                    rs.append([a_pass(i, b, c // 5 * 4 + n, 4, LT) for n in range(4)][0])
                for tasks, c0, c1, lag, src, dst in side:
                    if c0 <= c < c1:
                        if len(rs) < lag:
                            _run(_share(tasks, c - c0, c1 - c0))
                        else:
                            paced(_share(tasks, c - c0, c1 - c0), src, rs[-lag])
                        tie(dst)
            ties.clear()
        return carry

    lax.fori_loop(1, NB // 2, a_step, 0)
    got_w(raw, V * NF + 41, 7, NB)
    c_mem.wait()
    c_bx[0].wait()
    got_w(raw_o, 0, 12, 0)
    for t in range(24, NF, 6):
        get_w(O, t, 6, 1 if t < 30 else NB + 1)

    def tokens(s):
        return [bx[_ds(s, SEG), k * 128:(k + 1) * 128].astype(F32) for k in range(LT)]

    def project_group(odd, g, product, nm):
        pa, pb = (g.ws, g.us) if odd else (g.us, g.ws)
        half, same, cross = slice(HALF * odd, HALF * odd + HALF), {}, {}

        def with_memory(x, k):
            return _cat([x, f_one[odd, k, SEG:SEG + nm]])

        def prod(lhs, *name):
            return product.now(lhs, weight(g, name))

        def direct(c):
            for _, k in [x for x in g.direct if x[0] == c]:
                r = prod(lambda: f_one[odd, k, 0:SEG + nm], "cell", c, k)
                same[c] = list(map(_add, same[c], r))

        def other(a):
            return cols1.at[g.j, a, M:L] if odd else part.at[place(g.j, a), a % 10]

        def mixed(a, b, r):
            cross[a] = list(map(_add, cross[a] if a in cross else _vregs(other(a)[half]), r))
            for x, h in zip(r, (2 * odd, 2 * odd + 1, *range(4, 9))):
                same[b][h] = same[b][h] + x

        def save_cross(a):
            other(a)[half] = _cat(cross.pop(a))

        def save(c, more=None):
            cols[odd][g.j, c, 0:nm] = _cat(same[c][4:])
            cols[1 - odd][g.j, c, M:L] = _add(more, _cat(same[c][:4]))
        for some in (pb[:-2], pb[-2:]):
            for b, j in some:
                same[b] = list(prod(lambda: with_memory(f_dif[odd, j], j), "+", b))
                direct(b)
            for a, i in pa:
                if a not in same:
                    same[a] = prod(lambda: f_one[odd, i, 0:SEG + nm], "-", a)
                    x = _add(other(a)[...] if odd else None, _cat(same[a][:4]))
                    other(a)[HALF - half.start:SEG - half.start] = x[HALF - half.start:SEG - half.start]
                    cross[a] = _vregs(x[half])
                    direct(a)
                else:
                    same[a] = _vregs(cols[1 - odd][g.j, a, M:L]) + _vregs(cols[odd][g.j, a, 0:nm])
                for b, j in some:
                    if i != j:
                        product.tick()
                        product.soon(with_memory(f_mix[odd, MIXES.index((i, j))], i),
                                     weight(g, ("both", b, a) if odd else ("both", a, b)),
                                     functools.partial(mixed, a, b))
                for b, j in some:
                    if i != j:
                        r = prod(lambda: f_sum[odd, SUMS.index((min(i, j), max(i, j))), 0:SEG + nm], "cell", a, j)
                        same[a] = list(map(_add, same[a], r))
                        same[b] = list(map(_sub, same[b], r))
                save(a)
                product.after(HALF + nm, functools.partial(save_cross, a))
            for b, _ in some:
                product.after(HALF + nm, functools.partial(save, b, part[place(g.j, b), b % 10] if odd else None))
        product.after(HALF + nm, lambda: product.ready.extend((g.j, c) for c in g.seat))

    def last_queries(g, product):
        product.passed(0, True)
        for w, i in g.ws:
            r = list(map(_add, _vregs(cols1[Q, w, M:L]), product.now(lambda: f_one[1, i, 0:SEG], weight(g, ("-", w)))))
            for u, j in g.us:
                if i != j:
                    x = product.now(lambda: f_mix[1, MIXES.index((i, j))], weight(g, ("both", u, w)))
                    r[2:] = list(map(_add, r[2:], x))
            cols1[Q, w, M:L] = _cat(r)
        product.ready += [(Q, c) for c in g.seat]

    def out_groups(odd, gs, same, cross, product, last):
        h0, nh = (0, SEG * odd) if last else (2 - 2 * odd, HALF)
        mix = {}

        def xa(c, r0=0, n=SEG):
            return att[c, M + SEG * (1 - odd) + r0:M + SEG * (1 - odd) + r0 + n]

        def xb(c, r0=0, n=SEG):
            return att[c, L + r0:L + r0 + n] if odd else keep[c, r0:r0 + n]

        def xm(c):
            return att[c, 0:M]

        def prod(g, m, x, *name):
            r = product.now(lambda: x() if last else _cat([m(), x()]), weight(g, name))
            return r if last else r[1:] + r[:1]

        def mixed(s, t, r):
            mix[s, t] = list(map(_add, mix.get((s, t), [None] * 4), r))

        def spend(s, t):
            for x, h in zip(mix.pop((s, t), []), list(range(h0, h0 + nh // 8)) + [4]):
                same[t][h] = _add(same[t][h], x)
                if h < 4:
                    cross[s][h] = _add(cross[s][h], x)
        sides = [(g, {d: c for c, d in (g.us if odd else g.ws)}, {d: c for c, d in (g.ws if odd else g.us)})
                 for g in gs]
        for i in range(LT):
            shared = [None] * 5
            for g, pa, pb in sides:
                rs = [prod(g, lambda: xm(pb[i]), lambda: xa(pb[i]) - xb(pb[i]), "+", pb[i])] if i in pb else []
                rs += [prod(g, lambda: xm(c), lambda: xa(c), "cell", c, k) for c, k in g.direct if k == i]
                for r in rs:
                    same[i] = list(map(_add, same[i], r))
                if i in pa:
                    shared = list(map(_add, shared, prod(g, lambda: xm(pa[i]), lambda: xa(pa[i]), "-", pa[i])))
                    if odd:
                        keep[pa[i]] = xa(pa[i])
            same[i] = list(map(_add, same[i], shared))
            cross[i] = list(map(_add, cross[i], shared))
            for j in range(i + 1, LT):
                diff = [None] * 5
                for s, t in ((i, j), (j, i)):
                    for g, pa, pb in sides:
                        if s in pa and t in pb:
                            a, b = pa[s], pb[t]
                            if nh:
                                product.tick()
                                x = xa(a, 8 * h0, nh) + xb(b, 8 * h0, nh)
                                product.soon(x if last else _cat([x, xm(a)]),
                                             weight(g, ("both", a, b) if odd else ("both", b, a)),
                                             functools.partial(mixed, s, t))
                            r = prod(g, lambda: xm(a) + xm(b), lambda: xa(a) + xa(b), "cell", b, s)
                            diff = list(map(_add if s == i else _sub, diff, r))
                    product.after(nh if last else nh + M, functools.partial(spend, s, t))
                same[i] = list(map(_add, same[i], diff))
                same[j] = list(map(_sub, same[j], diff))

    def project_out(odd, s, product, last=False):
        same, cross = [[None] * 5 for _ in range(LT)], [[None] * 4 for _ in range(LT)]
        for gs in (GO[:3], GO[3:]):
            assert all((O, c) in product.ready for g in gs for c in g.seat)
            out_groups(odd, gs, same, cross, product, last)
        product.passed(0, True)
        for k in range(LT):
            lanes = slice(k * 128, (k + 1) * 128)
            if odd:
                out_x[k], out_y[k] = _cat(same[k][:4]), _cat(cross[k])
            else:
                outb[_ds(s - 2, SEG), lanes] = (out_x[k] + _cat(cross[k])).astype(BF16)
                outb[_ds(s - 1, SEG), lanes] = (out_y[k] + _cat(same[k][:4])).astype(BF16)
        return [x[-1] for x in same]

    def attend(odd, s, m, product, last=False):
        xa, xb = tokens(jnp.minimum(s + 1, NSEG - 1)), tokens(s if odd else jnp.minimum(s + 2, NSEG - 1))
        nm = m[0].shape[0]
        for k in range(LT):
            f_one[odd, k, 0:SEG + m[k].shape[0]] = _cat([xa[k], m[k]])
            f_dif[odd, k] = xa[k] - xb[k]
        for n, (i, j) in enumerate(SUMS):
            f_sum[odd, n, 0:SEG + nm] = _cat([xa[i] + xa[j], m[i] + m[j]])
        for n, (i, j) in enumerate(MIXES):
            f_mix[odd, n] = (xa[i] + xb[j])[HALF * odd:HALF * odd + HALF]

        lane = lax.broadcasted_iota(jnp.int32, (L, 128), 1)
        zone = [(lane >= L * z) & (lane < L * z + L) for z in range(3)]
        some = [(lane >= 24 + 16 * n) & (lane < 40 + 16 * n) for n in range(2)]

        def tile(j, g, n, z):
            assert (j, 6 * g + TILE[n][z]) in product.ready
            return cols[odd][j, 6 * g + TILE[n][z]]

        def gathered(j, g, n):
            x = jnp.where(zone[2], tile(j, g, n, 2), 0.0) if j == K else tile(j, g, n, 2)
            return jnp.where(zone[0], tile(j, g, n, 0), jnp.where(zone[1], tile(j, g, n, 1), x))

        def stack(xs):
            return _cat(xs + [jnp.zeros((8, 128), F32)])

        def by_head(x, a, of_a):
            xs = [jnp.zeros((L, 128), F32)] * 2 + [x]
            if a < 2:
                xs[a], xs[2] = jnp.where(of_a, x, 0.0), jnp.where(of_a, 0.0, x)
            return stack(xs)

        def turned(slot, x):
            keys[slot] = x.T
            return keys[slot]

        def one_pass(x, w):
            r = _dot(x, w.astype(BF16))
            product.passed(1)
            return _cat(_vregs(r))

        def done(g, n, z, o):
            product.ready.append((O, 6 * g + TILE[n][z]))
            att[6 * g + TILE[n][z], 0:M] = o[0:M]
            att[6 * g + TILE[n][z], M + SEG * odd:L + SEG * odd] = o[M:L]

        def alone(j, g):
            sc = {}
            for z in (2, 1, 0):
                for n in range(2):
                    w = by_head(tile(j, g, n, z), z, ~zone[z] | some[n] if z == n else ~zone[z])
                    if j == V:
                        p = hold[g, 2 + n] if z in (2, n) else jnp.where(zone[2], hold[g, 2 + n], hold[g, 2 + z])
                        done(g, n, z, one_pass(p, w))
                        continue
                    r = one_pass(tile(Q, g, n, z), turned(3 * n + z, w))
                    if z in (2, n):
                        sc[n] = _add(sc.get(n), r)
                    else:
                        sc[n], sc[z] = sc[n] + jnp.where(zone[2], r, 0.0), sc[z] + jnp.where(zone[2], 0.0, r)
            for n in sc:
                hold[g, n] = sc[n]

        def together(g):
            for n in range(2):
                turned(4 * g + 2 + n, stack([tile(K, g, n, z) for z in range(3)]))
            for n in range(2):
                hold[g, n] = one_pass(gathered(Q, g, n), turned(4 * g + 4 + n, by_head(gathered(K, g, n), n, some[n])))
            for n in range(2):
                hold[g - 1, 4 + n] = one_pass(hold[g - 1, 2 + n], by_head(gathered(V, g - 1, n), n, some[n]))
                for z in range(3):
                    h = n if z == 2 else z
                    w = [jnp.where(zone[z][0:8], y, 0.0) for y in _vregs(keys[4 * g + 2 + n])]
                    w[5 * z:5 * z + 5] = [jnp.where(zone[z], 0.0, tile(V, g - 1, n, z))]
                    r = one_pass(jnp.where(zone[z], hold[g - 1, 2 + h], tile(Q, g, n, z)), _cat(w))
                    hold[g, h] = hold[g, h] + jnp.where(zone[z], r, 0.0)
                    done(g - 1, n, z, jnp.where(zone[z], hold[g - 1, 4 + n], r))

        def softmax(g):
            ahead = lane[0:8] % L - lax.broadcasted_iota(jnp.int32, (8, 128), 0)
            for n in range(2):
                x = _cat([jnp.where(ahead <= 8 * b, y, MASKED * DH ** 0.5) if b else y
                          for b, y in enumerate(_vregs(hold[g, n]))])
                top = [jnp.max(jnp.where(zone[z], x, -jnp.inf), axis=1, keepdims=True) for z in (n, 2)]
                e = jnp.exp2((x - jnp.where(zone[2], top[1], top[0])) * (DH ** -0.5 * LOG2E))
                e = [jnp.where(zone[z], e, 0.0) for z in (n, 2)]
                total = [jnp.sum(y, axis=1, keepdims=True) for y in e]
                hold[g, 2 + n] = (e[0] + e[1]) * _recip(jnp.where(zone[2], total[1], total[0]))

        for g, t in enumerate(TIMES["last" if last else "first" if nm > M else odd]):
            tasks = [functools.partial(alone, V if g else K, max(g - 1, 0)) if g % NG == 0 else functools.partial(together, g)]
            product.events.setdefault(t, []).extend(tasks + [functools.partial(softmax, g)] * (g < NG))
        for g in GQ:
            if last and g.j == Q:
                last_queries(g, product)
            else:
                project_group(odd, g, product, nm)
        return product

    first = _Products({}, tied)

    def spread(tasks, t0, t1, src=None, dst=None):
        def run(some):
            if src is None or len(first.results) < 16:
                _run(some)
            else:
                paced(some, src, first.results[-16])
            if dst is not None:
                tie(dst)
        for t in range(t0, t1):
            if _share(tasks, t - t0, t1 - t0):
                first.events.setdefault(t, []).append(functools.partial(run, _share(tasks, t - t0, t1 - t0)))

    def a_last(c, k):
        def use(r):
            x = _cat(list(map(_add, _vregs(tmp[c, 0:TB]), r)) if k else r)
            if k < LT - 1:
                tmp[c, 0:TB] = x
            else:
                outa[S - TB:S, c * 128:(c + 1) * 128] = x.astype(BF16)
        first.soon(oa1[k], wo_p.at[k * 64:(k + 1) * 64, c * 128:(c + 1) * 128], use)

    end = 3 * NF * LT
    spread(a_attention(1), 12, 138, qkv1, oa1)
    spread(w_turn(_Group(V, 40)), 138, 138 + 1)
    spread(w_combine(_Group(Q, 40)), 138, 223, cells1, sums2)
    spread(w_combine(GO[0]), 223, 311, raw_o, sums_o)
    spread([lambda: tie(cells2)], 311 - 20, 311 - 19)
    spread(w_combine(_Group(V, 40)), 311, 378, cells2, sums2)
    spread([lambda: got_w(raw_o, 12, 18, 1), c_bx[1].start], 378, 378 + 1)
    spread(w_combine(GO[1]) + w_combine(GO[2]), 378 + 6, 572, raw_o, sums_o)
    spread([lambda: got_w(raw_o, 30, 18, NB + 1)], 572, 572 + 1)
    spread(w_combine(GO[3]) + w_combine(GO[4]), 572 + 6, end + 32, raw_o, sums_o)
    spread([functools.partial(a_last, c, k) for k in range(LT) for c in range(LT)], end, end + LT * NF)
    attend(0, 0, [_cat([mem[:, k * 128:(k + 1) * 128].astype(F32), x]) for k, x in enumerate(tokens(0))], first)
    first.passed(0, True)
    m = [None] * LT
    for c in range(NF):
        assert (O, c) in first.ready
        for k in range(LT):
            m[k] = _add(m[k], first.now(lambda: att[c, 0:M], weight(GO[c // 10], ("cell", c, k)))[0])
    first.passed(0, True)
    for k in range(LT):
        mem_s[k] = m[k]
    c_out(0, pl.ds(0, S)).start()
    c_bx[1].wait()

    def b_step(n, carry):
        m = [mem_s[k] for k in range(LT)]
        for odd in (1, 0):
            m = project_out(odd, 2 * n + 2 - odd, attend(odd, 2 * n + 2 - odd, m, _Products({}, tied)))
        for k in range(LT):
            mem_s[k] = m[k]
        c_out(1, _ds(n, 2 * SEG)).start()
        return carry

    lax.fori_loop(0, NSEG // 2 - 1, b_step, 0)
    final = attend(1, NSEG - 1, [mem_s[k] for k in range(LT)], _Products({}, tied), last=True)
    final.passed(0, True)
    project_out(1, NSEG - 1, final, last=True)
    project_out(0, NSEG, final, last=True)
    c_out(1, _ds(NSEG // 2 - 1, 2 * SEG)).start()
    for j in range(2):
        c_out(j, pl.ds(0, S)).wait()


def pallas_concat_heads__sliding_local_dilated__memory_aug_recurrent_mem_tr__prompt_kernel(
    A_x, A_wqkv, A_wo, B_x, B_mem0, B_Wq, B_Wk, B_Wv, B_Wo, B_seg_len,
):
    assert B_seg_len == SEG
    assert A_x.shape == B_x.shape == (1, S, D) and B_mem0.shape == (1, M, D)
    assert B_Wq.shape == B_Wk.shape == B_Wv.shape == (D, H, DH) and B_Wo.shape == (H, DH, D)
    vmem, dma = pltpu.VMEM, pltpu.SemaphoreType.DMA
    call = pl.pallas_call(
        _kernel,
        out_shape=jax.ShapeDtypeStruct((S, 2 * D), BF16),
        in_specs=[pl.BlockSpec(memory_space=pl.ANY)] * 9,
        out_specs=pl.BlockSpec(memory_space=pl.ANY),
        scratch_shapes=[
            vmem((S, D), BF16),
            vmem((3, D, D), BF16),
            vmem((D, D), BF16),
            vmem((LT, D, 128), F32),
            vmem((3 * D // 2, D), U32),
            vmem((D // 2, D), U32),
            vmem((2, TB // 2, D), U32),
            vmem((3 * LT + 1, HALO + TB, 128), F32), vmem((3 * LT + 1, HALO + TB, 128), F32),
            vmem((LT + 1, TB, 128), F32), vmem((LT + 1, TB, 128), F32),
            vmem((S, D), BF16),
            vmem((S, D), BF16),
            vmem((M, D), BF16),
            vmem((LT, 3 * NF * 128, 128), BF16),
            vmem((351, 64, 128), U32), vmem((351, 64, 128), U32), vmem((51, 64, 128), U32),
            vmem((LT + 1, NF * 128, 128), BF16),
            vmem((521, 128, 128), BF16), vmem((81, 128, 128), BF16), vmem((201, 128, 128), BF16),
            vmem((LT, M, 128), F32),
            vmem((2, LT, L + SEG, 128), F32),
            vmem((2, len(SUMS), L + SEG, 128), F32),
            vmem((2, LT, SEG, 128), F32),
            vmem((2, len(MIXES), HALF, 128), F32),
            vmem((3, NF, L, 128), F32), vmem((3, NF, L, 128), F32),
            vmem((len(GQ), LT, SEG, 128), F32),
            vmem((4 * NG + 2, 128, 128), F32),
            vmem((NG, 6, L, 128), F32),
            vmem((NF, L + SEG, 128), F32),
            vmem((NF, SEG, 128), F32),
            vmem((LT, SEG, 128), F32), vmem((LT, SEG, 128), F32),
            pltpu.SMEM((30 * len(GQ),), jnp.int32),
            dma((7,)), dma((NB,)), dma((NB + 2,)), dma((2,)),
        ],
        compiler_params=pltpu.CompilerParams(
            vmem_limit_bytes=124 * 1024 * 1024, disable_bounds_checks=True, disable_semaphore_checks=True),
        name="sliding_and_memory_attention",
    )

    def by_feature(w):
        return w.transpose(1, 2, 0).reshape(H * DH, D)

    out = call(A_x.reshape(S, D), A_wqkv, A_wo, B_x.reshape(S, D), B_mem0.reshape(M, D),
               by_feature(B_Wq), by_feature(B_Wk), by_feature(B_Wv), B_Wo.reshape(H * DH, D))
    return out.reshape(1, S, 2 * D)
```
